```python
import jax
import jax.numpy as jnp

def _softmax(x, axis=-1):
    return jax.nn.softmax(x, axis=axis)

def _gelu(x):
    return jax.nn.gelu(x, approximate=True)

def _silu(x):
    return jax.nn.silu(x)

def _sigmoid(x):
    return jax.nn.sigmoid(x)

def _layernorm(x, axis=-1, eps=1e-05):
    m = jnp.mean(x, axis=axis, keepdims=True)
    v = jnp.var(x, axis=axis, keepdims=True)
    return (x - m) / jnp.sqrt(v + eps)

def _scatter_add(tgt, idx, src, axis=0):
    return tgt.at[idx].add(src)

def _segment_sum(src, seg, n):
    return jax.ops.segment_sum(src, seg, n)

class _Rng:

    def __init__(self, key):
        self._k = key

    def _next(self):
        self._k, sub = jax.random.split(self._k)
        return sub

    def normal(self, shape):
        return jax.random.normal(self._next(), shape, dtype=jnp.bfloat16)

    def randint(self, lo, hi, shape):
        return jax.random.randint(self._next(), shape, lo, hi, dtype=jnp.int32)

    def uniform(self, shape, lo=0.0, hi=1.0):
        return jax.random.uniform(self._next(), shape, jnp.bfloat16, lo, hi)

    def permutation(self, n):
        return jax.random.permutation(self._next(), n)
kernel_name = 'standalone__conformer_family_branchformer__speech'

def setup_inputs():
    _rng = _Rng(jax.random.key(int.from_bytes(__import__("os").urandom(4), "little")))
    _w = lambda a: (lambda t: t.astype(jnp.bfloat16) if jnp.issubdtype(t.dtype, jnp.floating) else t)(jnp.asarray(a))
    B, T, D, K = (2, 4000, 512, 31)
    s = float(D) ** (-0.5)
    return {'x': _w((lambda *s: _rng.normal(s) * 0.05)(B, T, D)), 'w_q': _w((lambda *s: _rng.normal(s) * 0.05)(D, D) * s), 'w_k': _w((lambda *s: _rng.normal(s) * 0.05)(D, D) * s), 'w_v': _w((lambda *s: _rng.normal(s) * 0.05)(D, D) * s), 'w_ao': _w((lambda *s: _rng.normal(s) * 0.05)(D, D) * s), 'w_up': _w((lambda *s: _rng.normal(s) * 0.05)(D, 2 * D) * s), 'dw': _w((lambda *s: _rng.normal(s) * 0.05)(K, D) * (1.0 / K)), 'w_dn': _w((lambda *s: _rng.normal(s) * 0.05)(D, D) * s), 'w_merge': _w((lambda *s: _rng.normal(s) * 0.05)(2 * D, D) * s)}

def reference(x, w_q, w_k, w_v, w_ao, w_up, dw, w_dn, w_merge):
    B, T, D = x.shape
    K = dw.shape[0]
    xa = _layernorm(x, axis=-1)
    q = jnp.einsum('btd,de->bte', xa, w_q)
    k = jnp.einsum('btd,de->bte', xa, w_k)
    v = jnp.einsum('btd,de->bte', xa, w_v)
    logits = jnp.einsum('btd,bsd->bts', q, k) * float(D) ** (-0.5)
    attn = _softmax(logits, axis=-1)
    ya = jnp.einsum('bts,bsd->btd', attn, v)
    ya = jnp.einsum('btd,de->bte', ya, w_ao)
    xc = _layernorm(x, axis=-1)
    h = _gelu(jnp.einsum('btd,de->bte', xc, w_up))
    u = h[..., :D].copy()
    g = _layernorm(h[..., D:], axis=-1)
    pad = K // 2
    gp = jnp.pad(g, ((0, 0), (pad, pad), (0, 0)))
    conv = jnp.zeros_like(g)
    for i in range(K):
        conv = conv + gp[:, i:i + T, :] * dw[i][None, None, :]
    yc = jnp.einsum('btd,de->bte', u * conv, w_dn)
    merged = jnp.concatenate([ya, yc], axis=-1)
    out = jnp.einsum('btf,fd->btd', merged, w_merge)
    return x + out
```

```python
import functools
import math
import jax
import jax.numpy as jnp
from jax import lax
from jax.experimental import pallas as pl
from jax.experimental.pallas import tpu as pltpu

F32 = jnp.float32
BF16 = jnp.bfloat16
U32 = jnp.uint32
EPS = 1e-5
LOG2E = 1.4426950408889634
HALO = 16


def _ln(x):
    m = jnp.mean(x, axis=-1, keepdims=True)
    c = x - m
    v = jnp.mean(c * c, axis=-1, keepdims=True)
    return c * lax.rsqrt(v + EPS)


def _gelu(x):
    c0 = math.sqrt(2.0 / math.pi)
    inner = x * (c0 + (c0 * 0.044715) * (x * x))
    hx = 0.5 * x
    return hx + hx * jnp.tanh(inner)


def _dot(a, b):
    return jnp.dot(a, b, preferred_element_type=F32)


def _dot_nt(a, b):
    return lax.dot_general(a, b, (((1,), (1,)), ((), ())), preferred_element_type=F32)


def _pack(x):
    return pltpu.bitcast(x.astype(BF16), U32)


def _unpack(x):
    return pltpu.bitcast(x, BF16)


def _split(x):
    r, c = x.shape
    return x[:r // 2, :c // 2], x[:r // 2, c // 2:], x[r // 2:, :c // 2], x[r // 2:, c // 2:]


def _join(c11, c12, c21, c22):
    return jnp.concatenate([jnp.concatenate([c11, c12], axis=1),
                            jnp.concatenate([c21, c22], axis=1)], axis=0)


def _ops(x, level, kind):
    if level == 0:
        return [x]
    x11, x12, x21, x22 = _split(x)
    if kind == "a":
        ops = [x11 + x22, x21 + x22, x11, x22, x11 + x12, x21 - x11, x12 - x22]
    elif kind == "b":
        ops = [x11 + x22, x11, x12 - x22, x21 - x11, x22, x11 + x12, x21 + x22]
    else:
        ops = [x11 + x22, x11, x21 - x22, x12 - x11, x22, x11 + x21, x12 + x22]
    return [z for o in ops for z in _ops(o, level - 1, kind)]


_A_AS_B = (0, 6, 1, 4, 5, 3, 2)


def _a_as_b(i, level):
    if level == 0:
        return 0
    n = 7 ** (level - 1)
    return _A_AS_B[i // n] * n + _a_as_b(i % n, level - 1)


ORDER = (0, 3, 4, 6, 2, 1, 5)


def _order(level, order=ORDER):
    if level == 0:
        return [0]
    n = 7 ** (level - 1)
    return [j * n + k for j in order for k in _order(level - 1, order)]


def _combine(get, level, transposed=False, base=0):
    if level == 0:
        return get(base)
    n = 7 ** (level - 1)
    sub = lambda j: _combine(get, level - 1, transposed, base + j * n)
    m0 = sub(0)
    m3 = sub(3)
    t = m0 + m3
    m4 = sub(4)
    t = t - m4
    m6 = sub(6)
    c11 = t + m6
    m2 = sub(2)
    c12 = m2 + m4
    t = m0 + m2
    m1 = sub(1)
    c21 = m1 + m3
    t = t - m1
    m5 = sub(5)
    c22 = t + m5
    if transposed:
        c12, c21 = c21, c12
    return _join(c11, c12, c21, c22)


def _vregs(x):
    return [x[r:r + 8, c:c + 128] for r in range(0, x.shape[0], 8) for c in range(0, x.shape[1], 128)]


def _pack_rows(x):
    return pltpu.bitcast(x.astype(BF16), U32)


def _zip(x):
    return pltpu.pack_elementwise([x[0:8], x[8:16]], packed_dtype=BF16)


def _unzip(x, gate=lambda w: w):
    w = gate(pltpu.bitcast(x, U32))
    return jnp.concatenate([pltpu.unpack_elementwise(w, index=n, packed_dtype=BF16, unpacked_dtype=F32)
                            for n in range(2)], axis=0)


def _tree(xs, arity):
    part = [functools.reduce(lambda a, b: a | b, xs[n::arity]) for n in range(min(arity, len(xs)))]
    while len(part) > 1:
        part = [functools.reduce(lambda a, b: a | b, part[n:n + 2]) for n in range(0, len(part), 2)]
    return part[0]


class Pacer:
    def __init__(self, zero, arity):
        self.arity = arity
        self.keep = lax.broadcasted_iota(jnp.int32, (8, 128), 0) >= zero
        self.tasks, self.due = [], []
        self.recent = []
        self.back = 0

    def spread(self, tasks, nslots, lag=0, back=0, parts=1):
        assert not self.tasks and not self.due
        self.tasks = list(tasks)
        self.rate = sum(c for _, c in tasks) / (nslots - lag)
        self.end = nslots - 1
        self.credit = tasks[0][1]
        self.slot, self.lag, self.back, self.parts = 0, lag, back, parts

    def seen(self, y):
        self.recent.append(y[0:8, 0:128])
        return y

    def after(self, x):
        tok = pltpu.bitcast(self.recent[max(0, len(self.recent) - 1 - self.back)], x.dtype)
        return jnp.concatenate([jnp.concatenate(
            [jnp.where(self.keep, x[r:r + 8, c:c + 128], tok) for c in range(0, x.shape[1], 128)], axis=1)
            for r in range(0, x.shape[0], 8)], axis=0)

    def tie(self, lhs):
        rows = []
        for r in range(0, lhs.shape[0], 8):
            t = lhs[r:r + 8]
            while self.tasks and self.credit >= self.tasks[0][1] * (1 - 1e-6):
                fn, cost = self.tasks.pop(0)
                self.credit -= cost
                out = [pltpu.bitcast(v, U32) for v in fn()]
                n = min(len(out), self.parts)
                for m in range(n):
                    part = out[m * len(out) // n:(m + 1) * len(out) // n]
                    when = min(self.end, self.slot + self.lag + m * cost / self.rate / n)
                    self.due.append((when, _tree(part, self.arity)))
                self.due.sort(key=lambda d: d[0])
            mine = None
            while self.due and self.due[0][0] <= self.slot:
                tok = self.due.pop(0)[1]
                mine = tok if mine is None else mine | tok
            self.slot += 1
            self.credit += self.rate
            if mine is not None:
                t0 = jnp.where(self.keep, t[:, 0:128], mine)
                t = t0 if t.shape[1] == 128 else jnp.concatenate([t0, t[:, 128:]], axis=1)
            rows.append(t)
        return _unpack(jnp.concatenate(rows, axis=0))


def _merge(xs, ys):
    if not ys:
        return xs
    keyed = [((n + 0.5) / len(xs), 0, n) for n in range(len(xs))] + [((n + 0.5) / len(ys), 1, n) for n in range(len(ys))]
    return [(xs, ys)[w][n] for _, w, n in sorted(keyed)]


def make(bm=448, LA=2, wq=128, chunks=(512, 512), R=64, rc=16, rs=16, nmid=2, flags=None, qk_frac=1.0,
         pv_frac=1.0, skip=1, pcost=70, scost=70, ptok=7, gsplit=(0.0, 0.0, 0.0), tailu=True, chains=1, phase=0.0, split=False, lag=(10, 30, 10, 6), back=(1, 6, 2, 0), arity=3, parts=(7, 7, 4, 2), rel=True, relscale=True, relsum=False):
    na = 2 ** LA
    nprod = 7 ** LA
    bq = bm // na
    rg = 16

    def kernel(xf_ref, xn_ref, xr_ref, wq_ref, wk_ref, wv_ref, wao_ref, wup_ref, dw_ref, wdn_ref, wm_ref,
               o_ref, wp_ref, dwf_ref, kv_ref, xa_ref, q_ref, u_ref, uc_ref, g_ref, gn_ref, s_ref,
               m_ref, yc_ref, hg_ref, hq_ref, hu_ref, acc_ref, ob_ref, ga_ref, *p_refs, nq):
        step = pl.program_id(0)
        i = step % nq
        T, D = xf_ref.shape
        Tp = s_ref.shape[1]
        K = dw_ref.shape[0]
        pad = K // 2
        nl = D // 128
        kw = Tp // na
        W = lambda w: _unpack(wp_ref[w])
        zero = pl.multiple_of(jnp.minimum(step, 0) * 8, 8)
        row16 = lax.broadcasted_iota(jnp.int32, (16, 1), 0)
        unzipped16 = 2 * (row16 % 8) + row16 // 8

        def fence(ref, val=None):
            idx = tuple(n - 1 for n in ref.shape[:-2]) + (pl.ds(zero + ref.shape[-2] - 8, 8), pl.ds(0, 128))
            ref[idx] = jnp.zeros((8, 128), ref.dtype) if val is None else pltpu.bitcast(val[-8:, -128:], ref.dtype)

        def norm_tasks(load, r0, gate=lambda w: w):
            def task(r):
                y = _zip(_ln(jnp.where(r0 + r + unzipped16 < T, _unzip(load(r), gate), 0.0)))
                xa_ref[r // 2:r // 2 + 8, :] = y
                if r + 16 == bm:
                    fence(xa_ref, y)
                return _vregs(y)
            return [(functools.partial(task, r), 40) for r in range(0, bm, 16)]

        def act_tasks(gate=lambda w: w):
            def task(r):
                y = _gelu(gate(hg_ref[r:r + 16, :]))
                ga_ref[r:r + 16, :] = y
                if r + 16 == bm:
                    fence(ga_ref, y)
                return _vregs(y)
            return [(functools.partial(task, r), 24) for r in range(HALO, bm, 16)]

        def gate_tasks(r0, gate=lambda w: w):
            def task(r):
                y = _gelu(gate(hg_ref[r:r + 16, :])) if r < HALO or not split else gate(ga_ref[r:r + 16, :])
                g = jnp.where(r0 + r + row16 < T, _ln(y), 0.0)
                for c in range(nl):
                    gn_ref[c, r:r + 16, :] = g[:, c * 128:(c + 1) * 128]
                    if r < HALO:
                        g_ref[c, HALO + bm + r:HALO + bm + r + 16, :] = g[:, c * 128:(c + 1) * 128]
                if r + 16 == bm:
                    fence(gn_ref, g)
                return _vregs(g)
            return [(functools.partial(task, r), 30) for r in range(0, bm, 16)]

        def u_tasks(gate=lambda w: w):
            def task(r):
                y = _gelu(gate(hu_ref[r:r + 16, :]))
                u_ref[r:r + 16, :] = y
                return _vregs(y)
            return [(functools.partial(task, r), 24) for r in range(0, bm, 16)]

        def q_tasks():
            def task(r):
                x = jnp.concatenate([hq_ref[a * bq + r:a * bq + r + 16, :] for a in range(na)], axis=0)
                zs = [_zip(z) for z in _ops(x, LA, "bt")]
                for j, z in enumerate(zs):
                    q_ref[j, r // 2:r // 2 + 8, :] = z
                return [v for z in zs for v in _vregs(z)]
            return [(functools.partial(task, r), 55) for r in range(0, bq, 16)]

        def shift_tasks():
            def head():
                out = []
                for c in range(nl):
                    y = g_ref[c, bm:bm + HALO, :]
                    g_ref[c, 0:HALO, :] = y
                    out += _vregs(y)
                return out

            def task(r):
                out = []
                for c in range(nl):
                    y = gn_ref[c, r:r + 32, :]
                    g_ref[c, HALO + r:HALO + r + 32, :] = y
                    out += _vregs(y)
                return out
            return [(head, 8)] + [(functools.partial(task, r), 16) for r in range(0, bm, 32)]

        @pl.when(step == 0)
        def _():
            wp_ref[0] = _pack_rows(_dot_nt(wq_ref[...], wk_ref[...]) * (LOG2E * float(D) ** -0.5))
            wp_ref[1] = pltpu.bitcast(wup_ref[:, 0:D], U32)
            wp_ref[2] = pltpu.bitcast(wup_ref[:, D:2 * D], U32)
            t = _dot(wv_ref[...], wao_ref[...]).astype(BF16)
            wp_ref[3] = _pack_rows(_dot(t, wm_ref[0:D, :]))
            wp_ref[4] = _pack_rows(_dot(wdn_ref[...], wm_ref[D:2 * D, :]))
            dwf_ref[0:K, :] = dw_ref[...].astype(F32)
            for t, _ in norm_tasks(lambda r: xf_ref[r:r + 16, :], 0):
                t()
            xa = _unpack(xa_ref[0:bm // 2, :])
            hg_ref[0:bm, :] = _dot(xa, W(2))
            hu_ref[0:bm, :] = _dot(xa, W(1))
            hq_ref[0:bm, :] = _dot(xa, W(0))
            for ref in (hg_ref, hu_ref, hq_ref):
                fence(ref)
            for t, _ in (act_tasks() if split else []) + gate_tasks(0):
                t()
            for c in range(nl):
                g_ref[c, bm:bm + HALO, :] = jnp.zeros((HALO, 128), F32)
            for t, _ in q_tasks() + u_tasks() + shift_tasks() + norm_tasks(lambda r: xf_ref[bm + r:bm + r + 16, :], bm):
                t()
            hg_ref[0:bm, :] = _dot(_unpack(xa_ref[0:bm // 2, :]), W(2))

        @pl.when(i == 0)
        def _():
            def prep(r0, nlast):
                for r in range(0, R, 16):
                    parts = [_ln(_unzip(xf_ref[pl.ds(a * kw + r0 + r, 16), :])) for a in range(na - 1 + (r < nlast))]
                    if r >= nlast:
                        parts.append(jnp.zeros((16, D), F32))
                    h0 = (r0 + r) // 2 if isinstance(r0, int) else pl.multiple_of((r0 + r) // 2, 8)
                    for j, z in enumerate(_ops(jnp.concatenate(parts, axis=0), LA, "b")):
                        kv_ref[j, pl.ds(h0, 8), :] = _zip(z)

            last = T - (na - 1) * kw
            nfull = last // R

            def body(j, carry):
                prep(pl.multiple_of(j * R, R), R)
                return carry
            lax.fori_loop(0, nfull, body, 0)
            for j in range(nfull, kw // R):
                prep(j * R, max(0, min(R, last - j * R)))

        pace = Pacer(zero, arity)

        def proj(src, w, dst, cols, skip=0):
            for n, c in enumerate(cols):
                lhs = _unpack(src[0:bm // 2, :]) if n < skip else pace.tie(src[0:bm // 2, :])
                y = pace.seen(_dot(lhs, _unpack(wp_ref[w, :, c * 128:(c + 1) * 128])))
                if len(dst.shape) == 3:
                    dst[c, 0:bm, :] = y
                else:
                    dst[0:bm, c * 128:(c + 1) * 128] = y
            return y

        gates = gate_tasks(((i + 1) % nq) * bm, pace.after)
        head = gate_tasks(((i + 1) % nq) * bm)[0]

        def conv_task(c, r):
            lanes = slice(c * 128, (c + 1) * 128)
            acc = None
            for s in range(8):
                taps = [k for k in range(K) if (HALO - pad + k) % 8 == s]
                lo = HALO - pad + taps[0] + r
                win = g_ref[c, lo:lo + rc + 8 * (len(taps) - 1), :]
                for n, k in enumerate(taps):
                    t = win[8 * n:8 * n + rc] * dwf_ref[k:k + 1, lanes]
                    acc = t if acc is None else acc + t
            y = _pack_rows(u_ref[r:r + rc, lanes] * acc)
            uc_ref[r // 2:(r + rc) // 2, lanes] = y
            return _vregs(y)
        convs = [(functools.partial(conv_task, c, r), 2 * rc) for r in range(0, bm, rc) for c in range(nl)]
        pace.spread([head] + convs, int(qk_frac * nprod * (kw // wq) * (bq // 16)))
        pace.credit += phase

        mx = None
        for c0 in range(0, kw, wq):
            def prod(j):
                return pace.seen(_dot_nt(pace.tie(q_ref[j]), _unpack(kv_ref[_a_as_b(j, LA), c0 // 2:(c0 + wq) // 2, :])))
            s = _combine(prod, LA, True)
            ts = []
            for a in range(na):
                for c in range(0, wq, 128):
                    t = s[:, a * wq + c:a * wq + c + 128]
                    col0 = a * kw + c0 + c
                    if col0 + 128 > T:
                        col = col0 + lax.broadcasted_iota(jnp.int32, t.shape, 1)
                        t = jnp.where(col < T, t, -jnp.inf)
                    s_ref[0:bm, col0:col0 + 128] = t
                    ts.append(t)
            for n in range(0, len(ts), 2):
                t = functools.reduce(jnp.maximum, ts[n:n + 2])
                mx = t if mx is None else jnp.maximum(mx, t)
        m_ref[0, 0:bm, :] = mx
        fence(s_ref, ts[-1])
        fence(m_ref, mx)

        rowmax, rowsum = {}, {}

        def max_task(r):
            rowmax[r] = jnp.broadcast_to(jnp.max(m_ref[0, r:r + rs, :], axis=-1, keepdims=True), (rs, 128))
            return _vregs(rowmax[r])

        def sum_task(r):
            part = [None] * chains
            mx = pace.after(rowmax[r]) if relsum else rowmax[r]
            for n, c in enumerate(range(0, Tp, 128)):
                e = jnp.exp2(s_ref[r:r + rs, c:c + 128] - mx)
                part[n % chains] = e if part[n % chains] is None else part[n % chains] + e
            rowsum[r] = functools.reduce(jnp.add, part)
            return _vregs(rowsum[r])

        def scale_task(r):
            rl = jnp.broadcast_to(1.0 / jnp.sum(pace.after(rowsum[r]) if relscale else rowsum[r], axis=-1, keepdims=True), (rs, 128))
            m_ref[0, r:r + rs, :] = rowmax[r]
            m_ref[1, r:r + rs, :] = rl
            if r + rs == bm:
                fence(s_ref, rl)
                fence(m_ref, rl)
            return _vregs(rl)

        def prob_task(p_ref, c0, r, c):
            rows = []
            for a in range(na):
                rr = slice(a * bq + r, a * bq + r + 16)
                mx, rl = (pace.after if rel else lambda v: v)(m_ref[0, rr, :]), m_ref[1, rr, :]
                rows.append(jnp.concatenate(
                    [jnp.exp2(s_ref[rr, b * kw + c:b * kw + c + 128] - mx) * rl for b in range(na)], axis=1))
            zs = [_zip(z) for z in _ops(jnp.concatenate(rows, axis=0), LA, "a")]
            for j, z in enumerate(zs):
                p_ref[j, r // 2:r // 2 + 8, c - c0:c - c0 + 128] = z
            return zs if ptok == 49 else [zs[j] for j in range(6, 49, 7)] if ptok == 7 else [zs[j] for j in (40, 41, 47, 48)]

        def prob_tasks(n):
            p_ref, c0, w = p_refs[n], sum(chunks[:n]), chunks[n]

            def last():
                out = prob_task(p_ref, c0, bq - 16, c0 + w - 128)
                fence(p_ref, out[-1])
                return out
            fns = [functools.partial(prob_task, p_ref, c0, r, c) for r in range(0, bq, 16) for c in range(c0, c0 + w, 128)]
            return [(f, pcost) for f in fns[:-1] + [last]]

        pace.spread([(functools.partial(f, r), c) for f, c in ((max_task, 3), (sum_task, scost), (scale_task, 6)) for r in range(0, bm, rs)] + prob_tasks(0),
                    (3 * nl - skip) * (bm // 16), lag[0], back[0], parts[0])
        fence(hq_ref, proj(xa_ref, 0, hq_ref, range(nl), skip))
        fence(hu_ref, proj(xa_ref, 1, hu_ref, range(nl)))
        fence(yc_ref, proj(uc_ref, 4, yc_ref, range(nl)))

        norms = norm_tasks(lambda r: xn_ref[r:r + 16, :], ((i + 2) % nq) * bm, pace.after)
        later = (act_tasks(pace.after) if split else []) + norms + _merge(gates[1:], q_tasks()) + shift_tasks() + ([] if tailu else u_tasks(pace.after))
        c0 = 0
        cut = 0
        for n, w in enumerate(chunks):
            if n + 1 < len(chunks):
                nxt = cut + int(gsplit[n] * len(later))
                pace.spread(_merge(prob_tasks(n + 1), later[cut:nxt]), int(pv_frac * nprod * (bq // 16)), lag[1], back[1], parts[1])
                cut = nxt
            else:
                pace.spread(later[cut:], nprod * (bq // 16), lag[2], back[2], parts[2])
            for j in _order(LA):
                t = pace.seen(_dot(pace.tie(p_refs[n][j]), _unpack(kv_ref[j, c0 // 2:(c0 + w) // 2, :])))
                t = t if c0 == 0 else acc_ref[j] + t
                acc_ref[j] = t
            fence(acc_ref, t)
            c0 += w

        def out_task(r):
            o = _combine(lambda j: acc_ref[j, r:r + 16, :], LA)
            toks = []
            for a in range(na):
                y = _zip(o[16 * a:16 * a + 16])
                ob_ref[(a * bq + r) // 2:(a * bq + r) // 2 + 8, :] = y
                toks += _vregs(y)
            if r + 16 == bq:
                fence(ob_ref, y)
            return toks
        pace.spread([(functools.partial(out_task, r), 1) for r in range(0, bq, 16)], (nl - 1) * (bm // 16))
        proj(xa_ref, 2, hg_ref, range(nl), 1)
        if tailu:
            pace.spread(u_tasks(pace.after), (nl - 1) * (bm // 16), lag[3], back[3], parts[3])
        for c in range(nl):
            lanes = slice(c * 128, (c + 1) * 128)
            lhs = ob_ref[0:bm // 2, :]
            out = _dot(pace.tie(lhs) if c else _unpack(lhs), _unpack(wp_ref[3, :, lanes]))
            for r in range(0, bm, 16):
                yc = jnp.concatenate([yc_ref[c, pl.ds(r + n, 8, stride=2), :] for n in range(2)], axis=0)
                o_ref[r:r + 16, lanes] = _unpack(_zip(_unzip(xr_ref[r:r + 16, lanes]) + (yc + out[r:r + 16])))

    @jax.jit
    def fn(x, w_q, w_k, w_v, w_ao, w_up, dw, w_dn, w_merge):
        B, T, D = x.shape
        Tp = pl.cdiv(T, 128 * na) * 128 * na
        nq = pl.cdiv(T, bm)
        ns = B * nq
        full = lambda a: pl.BlockSpec(a.shape, lambda s: (0,) * a.ndim)

        def nxt_map(s):
            n = jnp.minimum(s + 2, ns - 1)
            return (n // nq, n % nq, 0)
        return pl.pallas_call(
            functools.partial(kernel, nq=nq),
            grid=(ns,),
            in_specs=[pl.BlockSpec((None, T, D), lambda s: (s // nq, 0, 0)),
                      pl.BlockSpec((None, bm, D), nxt_map),
                      pl.BlockSpec((None, bm, D), lambda s: (s // nq, s % nq, 0))]
            + [full(a) for a in (w_q, w_k, w_v, w_ao, w_up, dw, w_dn, w_merge)],
            out_specs=pl.BlockSpec((None, bm, D), lambda s: (s // nq, s % nq, 0)),
            out_shape=jax.ShapeDtypeStruct(x.shape, x.dtype),
            scratch_shapes=[
                pltpu.VMEM((5, D // 2, D), U32),
                pltpu.VMEM((32, D), F32),
                pltpu.VMEM((nprod, Tp // na // 2, D // na), U32),
                pltpu.VMEM((bm // 2 + 8, D), U32),
                pltpu.VMEM((nprod + 1, bq // 2, D // na), U32),
                pltpu.VMEM((bm + 8, D), F32),
                pltpu.VMEM((bm // 2, D), U32),
                pltpu.VMEM((D // 128, bm + 2 * HALO, 128), F32),
                pltpu.VMEM((D // 128, bm + 8, 128), F32),
                pltpu.VMEM((bm + 8, Tp), F32),
                pltpu.VMEM((2, bm + 8, 128), F32),
                pltpu.VMEM((D // 128, bm + 8, 128), F32),
                pltpu.VMEM((bm + 8, D), F32),
                pltpu.VMEM((bm + 8, D), F32),
                pltpu.VMEM((bm + 8, D), F32),
                pltpu.VMEM((nprod + 1, bq, D // na), F32),
                pltpu.VMEM((bm // 2 + 8, D), U32),
                pltpu.VMEM((bm + 8, D), F32),
            ] + [pltpu.VMEM((nprod + 1, bq // 2, w), U32) for w in chunks],
            compiler_params=pltpu.CompilerParams(dimension_semantics=("arbitrary",), vmem_limit_bytes=120 * 2**20, flags=flags),
        )(x, x, x, w_q, w_k, w_v, w_ao, w_up, dw, w_dn, w_merge)
    return fn


_kernel = make(chunks=(384,640),pcost=100)


def pallas_standalone__conformer_family_branchformer__speech_kernel(x, w_q, w_k, w_v, w_ao, w_up, dw, w_dn, w_merge):
    return _kernel(x, w_q, w_k, w_v, w_ao, w_up, dw, w_dn, w_merge)
```

```python
import functools
import math
import jax
import jax.numpy as jnp
from jax import lax
from jax.experimental import pallas as pl
from jax.experimental.pallas import tpu as pltpu

F32 = jnp.float32
BF16 = jnp.bfloat16
U32 = jnp.uint32
EPS = 1e-5
LOG2E = 1.4426950408889634
HALO = 16


def _ln(x):
    m = jnp.mean(x, axis=-1, keepdims=True)
    c = x - m
    v = jnp.mean(c * c, axis=-1, keepdims=True)
    return c * lax.rsqrt(v + EPS)


def _gelu(x):
    c0 = math.sqrt(2.0 / math.pi)
    inner = x * (c0 + (c0 * 0.044715) * (x * x))
    hx = 0.5 * x
    return hx + hx * jnp.tanh(inner)


def _dot(a, b):
    return jnp.dot(a, b, preferred_element_type=F32)


def _dot_nt(a, b):
    return lax.dot_general(a, b, (((1,), (1,)), ((), ())), preferred_element_type=F32)


def _pack(x):
    return pltpu.bitcast(x.astype(BF16), U32)


def _unpack(x):
    return pltpu.bitcast(x, BF16)


def _split(x):
    r, c = x.shape
    return x[:r // 2, :c // 2], x[:r // 2, c // 2:], x[r // 2:, :c // 2], x[r // 2:, c // 2:]


def _join(c11, c12, c21, c22):
    return jnp.concatenate([jnp.concatenate([c11, c12], axis=1),
                            jnp.concatenate([c21, c22], axis=1)], axis=0)


def _ops(x, level, kind):
    if level == 0:
        return [x]
    x11, x12, x21, x22 = _split(x)
    if kind == "a":
        ops = [x11 + x22, x21 + x22, x11, x22, x11 + x12, x21 - x11, x12 - x22]
    elif kind == "b":
        ops = [x11 + x22, x11, x12 - x22, x21 - x11, x22, x11 + x12, x21 + x22]
    else:
        ops = [x11 + x22, x11, x21 - x22, x12 - x11, x22, x11 + x21, x12 + x22]
    return [z for o in ops for z in _ops(o, level - 1, kind)]


_A_AS_B = (0, 6, 1, 4, 5, 3, 2)


def _a_as_b(i, level):
    if level == 0:
        return 0
    n = 7 ** (level - 1)
    return _A_AS_B[i // n] * n + _a_as_b(i % n, level - 1)


ORDER = (0, 3, 4, 6, 2, 1, 5)


def _order(level, order=ORDER):
    if level == 0:
        return [0]
    n = 7 ** (level - 1)
    return [j * n + k for j in order for k in _order(level - 1, order)]


def _combine(get, level, transposed=False, base=0):
    if level == 0:
        return get(base)
    n = 7 ** (level - 1)
    sub = lambda j: _combine(get, level - 1, transposed, base + j * n)
    m0 = sub(0)
    m3 = sub(3)
    t = m0 + m3
    m4 = sub(4)
    t = t - m4
    m6 = sub(6)
    c11 = t + m6
    m2 = sub(2)
    c12 = m2 + m4
    t = m0 + m2
    m1 = sub(1)
    c21 = m1 + m3
    t = t - m1
    m5 = sub(5)
    c22 = t + m5
    if transposed:
        c12, c21 = c21, c12
    return _join(c11, c12, c21, c22)


def _vregs(x):
    return [x[r:r + 8, c:c + 128] for r in range(0, x.shape[0], 8) for c in range(0, x.shape[1], 128)]


def _pack_rows(x):
    return pltpu.bitcast(x.astype(BF16), U32)


def _zip(x):
    return pltpu.pack_elementwise([x[0:8], x[8:16]], packed_dtype=BF16)


def _unzip(x, gate=lambda w: w):
    w = gate(pltpu.bitcast(x, U32))
    return jnp.concatenate([pltpu.unpack_elementwise(w, index=n, packed_dtype=BF16, unpacked_dtype=F32)
                            for n in range(2)], axis=0)


def _tree(xs, arity):
    part = [functools.reduce(lambda a, b: a | b, xs[n::arity]) for n in range(min(arity, len(xs)))]
    while len(part) > 1:
        part = [functools.reduce(lambda a, b: a | b, part[n:n + 2]) for n in range(0, len(part), 2)]
    return part[0]


class Pacer:
    def __init__(self, zero, arity):
        self.arity = arity
        self.keep = lax.broadcasted_iota(jnp.int32, (8, 128), 0) >= zero
        self.tasks, self.due = [], []
        self.recent = []
        self.back = 0

    def spread(self, tasks, nslots, lag=0, back=0, parts=1):
        assert not self.tasks and not self.due
        self.tasks = list(tasks)
        self.rate = sum(c for _, c in tasks) / (nslots - lag)
        self.end = nslots - 1
        self.credit = tasks[0][1]
        self.slot, self.lag, self.back, self.parts = 0, lag, back, parts

    def seen(self, y):
        self.recent.append(y[0:8, 0:128])
        return y

    def after(self, x):
        tok = pltpu.bitcast(self.recent[max(0, len(self.recent) - 1 - self.back)], x.dtype)
        return jnp.concatenate([jnp.concatenate(
            [jnp.where(self.keep, x[r:r + 8, c:c + 128], tok) for c in range(0, x.shape[1], 128)], axis=1)
            for r in range(0, x.shape[0], 8)], axis=0)

    def tie(self, lhs):
        rows = []
        for r in range(0, lhs.shape[0], 8):
            t = lhs[r:r + 8]
            while self.tasks and self.credit >= self.tasks[0][1] * (1 - 1e-6):
                fn, cost = self.tasks.pop(0)
                self.credit -= cost
                out = [pltpu.bitcast(v, U32) for v in fn()]
                n = min(len(out), self.parts)
                for m in range(n):
                    part = out[m * len(out) // n:(m + 1) * len(out) // n]
                    when = min(self.end, self.slot + self.lag + m * cost / self.rate / n)
                    self.due.append((when, _tree(part, self.arity)))
                self.due.sort(key=lambda d: d[0])
            mine = None
            while self.due and self.due[0][0] <= self.slot:
                tok = self.due.pop(0)[1]
                mine = tok if mine is None else mine | tok
            self.slot += 1
            self.credit += self.rate
            if mine is not None:
                t0 = jnp.where(self.keep, t[:, 0:128], mine)
                t = t0 if t.shape[1] == 128 else jnp.concatenate([t0, t[:, 128:]], axis=1)
            rows.append(t)
        return _unpack(jnp.concatenate(rows, axis=0))


def _merge(xs, ys):
    if not ys:
        return xs
    keyed = [((n + 0.5) / len(xs), 0, n) for n in range(len(xs))] + [((n + 0.5) / len(ys), 1, n) for n in range(len(ys))]
    return [(xs, ys)[w][n] for _, w, n in sorted(keyed)]


def make(bm=448, LA=2, wq=256, chunks=(512, 512), R=64, rc=16, rs=16, nmid=2, flags=None, qk_frac=1.0,
         pv_frac=1.0, skip=1, pcost=100, scost=70, ptok=7, gsplit=(0.0, 0.0, 0.0), tailu=True, chains=1, phase=0.0, split=False, lag=(10, 30, 10, 6, 14), back=(1, 6, 2, 0), arity=3, parts=(7, 7, 4, 2, 4), rel=True, relscale=True, relsum=False, cparts=8, qkmax=False, ahead=3, relmax=False, mcost=10, kcost=6):
    na = 2 ** LA
    nprod = 7 ** LA
    bq = bm // na
    rg = 16

    def kernel(x_hbm, wq_hbm, wk_hbm, wv_hbm, wao_hbm, wup_hbm, dw_hbm, wdn_hbm, wm_hbm, o_ref,
               x_ref, wq_ref, wk_ref, wv_ref, wao_ref, wup_ref, dw_ref, wdn_ref, wm_ref, sems,
               wp_ref, dwf_ref, kv_ref, xa_ref, q_ref, u_ref, uc_ref, g_ref, gn_ref, s_ref,
               m_ref, yc_ref, hg_ref, hq_ref, hu_ref, acc_ref, ob_ref, ga_ref, *p_refs):
        step = pl.program_id(0)
        B, T, D = x_hbm.shape
        nq = pl.cdiv(T, bm)
        i = step % nq
        base = (step // nq) * (nq * bm)
        Tp = s_ref.shape[1]
        K = dw_ref.shape[0]
        pad = K // 2
        nl = D // 128
        kw = Tp // na
        W = lambda w: _unpack(wp_ref[w])
        zero = pl.multiple_of(jnp.minimum(step, 0) * 8, 8)
        row16 = lax.broadcasted_iota(jnp.int32, (16, 1), 0)
        unzipped16 = 2 * (row16 % 8) + row16 // 8

        def fence(ref, val=None):
            idx = tuple(n - 1 for n in ref.shape[:-2]) + (pl.ds(zero + ref.shape[-2] - 8, 8), pl.ds(0, 128))
            ref[idx] = jnp.zeros((8, 128), ref.dtype) if val is None else pltpu.bitcast(val[-8:, -128:], ref.dtype)

        def norm_tasks(load, r0, gate=lambda w: w):
            def task(r):
                y = _zip(_ln(jnp.where(r0 + r + unzipped16 < T, _unzip(load(r), gate), 0.0)))
                xa_ref[r // 2:r // 2 + 8, :] = y
                if r + 16 == bm:
                    fence(xa_ref, y)
                return _vregs(y)
            return [(functools.partial(task, r), 40) for r in range(0, bm, 16)]

        def act_tasks(gate=lambda w: w):
            def task(r):
                y = _gelu(gate(hg_ref[r:r + 16, :]))
                ga_ref[r:r + 16, :] = y
                if r + 16 == bm:
                    fence(ga_ref, y)
                return _vregs(y)
            return [(functools.partial(task, r), 24) for r in range(HALO, bm, 16)]

        def gate_tasks(r0, gate=lambda w: w):
            def task(r):
                y = _gelu(gate(hg_ref[r:r + 16, :])) if r < HALO or not split else gate(ga_ref[r:r + 16, :])
                g = jnp.where(r0 + r + row16 < T, _ln(y), 0.0)
                for c in range(nl):
                    gn_ref[c, r:r + 16, :] = g[:, c * 128:(c + 1) * 128]
                    if r < HALO:
                        g_ref[c, HALO + bm + r:HALO + bm + r + 16, :] = g[:, c * 128:(c + 1) * 128]
                if r + 16 == bm:
                    fence(gn_ref, g)
                return _vregs(g)
            return [(functools.partial(task, r), 30) for r in range(0, bm, 16)]

        def u_tasks(gate=lambda w: w):
            def task(r):
                y = _gelu(gate(hu_ref[r:r + 16, :]))
                u_ref[r:r + 16, :] = y
                return _vregs(y)
            return [(functools.partial(task, r), 24) for r in range(0, bm, 16)]

        def q_tasks():
            def task(r):
                x = jnp.concatenate([hq_ref[a * bq + r:a * bq + r + 16, :] for a in range(na)], axis=0)
                zs = [_zip(z) for z in _ops(x, LA, "bt")]
                for j, z in enumerate(zs):
                    q_ref[j, r // 2:r // 2 + 8, :] = z
                return [v for z in zs for v in _vregs(z)]
            return [(functools.partial(task, r), 55) for r in range(0, bq, 16)]

        def shift_tasks():
            def head():
                out = []
                for c in range(nl):
                    y = g_ref[c, bm:bm + HALO, :]
                    g_ref[c, 0:HALO, :] = y
                    out += _vregs(y)
                return out

            def task(r):
                out = []
                for c in range(nl):
                    y = gn_ref[c, r:r + 32, :]
                    g_ref[c, HALO + r:HALO + r + 32, :] = y
                    out += _vregs(y)
                return out
            return [(head, 8)] + [(functools.partial(task, r), 16) for r in range(0, bm, 32)]

        def fetch_x(b, r0, n, sem):
            return pltpu.make_async_copy(x_hbm.at[b, pl.ds(r0, n)], x_ref.at[pl.ds(b * nq * bm + r0, n)], sems.at[sem])

        pairs = ((wq_hbm, wq_ref), (wk_hbm, wk_ref), (wup_hbm, wup_ref), (dw_hbm, dw_ref), (wv_hbm, wv_ref),
                 (wao_hbm, wao_ref), (wdn_hbm, wdn_ref), (wm_hbm, wm_ref))
        fetch_w = [pltpu.make_async_copy(src, dst, sems.at[n]) for n, (src, dst) in enumerate(pairs)]
        head_x = fetch_x(0, 0, 2 * bm, len(pairs))
        rest_x = [fetch_x(0, 2 * bm, T - 2 * bm, len(pairs) + 1)] + [fetch_x(b, 0, T, len(pairs) + 1 + b) for b in range(1, B)]

        @pl.when(step == 0)
        def _():
            for c in fetch_w[0:2] + [head_x] + fetch_w[2:4] + [rest_x[0]] + fetch_w[4:] + rest_x[1:]:
                c.start()
            for b in range(B):
                x_ref[b * nq * bm + T:(b + 1) * nq * bm, :] = jnp.zeros((nq * bm - T, D), BF16)
            fetch_w[0].wait()
            fetch_w[1].wait()
            wp_ref[0] = _pack_rows(_dot_nt(wq_ref[...], wk_ref[...]) * (LOG2E * float(D) ** -0.5))
            head_x.wait()
            for t, _ in norm_tasks(lambda r: x_ref[r:r + 16, :], 0):
                t()
            fetch_w[2].wait()
            fetch_w[3].wait()
            wp_ref[1] = pltpu.bitcast(wup_ref[:, 0:D], U32)
            wp_ref[2] = pltpu.bitcast(wup_ref[:, D:2 * D], U32)
            dwf_ref[0:K, :] = dw_ref[...].astype(F32)
            xa = _unpack(xa_ref[0:bm // 2, :])
            hg_ref[0:bm, :] = _dot(xa, W(2))
            hu_ref[0:bm, :] = _dot(xa, W(1))
            hq_ref[0:bm, :] = _dot(xa, W(0))
            for ref in (hg_ref, hu_ref, hq_ref):
                fence(ref)
            for t, _ in (act_tasks() if split else []) + gate_tasks(0):
                t()
            for c in range(nl):
                g_ref[c, bm:bm + HALO, :] = jnp.zeros((HALO, 128), F32)
            for t, _ in q_tasks() + u_tasks() + shift_tasks() + norm_tasks(lambda r: x_ref[bm + r:bm + r + 16, :], bm):
                t()
            for c in fetch_w[4:]:
                c.wait()
            t = _dot(wv_ref[...], wao_ref[...]).astype(BF16)
            wp_ref[3] = _pack_rows(_dot(t, wm_ref[0:D, :]))
            wp_ref[4] = _pack_rows(_dot(wdn_ref[...], wm_ref[D:2 * D, :]))
            rest_x[0].wait()

        for b in range(1, B):
            @pl.when(step == b * nq - 2)
            def _():
                rest_x[b].wait()

        @pl.when(i == 0)
        def _():
            def prep(r0, nlast):
                for r in range(0, R, 16):
                    parts = [_ln(_unzip(x_ref[pl.ds(pl.multiple_of(base + a * kw + r0 + r, 16), 16), :])) for a in range(na - 1 + (r < nlast))]
                    if r >= nlast:
                        parts.append(jnp.zeros((16, D), F32))
                    h0 = (r0 + r) // 2 if isinstance(r0, int) else pl.multiple_of((r0 + r) // 2, 8)
                    for j, z in enumerate(_ops(jnp.concatenate(parts, axis=0), LA, "b")):
                        kv_ref[j, pl.ds(h0, 8), :] = _zip(z)

            last = T - (na - 1) * kw
            nfull = last // R

            def body(j, carry):
                prep(pl.multiple_of(j * R, R), R)
                return carry
            lax.fori_loop(0, nfull, body, 0)
            for j in range(nfull, kw // R):
                prep(j * R, max(0, min(R, last - j * R)))

        pace = Pacer(zero, arity)

        def proj(src, w, dst, cols, skip=0):
            for n, c in enumerate(cols):
                lhs = _unpack(src[0:bm // 2, :]) if n < skip else pace.tie(src[0:bm // 2, :])
                y = pace.seen(_dot(lhs, _unpack(wp_ref[w, :, c * 128:(c + 1) * 128])))
                if len(dst.shape) == 3:
                    dst[c, 0:bm, :] = y
                else:
                    dst[0:bm, c * 128:(c + 1) * 128] = y
            return y

        gates = gate_tasks(((i + 1) % nq) * bm, pace.after)

        def conv_task(c, r):
            lanes = slice(c * 128, (c + 1) * 128)
            acc = None
            steps = []
            for s in range(8):
                if s and s % (8 // cparts) == 0:
                    steps.append(acc[0:8])
                taps = [k for k in range(K) if (HALO - pad + k) % 8 == s]
                lo = HALO - pad + taps[0] + r
                win = g_ref[c, lo:lo + rc + 8 * (len(taps) - 1), :]
                for n, k in enumerate(taps):
                    t = win[8 * n:8 * n + rc] * dwf_ref[k:k + 1, lanes]
                    acc = t if acc is None else acc + t
            y = _pack_rows(u_ref[r:r + rc, lanes] * acc)
            uc_ref[r // 2:(r + rc) // 2, lanes] = y
            return steps + _vregs(y)
        convs = [(functools.partial(conv_task, c, r), 2 * rc) for r in range(0, bm, rc) for c in range(nl)]
        nlate = nl * pl.cdiv(pad, rc)
        pace.spread(convs[:-nlate], int(qk_frac * nprod * (kw // wq) * (bq // 16)), parts=cparts)
        pace.credit += phase

        mx = None
        for c0 in range(0, kw, wq):
            def prod(j):
                return pace.seen(_dot_nt(pace.tie(q_ref[j]), _unpack(kv_ref[_a_as_b(j, LA), c0 // 2:(c0 + wq) // 2, :])))
            s = _combine(prod, LA, True)
            ts = []
            for a in range(na):
                for c in range(0, wq, 128):
                    t = s[:, a * wq + c:a * wq + c + 128]
                    col0 = a * kw + c0 + c
                    if col0 + 128 > T:
                        col = col0 + lax.broadcasted_iota(jnp.int32, t.shape, 1)
                        t = jnp.where(col < T, t, -jnp.inf)
                    s_ref[0:bm, col0:col0 + 128] = t
                    ts.append(t)
            for n in range(0, len(ts) if qkmax else 0, 2):
                t = functools.reduce(jnp.maximum, ts[n:n + 2])
                mx = t if mx is None else jnp.maximum(mx, t)
        fence(s_ref, ts[-1])
        if qkmax:
            m_ref[0, 0:bm, :] = mx
            fence(m_ref, mx)

        rowmax, rowsum = {}, {}

        def max_task(r):
            if qkmax:
                mx = m_ref[0, r:r + rs, :]
            else:
                part = [s_ref[pl.ds(zero + r, rs), c:c + 128] for c in range(0, Tp, 128)]
                part = [pace.after(t) if n < 2 and relmax else t for n, t in enumerate(part)]
                part = [functools.reduce(jnp.maximum, part[n::2]) for n in range(2)]
                mx = jnp.maximum(*part)
            rowmax[r] = jnp.broadcast_to(jnp.max(mx, axis=-1, keepdims=True), (rs, 128))
            return _vregs(rowmax[r])

        def sum_task(r):
            part = [None] * chains
            mx = pace.after(rowmax[r]) if relsum else rowmax[r]
            for n, c in enumerate(range(0, Tp, 128)):
                e = jnp.exp2(s_ref[r:r + rs, c:c + 128] - mx)
                part[n % chains] = e if part[n % chains] is None else part[n % chains] + e
            rowsum[r] = functools.reduce(jnp.add, part)
            return _vregs(rowsum[r])

        def scale_task(r):
            rl = jnp.broadcast_to(1.0 / jnp.sum(pace.after(rowsum[r]) if relscale else rowsum[r], axis=-1, keepdims=True), (rs, 128))
            m_ref[0, r:r + rs, :] = rowmax[r]
            m_ref[1, r:r + rs, :] = rl
            if r + rs == bm:
                fence(s_ref, rl)
                fence(m_ref, rl)
            return _vregs(rl)

        def prob_task(p_ref, c0, r, c):
            rows = []
            for a in range(na):
                rr = slice(a * bq + r, a * bq + r + 16)
                mx, rl = (pace.after if rel else lambda v: v)(m_ref[0, rr, :]), m_ref[1, rr, :]
                rows.append(jnp.concatenate(
                    [jnp.exp2(s_ref[rr, b * kw + c:b * kw + c + 128] - mx) * rl for b in range(na)], axis=1))
            zs = [_zip(z) for z in _ops(jnp.concatenate(rows, axis=0), LA, "a")]
            for j, z in enumerate(zs):
                p_ref[j, r // 2:r // 2 + 8, c - c0:c - c0 + 128] = z
            return zs if ptok == 49 else [zs[j] for j in range(6, 49, 7)] if ptok == 7 else [zs[j] for j in (40, 41, 47, 48)]

        def prob_tasks(n):
            p_ref, c0, w = p_refs[n], sum(chunks[:n]), chunks[n]

            def last():
                out = prob_task(p_ref, c0, bq - 16, c0 + w - 128)
                fence(p_ref, out[-1])
                return out
            fns = [functools.partial(prob_task, p_ref, c0, r, c) for r in range(0, bq, 16) for c in range(c0, c0 + w, 128)]
            return [(f, pcost) for f in fns[:-1] + [last]]

        rows = list(range(0, bm, rs))
        maxes = [(functools.partial(max_task, r), mcost) for r in rows]
        sums = [(functools.partial(sum_task, r), scost) for r in rows]
        stats = maxes[:ahead]
        for n, t in enumerate(sums):
            stats += [t] + maxes[ahead + n:ahead + n + 1]
        stats += [(functools.partial(scale_task, r), kcost) for r in rows]
        pace.spread(stats + gates[:1] + convs[-nlate:] + prob_tasks(0),
                    (3 * nl + nmid - skip) * (bm // 16), lag[0], back[0], parts[0])
        fence(hg_ref, proj(xa_ref, 2, hg_ref, range(nl), skip))
        proj(xa_ref, 0, hq_ref, range(nl))
        fence(hq_ref, pace.recent[-1])
        proj(xa_ref, 1, hu_ref, range(nl))
        fence(hu_ref, pace.recent[-1])
        assert len(pace.tasks) <= len(prob_tasks(0))
        fence(uc_ref, pace.recent[-1])
        if nmid:
            proj(uc_ref, 4, yc_ref, range(nmid))

        ahead2 = jnp.minimum(step + 2, B * nq - 1) * bm
        norms = norm_tasks(lambda r: x_ref[pl.ds(pl.multiple_of(ahead2 + r, 16), 16), :], ((i + 2) % nq) * bm, pace.after)
        later = (act_tasks(pace.after) if split else []) + norms + _merge(gates[1:], q_tasks()) + shift_tasks() + ([] if tailu else u_tasks(pace.after))
        c0 = 0
        cut = 0
        for n, w in enumerate(chunks):
            if n + 1 < len(chunks):
                nxt = cut + int(gsplit[n] * len(later))
                pace.spread(_merge(prob_tasks(n + 1), later[cut:nxt]), int(pv_frac * nprod * (bq // 16)), lag[1], back[1], parts[1])
                cut = nxt
            else:
                pace.spread(later[cut:], nprod * (bq // 16), lag[2], back[2], parts[2])
            for j in _order(LA):
                t = pace.seen(_dot(pace.tie(p_refs[n][j]), _unpack(kv_ref[j, c0 // 2:(c0 + w) // 2, :])))
                t = t if c0 == 0 else acc_ref[j] + t
                acc_ref[j] = t
            fence(acc_ref, t)
            c0 += w

        def out_task(r):
            o = _combine(lambda j: acc_ref[j, r:r + 16, :], LA)
            toks = []
            for a in range(na):
                y = _zip(o[16 * a:16 * a + 16])
                ob_ref[(a * bq + r) // 2:(a * bq + r) // 2 + 8, :] = y
                toks += _vregs(y)
            if r + 16 == bq:
                fence(ob_ref, y)
            return toks
        pace.spread([(functools.partial(out_task, r), 1) for r in range(0, bq, 16)],
                    (nl - nmid) * (bm // 16), lag[4], 0, parts[4])
        fence(yc_ref, proj(uc_ref, 4, yc_ref, range(nmid, nl)))
        if tailu:
            pace.spread(u_tasks(pace.after), (nl - 1) * (bm // 16), lag[3], back[3], parts[3])
        for c in range(nl):
            lanes = slice(c * 128, (c + 1) * 128)
            lhs = ob_ref[0:bm // 2, :]
            out = _dot(pace.tie(lhs) if c else _unpack(lhs), _unpack(wp_ref[3, :, lanes]))
            for r in range(0, bm, 16):
                yc = jnp.concatenate([yc_ref[c, pl.ds(r + n, 8, stride=2), :] for n in range(2)], axis=0)
                o_ref[r:r + 16, lanes] = _unpack(_zip(_unzip(x_ref[pl.ds(pl.multiple_of(step * bm + r, 16), 16), lanes]) + (yc + out[r:r + 16])))

    @jax.jit
    def fn(x, w_q, w_k, w_v, w_ao, w_up, dw, w_dn, w_merge):
        B, T, D = x.shape
        Tp = pl.cdiv(T, 128 * na) * 128 * na
        nq = pl.cdiv(T, bm)
        ns = B * nq
        ws = (w_q, w_k, w_v, w_ao, w_up, dw, w_dn, w_merge)
        return pl.pallas_call(
            kernel,
            grid=(ns,),
            in_specs=[pl.BlockSpec(memory_space=pl.ANY)] * 9,
            out_specs=pl.BlockSpec((None, bm, D), lambda s: (s // nq, s % nq, 0)),
            out_shape=jax.ShapeDtypeStruct(x.shape, x.dtype),
            scratch_shapes=[pltpu.VMEM((ns * bm, D), x.dtype)] + [pltpu.VMEM(w.shape, w.dtype) for w in ws] + [
                pltpu.SemaphoreType.DMA((len(ws) + 1 + B,)),
                pltpu.VMEM((5, D // 2, D), U32),
                pltpu.VMEM((32, D), F32),
                pltpu.VMEM((nprod, Tp // na // 2, D // na), U32),
                pltpu.VMEM((bm // 2 + 8, D), U32),
                pltpu.VMEM((nprod + 1, bq // 2, D // na), U32),
                pltpu.VMEM((bm + 8, D), F32),
                pltpu.VMEM((bm // 2 + 8, D), U32),
                pltpu.VMEM((D // 128, bm + 2 * HALO, 128), F32),
                pltpu.VMEM((D // 128, bm + 8, 128), F32),
                pltpu.VMEM((bm + 8, Tp), F32),
                pltpu.VMEM((2, bm + 8, 128), F32),
                pltpu.VMEM((D // 128, bm + 8, 128), F32),
                pltpu.VMEM((bm + 8, D), F32),
                pltpu.VMEM((bm + 8, D), F32),
                pltpu.VMEM((bm + 8, D), F32),
                pltpu.VMEM((nprod + 1, bq, D // na), F32),
                pltpu.VMEM((bm // 2 + 8, D), U32),
                pltpu.VMEM((bm + 8, D), F32),
            ] + [pltpu.VMEM((nprod + 1, bq // 2, w), U32) for w in chunks],
            compiler_params=pltpu.CompilerParams(dimension_semantics=("arbitrary",), vmem_limit_bytes=120 * 2**20, flags=flags),
        )(x, w_q, w_k, w_v, w_ao, w_up, dw, w_dn, w_merge)
    return fn


_kernel = make()


def pallas_standalone__conformer_family_branchformer__speech_kernel(x, w_q, w_k, w_v, w_ao, w_up, dw, w_dn, w_merge):
    return _kernel(x, w_q, w_k, w_v, w_ao, w_up, dw, w_dn, w_merge)
```

```python
import functools
import math
import jax
import jax.numpy as jnp
from jax import lax
from jax.experimental import pallas as pl
from jax.experimental.pallas import tpu as pltpu

F32 = jnp.float32
BF16 = jnp.bfloat16
U32 = jnp.uint32
EPS = 1e-5
LOG2E = 1.4426950408889634
HALO = 16


def _ln(x):
    m = jnp.mean(x, axis=-1, keepdims=True)
    c = x - m
    v = jnp.mean(c * c, axis=-1, keepdims=True)
    return c * lax.rsqrt(v + EPS)


def _gelu(x):
    c0 = math.sqrt(2.0 / math.pi)
    inner = x * (c0 + (c0 * 0.044715) * (x * x))
    hx = 0.5 * x
    return hx + hx * jnp.tanh(inner)


def _dot(a, b):
    return jnp.dot(a, b, preferred_element_type=F32)


def _dot_nt(a, b):
    return lax.dot_general(a, b, (((1,), (1,)), ((), ())), preferred_element_type=F32)


def _pack(x):
    return pltpu.bitcast(x.astype(BF16), U32)


def _unpack(x):
    return pltpu.bitcast(x, BF16)


def _split(x):
    r, c = x.shape
    return x[:r // 2, :c // 2], x[:r // 2, c // 2:], x[r // 2:, :c // 2], x[r // 2:, c // 2:]


def _join(c11, c12, c21, c22):
    return jnp.concatenate([jnp.concatenate([c11, c12], axis=1),
                            jnp.concatenate([c21, c22], axis=1)], axis=0)


def _ops(x, level, kind):
    if level == 0:
        return [x]
    x11, x12, x21, x22 = _split(x)
    if kind == "a":
        ops = [x11 + x22, x21 + x22, x11, x22, x11 + x12, x21 - x11, x12 - x22]
    elif kind == "b":
        ops = [x11 + x22, x11, x12 - x22, x21 - x11, x22, x11 + x12, x21 + x22]
    else:
        ops = [x11 + x22, x11, x21 - x22, x12 - x11, x22, x11 + x21, x12 + x22]
    return [z for o in ops for z in _ops(o, level - 1, kind)]


_A_AS_B = (0, 6, 1, 4, 5, 3, 2)


def _a_as_b(i, level):
    if level == 0:
        return 0
    n = 7 ** (level - 1)
    return _A_AS_B[i // n] * n + _a_as_b(i % n, level - 1)


ORDER = (0, 3, 4, 6, 2, 1, 5)


def _order(level, order=ORDER):
    if level == 0:
        return [0]
    n = 7 ** (level - 1)
    return [j * n + k for j in order for k in _order(level - 1, order)]


def _combine(get, level, transposed=False, base=0):
    if level == 0:
        return get(base)
    n = 7 ** (level - 1)
    sub = lambda j: _combine(get, level - 1, transposed, base + j * n)
    m0 = sub(0)
    m3 = sub(3)
    t = m0 + m3
    m4 = sub(4)
    t = t - m4
    m6 = sub(6)
    c11 = t + m6
    m2 = sub(2)
    c12 = m2 + m4
    t = m0 + m2
    m1 = sub(1)
    c21 = m1 + m3
    t = t - m1
    m5 = sub(5)
    c22 = t + m5
    if transposed:
        c12, c21 = c21, c12
    return _join(c11, c12, c21, c22)


def _vregs(x):
    return [x[r:r + 8, c:c + 128] for r in range(0, x.shape[0], 8) for c in range(0, x.shape[1], 128)]


def _pack_rows(x):
    return pltpu.bitcast(x.astype(BF16), U32)


def _zip(x):
    return pltpu.pack_elementwise([x[0:8], x[8:16]], packed_dtype=BF16)


def _unzip(x, gate=lambda w: w):
    w = gate(pltpu.bitcast(x, U32))
    return jnp.concatenate([pltpu.unpack_elementwise(w, index=n, packed_dtype=BF16, unpacked_dtype=F32)
                            for n in range(2)], axis=0)


def _tree(xs, arity):
    part = [functools.reduce(lambda a, b: a | b, xs[n::arity]) for n in range(min(arity, len(xs)))]
    while len(part) > 1:
        part = [functools.reduce(lambda a, b: a | b, part[n:n + 2]) for n in range(0, len(part), 2)]
    return part[0]


class Pacer:
    def __init__(self, zero, arity):
        self.arity = arity
        self.keep = lax.broadcasted_iota(jnp.int32, (8, 128), 0) >= zero
        self.tasks, self.due = [], []
        self.recent = []
        self.back = 0
        self.rate = self.credit = self.slot = 0

    def spread(self, tasks, nslots, lag=0, back=0, parts=1):
        assert not self.tasks and not self.due
        self.tasks = list(tasks)
        self.rate = sum(c for _, c in tasks) / (nslots - lag)
        self.end = nslots - 1
        self.credit = tasks[0][1]
        self.slot, self.lag, self.back, self.parts = 0, lag, back, parts

    def seen(self, y):
        self.recent.append(y[0:8, 0:128])
        return y

    def after(self, x):
        tok = pltpu.bitcast(self.recent[max(0, len(self.recent) - 1 - self.back)], x.dtype)
        return jnp.concatenate([jnp.concatenate(
            [jnp.where(self.keep, x[r:r + 8, c:c + 128], tok) for c in range(0, x.shape[1], 128)], axis=1)
            for r in range(0, x.shape[0], 8)], axis=0)

    def tie(self, lhs):
        rows = []
        for r in range(0, lhs.shape[0], 8):
            t = lhs[r:r + 8]
            while self.tasks and self.credit >= self.tasks[0][1] * (1 - 1e-6):
                fn, cost = self.tasks.pop(0)
                self.credit -= cost
                out = [pltpu.bitcast(v, U32) for v in fn()]
                n = min(len(out), self.parts)
                for m in range(n):
                    part = out[m * len(out) // n:(m + 1) * len(out) // n]
                    when = min(self.end, self.slot + self.lag + m * cost / self.rate / n)
                    self.due.append((when, _tree(part, self.arity)))
                self.due.sort(key=lambda d: d[0])
            mine = None
            while self.due and self.due[0][0] <= self.slot:
                tok = self.due.pop(0)[1]
                mine = tok if mine is None else mine | tok
            self.slot += 1
            self.credit += self.rate
            if mine is not None:
                t0 = jnp.where(self.keep, t[:, 0:128], mine)
                t = t0 if t.shape[1] == 128 else jnp.concatenate([t0, t[:, 128:]], axis=1)
            rows.append(t)
        return _unpack(jnp.concatenate(rows, axis=0))


def _merge(xs, ys):
    if not ys:
        return xs
    keyed = [((n + 0.5) / len(xs), 0, n) for n in range(len(xs))] + [((n + 0.5) / len(ys), 1, n) for n in range(len(ys))]
    return [(xs, ys)[w][n] for _, w, n in sorted(keyed)]


def make(bm=448, LA=2, wq=256, chunks=(512, 512), R=64, rpre=8, kcost2=160, ktok=True, kparts=7, kfine=True, rc=16, rs=16, nmid=2, flags=None, qk_frac=1.0,
         pv_frac=1.0, skip=1, pcost=100, scost=70, ptok=7, gsplit=(0.0, 0.0, 0.0), tailu=True, chains=1, phase=0.0, split=False, lag=(10, 30, 10, 6, 14), back=(1, 6, 2, 0), arity=3, parts=(7, 7, 4, 2, 4), rel=True, relscale=True, relsum=False, cparts=8, qkmax=False, ahead=3, relmax=False, mcost=10, kcost=6):
    na = 2 ** LA
    nprod = 7 ** LA
    bq = bm // na
    rg = 16

    def kernel(x_hbm, wq_hbm, wk_hbm, wv_hbm, wao_hbm, wup_hbm, dw_hbm, wdn_hbm, wm_hbm, o_ref,
               x_ref, wq_ref, wk_ref, wv_ref, wao_ref, wup_ref, dw_ref, wdn_ref, wm_ref, sems,
               wp_ref, dwf_ref, kv_ref, xa_ref, q_ref, u_ref, uc_ref, g_ref, gn_ref, s_ref,
               m_ref, yc_ref, hg_ref, hq_ref, hu_ref, acc_ref, ob_ref, ga_ref, *p_refs):
        step = pl.program_id(0)
        B, T, D = x_hbm.shape
        nq = pl.cdiv(T, bm)
        i = step % nq
        Tp = s_ref.shape[1]
        K = dw_ref.shape[0]
        pad = K // 2
        nl = D // 128
        kw = Tp // na
        block_row = lambda n: (n // nq) * Tp + (n % nq) * bm
        W = lambda w: _unpack(wp_ref[w])
        zero = pl.multiple_of(jnp.minimum(step, 0) * 8, 8)

        def fence(ref, val=None):
            idx = tuple(n - 1 for n in ref.shape[:-2]) + (pl.ds(zero + ref.shape[-2] - 8, 8), pl.ds(0, 128))
            ref[idx] = jnp.zeros((8, 128), ref.dtype) if val is None else pltpu.bitcast(val[-8:, -128:], ref.dtype)

        def x_rows(r, lanes=slice(None)):
            return x_ref[pl.ds(r if isinstance(r, int) else pl.multiple_of(r, 16), 16), lanes]

        def norm_tasks(r0, gate=lambda w: w):
            def task(r):
                y = _zip(_ln(_unzip(x_rows(r0 + r), gate)))
                xa_ref[r // 2:r // 2 + 8, :] = y
                if r + 16 == bm:
                    fence(xa_ref, y)
                return _vregs(y)
            return [(functools.partial(task, r), 40) for r in range(0, bm, 16)]

        def act_tasks(gate=lambda w: w):
            def task(r):
                y = _gelu(gate(hg_ref[r:r + 16, :]))
                ga_ref[r:r + 16, :] = y
                if r + 16 == bm:
                    fence(ga_ref, y)
                return _vregs(y)
            return [(functools.partial(task, r), 24) for r in range(HALO, bm, 16)]

        def gate_tasks(gate=lambda w: w):
            def task(r):
                y = _gelu(gate(hg_ref[r:r + 16, :])) if r < HALO or not split else gate(ga_ref[r:r + 16, :])
                g = _ln(y)
                for c in range(nl):
                    gn_ref[c, r:r + 16, :] = g[:, c * 128:(c + 1) * 128]
                    if r < HALO:
                        g_ref[c, HALO + bm + r:HALO + bm + r + 16, :] = g[:, c * 128:(c + 1) * 128]
                if r + 16 == bm:
                    fence(gn_ref, g)
                return _vregs(g)
            return [(functools.partial(task, r), 30) for r in range(0, bm, 16)]

        def u_tasks(gate=lambda w: w):
            def task(r):
                y = _gelu(gate(hu_ref[r:r + 16, :]))
                u_ref[r:r + 16, :] = y
                return _vregs(y)
            return [(functools.partial(task, r), 24) for r in range(0, bm, 16)]

        def q_tasks():
            def task(r):
                x = jnp.concatenate([hq_ref[a * bq + r:a * bq + r + 16, :] for a in range(na)], axis=0)
                zs = [_zip(z) for z in _ops(x, LA, "bt")]
                for j, z in enumerate(zs):
                    q_ref[j, r // 2:r // 2 + 8, :] = z
                return [v for z in zs for v in _vregs(z)]
            return [(functools.partial(task, r), 55) for r in range(0, bq, 16)]

        def shift_tasks():
            def head():
                out = []
                for c in range(nl):
                    y = g_ref[c, bm:bm + HALO, :]
                    g_ref[c, 0:HALO, :] = y
                    out += _vregs(y)
                return out

            def task(r):
                out = []
                for c in range(nl):
                    y = gn_ref[c, r:r + 32, :]
                    g_ref[c, HALO + r:HALO + r + 32, :] = y
                    out += _vregs(y)
                return out
            return [(head, 8)] + [(functools.partial(task, r), 16) for r in range(0, bm, 32)]

        def key_tasks(base, r0, n, gate=lambda w: w):
            def task(r):
                parts = [_ln(_unzip(x_rows(base + a * kw + r0 + r), gate)) for a in range(na)]
                zs = [_zip(z) for z in _ops(jnp.concatenate(parts, axis=0), LA, "b")]
                for j, z in enumerate(zs):
                    kv_ref[j, pl.ds(pl.multiple_of((r0 + r) // 2, 8), 8), :] = z
                return [v for z in (zs if ktok else zs[6::7]) for v in _vregs(z)]
            return [(functools.partial(task, r), kcost2) for r in range(0, n, 16)]

        def proj(pacer, src, w, dst, cols, skip=0):
            for n, c in enumerate(cols):
                lhs = _unpack(src[0:bm // 2, :]) if n < skip else pacer.tie(src[0:bm // 2, :])
                y = pacer.seen(_dot(lhs, _unpack(wp_ref[w, :, c * 128:(c + 1) * 128])))
                if len(dst.shape) == 3:
                    dst[c, 0:bm, :] = y
                else:
                    dst[0:bm, c * 128:(c + 1) * 128] = y
            return y

        copies = []

        def fetch(src, dst):
            copies.append(pltpu.make_async_copy(src, dst, sems.at[len(copies)]))
            return copies[-1]

        def fetch_x(b, r0, r1):
            return fetch(x_hbm.at[b, pl.ds(r0, r1 - r0)], x_ref.at[pl.ds(b * Tp + r0, r1 - r0)])

        pre = R * rpre
        first = [fetch(wq_hbm, wq_ref), fetch(wk_hbm, wk_ref), fetch_x(0, 0, bm)]
        second = [fetch(wup_hbm, wup_ref)]
        third = [fetch(wv_hbm, wv_ref), fetch(wao_hbm, wao_ref), fetch_x(0, bm, kw)]
        third += [fetch_x(0, a * kw, a * kw + pre) for a in range(1, na)]
        fourth = [fetch(wdn_hbm, wdn_ref), fetch(wm_hbm, wm_ref), fetch(dw_hbm, dw_ref)]
        fifth = [fetch_x(0, a * kw + pre, min(T, (a + 1) * kw)) for a in range(1, na)]
        batches = {b: fetch_x(b, 0, T) for b in range(1, B)}

        def start(group):
            for c in group:
                c.start()

        def wait(group):
            for c in group:
                c.wait()

        @pl.when(step == 0)
        def _():
            start(first)
            for b in range(B):
                x_ref[b * Tp + T:(b + 1) * Tp, :] = jnp.zeros((Tp - T, D), BF16)
            for c in range(nl):
                g_ref[c, bm:bm + HALO, :] = jnp.zeros((HALO, 128), F32)
            wait(first)
            start(second + third)
            early = Pacer(zero, arity)

            def mm(lhs, rhs_ref, r0):
                cols = [_dot(early.tie(lhs), rhs_ref[r0:r0 + D, c:c + 128]) for c in range(0, D, 128)]
                return jnp.concatenate([early.seen(y) for y in cols], axis=1)
            early.spread(norm_tasks(0), D // 16)
            m = _dot_nt(early.tie(pltpu.bitcast(wq_ref[...], U32)), wk_ref[...])
            wp_ref[0] = _pack_rows(m * (LOG2E * float(D) ** -0.5))
            fence(hq_ref, proj(early, xa_ref, 0, hq_ref, range(nl)))
            wait(second)
            start(fourth)
            wp_ref[1] = pltpu.bitcast(wup_ref[:, 0:D], U32)
            wp_ref[2] = pltpu.bitcast(wup_ref[:, D:2 * D], U32)
            early.spread(q_tasks(), nl * (bm // 16), 14, 0, 4)
            fence(hg_ref, proj(early, xa_ref, 2, hg_ref, range(nl)))
            early.spread(gate_tasks(early.after), nl * (bm // 16), 14, 0, 2)
            fence(hu_ref, proj(early, xa_ref, 1, hu_ref, range(nl)))
            wait(third)
            start(fifth)
            early.spread(u_tasks(early.after) + norm_tasks(bm, early.after) + shift_tasks() + key_tasks(0, 0, pre, early.after),
                         3 * nl * (D // 16), 14, 0, kparts)
            t = mm(pltpu.bitcast(wv_ref[...], U32), wao_ref, 0)
            wait(fourth)
            dwf_ref[0:K, :] = dw_ref[...].astype(F32)
            wp_ref[4] = _pack_rows(mm(pltpu.bitcast(wdn_ref[...], U32), wm_ref, D))
            wp_ref[3] = _pack_rows(mm(_pack_rows(t), wm_ref, 0))
            wait(fifth)
            start(batches.values())

        for b in range(1, B):
            @pl.when(step == b * nq - 2)
            def _():
                batches[b].wait()

        @pl.when(i == 0)
        def _():
            def body(j, carry):
                for t, _ in key_tasks(block_row(step), j * R, R):
                    t()
                return carry
            lax.fori_loop(jnp.where(step == 0, rpre, 0), kw // R, body, 0)

        pace = Pacer(zero, arity)
        gates = gate_tasks(pace.after)

        def conv_task(c, r):
            lanes = slice(c * 128, (c + 1) * 128)
            acc = None
            steps = []
            for s in range(8):
                if s and s % (8 // cparts) == 0:
                    steps.append(acc[0:8])
                taps = [k for k in range(K) if (HALO - pad + k) % 8 == s]
                lo = HALO - pad + taps[0] + r
                win = g_ref[c, lo:lo + rc + 8 * (len(taps) - 1), :]
                for n, k in enumerate(taps):
                    t = win[8 * n:8 * n + rc] * dwf_ref[k:k + 1, lanes]
                    acc = t if acc is None else acc + t
            y = _pack_rows(u_ref[r:r + rc, lanes] * acc)
            uc_ref[r // 2:(r + rc) // 2, lanes] = y
            return steps + _vregs(y)
        convs = [(functools.partial(conv_task, c, r), 2 * rc) for r in range(0, bm, rc) for c in range(nl)]
        nlate = nl * pl.cdiv(pad, rc)
        pace.spread(convs[:-nlate], int(qk_frac * nprod * (kw // wq) * (bq // 16)), parts=cparts)
        pace.credit += phase

        mx = None
        for c0 in range(0, kw, wq):
            def prod(j):
                return pace.seen(_dot_nt(pace.tie(q_ref[j]), _unpack(kv_ref[_a_as_b(j, LA), c0 // 2:(c0 + wq) // 2, :])))
            s = _combine(prod, LA, True)
            ts = []
            for a in range(na):
                for c in range(0, wq, 128):
                    t = s[:, a * wq + c:a * wq + c + 128]
                    col0 = a * kw + c0 + c
                    if col0 + 128 > T:
                        col = col0 + lax.broadcasted_iota(jnp.int32, t.shape, 1)
                        t = jnp.where(col < T, t, -jnp.inf)
                    s_ref[0:bm, col0:col0 + 128] = t
                    ts.append(t)
            for n in range(0, len(ts) if qkmax else 0, 2):
                t = functools.reduce(jnp.maximum, ts[n:n + 2])
                mx = t if mx is None else jnp.maximum(mx, t)
        fence(s_ref, ts[-1])
        if qkmax:
            m_ref[0, 0:bm, :] = mx
            fence(m_ref, mx)

        rowmax, rowsum = {}, {}

        def max_task(r):
            if qkmax:
                mx = m_ref[0, r:r + rs, :]
            else:
                part = [s_ref[pl.ds(zero + r, rs), c:c + 128] for c in range(0, Tp, 128)]
                part = [pace.after(t) if n < 2 and relmax else t for n, t in enumerate(part)]
                part = [functools.reduce(jnp.maximum, part[n::2]) for n in range(2)]
                mx = jnp.maximum(*part)
            rowmax[r] = jnp.broadcast_to(jnp.max(mx, axis=-1, keepdims=True), (rs, 128))
            return _vregs(rowmax[r])

        def sum_task(r):
            part = [None] * chains
            mx = pace.after(rowmax[r]) if relsum else rowmax[r]
            for n, c in enumerate(range(0, Tp, 128)):
                e = jnp.exp2(s_ref[r:r + rs, c:c + 128] - mx)
                part[n % chains] = e if part[n % chains] is None else part[n % chains] + e
            rowsum[r] = functools.reduce(jnp.add, part)
            return _vregs(rowsum[r])

        def scale_task(r):
            rl = jnp.broadcast_to(1.0 / jnp.sum(pace.after(rowsum[r]) if relscale else rowsum[r], axis=-1, keepdims=True), (rs, 128))
            m_ref[0, r:r + rs, :] = rowmax[r]
            m_ref[1, r:r + rs, :] = rl
            if r + rs == bm:
                fence(s_ref, rl)
                fence(m_ref, rl)
            return _vregs(rl)

        def prob_task(p_ref, c0, r, c):
            rows = []
            for a in range(na):
                rr = slice(a * bq + r, a * bq + r + 16)
                mx, rl = (pace.after if rel else lambda v: v)(m_ref[0, rr, :]), m_ref[1, rr, :]
                rows.append(jnp.concatenate(
                    [jnp.exp2(s_ref[rr, b * kw + c:b * kw + c + 128] - mx) * rl for b in range(na)], axis=1))
            zs = [_zip(z) for z in _ops(jnp.concatenate(rows, axis=0), LA, "a")]
            for j, z in enumerate(zs):
                p_ref[j, r // 2:r // 2 + 8, c - c0:c - c0 + 128] = z
            return zs if ptok == 49 else [zs[j] for j in range(6, 49, 7)] if ptok == 7 else [zs[j] for j in (40, 41, 47, 48)]

        def prob_tasks(n):
            p_ref, c0, w = p_refs[n], sum(chunks[:n]), chunks[n]

            def last():
                out = prob_task(p_ref, c0, bq - 16, c0 + w - 128)
                fence(p_ref, out[-1])
                return out
            fns = [functools.partial(prob_task, p_ref, c0, r, c) for r in range(0, bq, 16) for c in range(c0, c0 + w, 128)]
            return [(f, pcost) for f in fns[:-1] + [last]]

        rows = list(range(0, bm, rs))
        maxes = [(functools.partial(max_task, r), mcost) for r in rows]
        sums = [(functools.partial(sum_task, r), scost) for r in rows]
        stats = maxes[:ahead]
        for n, t in enumerate(sums):
            stats += [t] + maxes[ahead + n:ahead + n + 1]
        stats += [(functools.partial(scale_task, r), kcost) for r in rows]
        pace.spread(stats + gates[:1] + convs[-nlate:] + prob_tasks(0),
                    (3 * nl + nmid - skip) * (bm // 16), lag[0], back[0], parts[0])
        fence(hg_ref, proj(pace, xa_ref, 2, hg_ref, range(nl), skip))
        proj(pace, xa_ref, 0, hq_ref, range(nl))
        fence(hq_ref, pace.recent[-1])
        proj(pace, xa_ref, 1, hu_ref, range(nl))
        fence(hu_ref, pace.recent[-1])
        assert len(pace.tasks) <= len(prob_tasks(0))
        fence(uc_ref, pace.recent[-1])
        if nmid:
            proj(pace, uc_ref, 4, yc_ref, range(nmid))

        norms = norm_tasks(block_row(jnp.minimum(step + 2, B * nq - 1)), pace.after)
        later = (act_tasks(pace.after) if split else []) + norms + _merge(gates[1:], q_tasks()) + shift_tasks() + ([] if tailu else u_tasks(pace.after))
        c0 = 0
        cut = 0
        for n, w in enumerate(chunks):
            if n + 1 < len(chunks):
                nxt = cut + int(gsplit[n] * len(later))
                pace.spread(_merge(prob_tasks(n + 1), later[cut:nxt]), int(pv_frac * nprod * (bq // 16)), lag[1], back[1], parts[1])
                cut = nxt
            else:
                pace.spread(later[cut:], nprod * (bq // 16), lag[2], back[2], parts[2])
            for j in _order(LA):
                t = pace.seen(_dot(pace.tie(p_refs[n][j]), _unpack(kv_ref[j, c0 // 2:(c0 + w) // 2, :])))
                t = t if c0 == 0 else acc_ref[j] + t
                acc_ref[j] = t
            fence(acc_ref, t)
            c0 += w

        def out_task(r):
            o = _combine(lambda j: acc_ref[j, r:r + 16, :], LA)
            toks = []
            for a in range(na):
                y = _zip(o[16 * a:16 * a + 16])
                ob_ref[(a * bq + r) // 2:(a * bq + r) // 2 + 8, :] = y
                toks += _vregs(y)
            if r + 16 == bq:
                fence(ob_ref, y)
            return toks
        pace.spread([(functools.partial(out_task, r), 1) for r in range(0, bq, 16)],
                    (nl - nmid) * (bm // 16), lag[4], 0, parts[4])
        fence(yc_ref, proj(pace, uc_ref, 4, yc_ref, range(nmid, nl)))
        if tailu:
            pace.spread(u_tasks(pace.after), (nl - 1) * (bm // 16), lag[3], back[3], parts[3])
        for c in range(nl):
            lanes = slice(c * 128, (c + 1) * 128)
            lhs = ob_ref[0:bm // 2, :]
            out = _dot(pace.tie(lhs) if c else _unpack(lhs), _unpack(wp_ref[3, :, lanes]))
            for r in range(0, bm, 16):
                yc = jnp.concatenate([yc_ref[c, pl.ds(r + n, 8, stride=2), :] for n in range(2)], axis=0)
                o_ref[r:r + 16, lanes] = _unpack(_zip(_unzip(x_rows(block_row(step) + r, lanes)) + (yc + out[r:r + 16])))

    @jax.jit
    def fn(x, w_q, w_k, w_v, w_ao, w_up, dw, w_dn, w_merge):
        B, T, D = x.shape
        Tp = pl.cdiv(T, 128 * na) * 128 * na
        nq = pl.cdiv(T, bm)
        ns = B * nq
        ws = (w_q, w_k, w_v, w_ao, w_up, dw, w_dn, w_merge)
        return pl.pallas_call(
            kernel,
            grid=(ns,),
            in_specs=[pl.BlockSpec(memory_space=pl.ANY)] * 9,
            out_specs=pl.BlockSpec((None, bm, D), lambda s: (s // nq, s % nq, 0)),
            out_shape=jax.ShapeDtypeStruct(x.shape, x.dtype),
            scratch_shapes=[pltpu.VMEM((B * Tp, D), x.dtype)] + [pltpu.VMEM(w.shape, w.dtype) for w in ws] + [
                pltpu.SemaphoreType.DMA((len(ws) + 2 * na + B - 1,)),
                pltpu.VMEM((5, D // 2, D), U32),
                pltpu.VMEM((32, D), F32),
                pltpu.VMEM((nprod, Tp // na // 2, D // na), U32),
                pltpu.VMEM((bm // 2 + 8, D), U32),
                pltpu.VMEM((nprod + 1, bq // 2, D // na), U32),
                pltpu.VMEM((bm + 8, D), F32),
                pltpu.VMEM((bm // 2 + 8, D), U32),
                pltpu.VMEM((D // 128, bm + 2 * HALO, 128), F32),
                pltpu.VMEM((D // 128, bm + 8, 128), F32),
                pltpu.VMEM((bm + 8, Tp), F32),
                pltpu.VMEM((2, bm + 8, 128), F32),
                pltpu.VMEM((D // 128, bm + 8, 128), F32),
                pltpu.VMEM((bm + 8, D), F32),
                pltpu.VMEM((bm + 8, D), F32),
                pltpu.VMEM((bm + 8, D), F32),
                pltpu.VMEM((nprod + 1, bq, D // na), F32),
                pltpu.VMEM((bm // 2 + 8, D), U32),
                pltpu.VMEM((bm + 8, D), F32),
            ] + [pltpu.VMEM((nprod + 1, bq // 2, w), U32) for w in chunks],
            compiler_params=pltpu.CompilerParams(dimension_semantics=("arbitrary",), vmem_limit_bytes=120 * 2**20, flags=flags),
        )(x, w_q, w_k, w_v, w_ao, w_up, dw, w_dn, w_merge)
    return fn


_kernel = make()


def pallas_standalone__conformer_family_branchformer__speech_kernel(x, w_q, w_k, w_v, w_ao, w_up, dw, w_dn, w_merge):
    return _kernel(x, w_q, w_k, w_v, w_ao, w_up, dw, w_dn, w_merge)
```

```python
import functools
import math
import jax
import jax.numpy as jnp
from jax import lax
from jax.experimental import pallas as pl
from jax.experimental.pallas import tpu as pltpu

F32 = jnp.float32
BF16 = jnp.bfloat16
U32 = jnp.uint32
EPS = 1e-5
LOG2E = 1.4426950408889634
HALO = 16


def _ln(x):
    m = jnp.mean(x, axis=-1, keepdims=True)
    c = x - m
    v = jnp.mean(c * c, axis=-1, keepdims=True)
    return c * lax.rsqrt(v + EPS)


def _gelu(x):
    c0 = math.sqrt(2.0 / math.pi)
    inner = x * (c0 + (c0 * 0.044715) * (x * x))
    hx = 0.5 * x
    return hx + hx * jnp.tanh(inner)


def _dot(a, b):
    return jnp.dot(a, b, preferred_element_type=F32)


def _dot_nt(a, b):
    return lax.dot_general(a, b, (((1,), (1,)), ((), ())), preferred_element_type=F32)


def _pack(x):
    return pltpu.bitcast(x.astype(BF16), U32)


def _unpack(x):
    return pltpu.bitcast(x, BF16)


def _split(x):
    r, c = x.shape
    return x[:r // 2, :c // 2], x[:r // 2, c // 2:], x[r // 2:, :c // 2], x[r // 2:, c // 2:]


def _join(c11, c12, c21, c22):
    return jnp.concatenate([jnp.concatenate([c11, c12], axis=1),
                            jnp.concatenate([c21, c22], axis=1)], axis=0)


def _ops(x, level, kind):
    if level == 0:
        return [x]
    x11, x12, x21, x22 = _split(x)
    if kind == "a":
        ops = [x11 + x22, x21 + x22, x11, x22, x11 + x12, x21 - x11, x12 - x22]
    elif kind == "b":
        ops = [x11 + x22, x11, x12 - x22, x21 - x11, x22, x11 + x12, x21 + x22]
    else:
        ops = [x11 + x22, x11, x21 - x22, x12 - x11, x22, x11 + x21, x12 + x22]
    return [z for o in ops for z in _ops(o, level - 1, kind)]


_A_AS_B = (0, 6, 1, 4, 5, 3, 2)


def _a_as_b(i, level):
    if level == 0:
        return 0
    n = 7 ** (level - 1)
    return _A_AS_B[i // n] * n + _a_as_b(i % n, level - 1)


ORDER = (0, 3, 4, 6, 2, 1, 5)


def _order(level, order=ORDER):
    if level == 0:
        return [0]
    n = 7 ** (level - 1)
    return [j * n + k for j in order for k in _order(level - 1, order)]


def _combine(get, level, transposed=False, base=0):
    if level == 0:
        return get(base)
    n = 7 ** (level - 1)
    sub = lambda j: _combine(get, level - 1, transposed, base + j * n)
    m0 = sub(0)
    m3 = sub(3)
    t = m0 + m3
    m4 = sub(4)
    t = t - m4
    m6 = sub(6)
    c11 = t + m6
    m2 = sub(2)
    c12 = m2 + m4
    t = m0 + m2
    m1 = sub(1)
    c21 = m1 + m3
    t = t - m1
    m5 = sub(5)
    c22 = t + m5
    if transposed:
        c12, c21 = c21, c12
    return _join(c11, c12, c21, c22)


def _vregs(x):
    return [x[r:r + 8, c:c + 128] for r in range(0, x.shape[0], 8) for c in range(0, x.shape[1], 128)]


def _pack_rows(x):
    return pltpu.bitcast(x.astype(BF16), U32)


def _zip(x):
    return pltpu.pack_elementwise([x[0:8], x[8:16]], packed_dtype=BF16)


def _unzip(x, gate=lambda w: w):
    w = gate(pltpu.bitcast(x, U32))
    return jnp.concatenate([pltpu.unpack_elementwise(w, index=n, packed_dtype=BF16, unpacked_dtype=F32)
                            for n in range(2)], axis=0)


def _tree(xs, arity):
    part = [functools.reduce(lambda a, b: a | b, xs[n::arity]) for n in range(min(arity, len(xs)))]
    while len(part) > 1:
        part = [functools.reduce(lambda a, b: a | b, part[n:n + 2]) for n in range(0, len(part), 2)]
    return part[0]


class Pacer:
    def __init__(self, zero, arity):
        self.arity = arity
        self.keep = lax.broadcasted_iota(jnp.int32, (8, 128), 0) >= zero
        self.tasks, self.due = [], []
        self.recent = []
        self.back = 0
        self.rate = self.credit = self.slot = 0

    def spread(self, tasks, nslots, lag=0, back=0, parts=1):
        assert not self.tasks and not self.due
        self.tasks = list(tasks)
        self.rate = sum(c for _, c in tasks) / (nslots - lag)
        self.end = nslots - 1
        self.credit = tasks[0][1]
        self.slot, self.lag, self.back, self.parts = 0, lag, back, parts

    def seen(self, y):
        self.recent.append(y[0:8, 0:128])
        return y

    def after(self, x):
        tok = pltpu.bitcast(self.recent[max(0, len(self.recent) - 1 - self.back)], x.dtype)
        return jnp.concatenate([jnp.concatenate(
            [jnp.where(self.keep, x[r:r + 8, c:c + 128], tok) for c in range(0, x.shape[1], 128)], axis=1)
            for r in range(0, x.shape[0], 8)], axis=0)

    def tie(self, lhs):
        rows = []
        for r in range(0, lhs.shape[0], 8):
            t = lhs[r:r + 8]
            while self.tasks and self.credit >= self.tasks[0][1] * (1 - 1e-6):
                fn, cost = self.tasks.pop(0)
                self.credit -= cost
                out = [pltpu.bitcast(v, U32) for v in fn()]
                n = min(len(out), self.parts)
                for m in range(n):
                    part = out[m * len(out) // n:(m + 1) * len(out) // n]
                    when = min(self.end, self.slot + self.lag + m * cost / self.rate / n)
                    self.due.append((when, _tree(part, self.arity)))
                self.due.sort(key=lambda d: d[0])
            mine = None
            while self.due and self.due[0][0] <= self.slot:
                tok = self.due.pop(0)[1]
                mine = tok if mine is None else mine | tok
            self.slot += 1
            self.credit += self.rate
            if mine is not None:
                t0 = jnp.where(self.keep, t[:, 0:128], mine)
                t = t0 if t.shape[1] == 128 else jnp.concatenate([t0, t[:, 128:]], axis=1)
            rows.append(t)
        return _unpack(jnp.concatenate(rows, axis=0))


def _merge(xs, ys):
    if not ys:
        return xs
    keyed = [((n + 0.5) / len(xs), 0, n) for n in range(len(xs))] + [((n + 0.5) / len(ys), 1, n) for n in range(len(ys))]
    return [(xs, ys)[w][n] for _, w, n in sorted(keyed)]


def make(bm=448, LA=2, wq=256, chunks=(512, 512), R=64, rpre=8, kcost2=160, ktok=True, kparts=7, kfine=True, rc=16, rs=16, nmid=2, flags=None, qk_frac=1.0,
         pv_frac=1.0, skip=1, pcost=80, scost=70, ptok=7, gsplit=(0.0, 0.0, 0.0), tailu=True, chains=1, phase=0.0, split=False, lag=(10, 30, 10, 6, 14), back=(1, 6, 2, 0), arity=3, parts=(4, 7, 4, 2, 4), rel=True, relscale=True, relsum=False, cparts=8, qkmax=False, ahead=3, relmax=False, mcost=30, kcost=4):
    na = 2 ** LA
    nprod = 7 ** LA
    bq = bm // na
    rg = 16

    def kernel(x_hbm, wq_hbm, wk_hbm, wv_hbm, wao_hbm, wup_hbm, dw_hbm, wdn_hbm, wm_hbm, o_ref,
               x_ref, wq_ref, wk_ref, wv_ref, wao_ref, wup_ref, dw_ref, wdn_ref, wm_ref, sems,
               wp_ref, dwf_ref, kv_ref, xa_ref, q_ref, u_ref, uc_ref, g_ref, gn_ref, s_ref,
               m_ref, yc_ref, hg_ref, hq_ref, hu_ref, acc_ref, ob_ref, ga_ref, *p_refs):
        step = pl.program_id(0)
        B, T, D = x_hbm.shape
        nq = pl.cdiv(T, bm)
        i = step % nq
        Tp = s_ref.shape[1]
        K = dw_ref.shape[0]
        pad = K // 2
        nl = D // 128
        kw = Tp // na
        block_row = lambda n: (n // nq) * Tp + (n % nq) * bm
        W = lambda w: _unpack(wp_ref[w])
        zero = pl.multiple_of(jnp.minimum(step, 0) * 8, 8)

        def fence(ref, val=None):
            idx = tuple(n - 1 for n in ref.shape[:-2]) + (pl.ds(zero + ref.shape[-2] - 8, 8), pl.ds(0, 128))
            ref[idx] = jnp.zeros((8, 128), ref.dtype) if val is None else pltpu.bitcast(val[-8:, -128:], ref.dtype)

        def x_rows(r, lanes=slice(None)):
            return x_ref[pl.ds(r if isinstance(r, int) else pl.multiple_of(r, 16), 16), lanes]

        def norm_tasks(r0, gate=lambda w: w):
            def task(r):
                y = _zip(_ln(_unzip(x_rows(r0 + r), gate)))
                xa_ref[r // 2:r // 2 + 8, :] = y
                if r + 16 == bm:
                    fence(xa_ref, y)
                return _vregs(y)
            return [(functools.partial(task, r), 40) for r in range(0, bm, 16)]

        def act_tasks(gate=lambda w: w):
            def task(r):
                y = _gelu(gate(hg_ref[r:r + 16, :]))
                ga_ref[r:r + 16, :] = y
                if r + 16 == bm:
                    fence(ga_ref, y)
                return _vregs(y)
            return [(functools.partial(task, r), 24) for r in range(HALO, bm, 16)]

        def gate_tasks(gate=lambda w: w):
            def task(r):
                y = _gelu(gate(hg_ref[r:r + 16, :])) if r < HALO or not split else gate(ga_ref[r:r + 16, :])
                g = _ln(y)
                for c in range(nl):
                    gn_ref[c, r:r + 16, :] = g[:, c * 128:(c + 1) * 128]
                    if r < HALO:
                        g_ref[c, HALO + bm + r:HALO + bm + r + 16, :] = g[:, c * 128:(c + 1) * 128]
                if r + 16 == bm:
                    fence(gn_ref, g)
                return _vregs(g)
            return [(functools.partial(task, r), 30) for r in range(0, bm, 16)]

        def u_tasks(gate=lambda w: w):
            def task(r):
                y = _gelu(gate(hu_ref[r:r + 16, :]))
                u_ref[r:r + 16, :] = y
                return _vregs(y)
            return [(functools.partial(task, r), 24) for r in range(0, bm, 16)]

        def q_tasks():
            def task(r):
                x = jnp.concatenate([hq_ref[a * bq + r:a * bq + r + 16, :] for a in range(na)], axis=0)
                zs = [_zip(z) for z in _ops(x, LA, "bt")]
                for j, z in enumerate(zs):
                    q_ref[j, r // 2:r // 2 + 8, :] = z
                return [v for z in zs for v in _vregs(z)]
            return [(functools.partial(task, r), 55) for r in range(0, bq, 16)]

        def shift_tasks():
            def head():
                out = []
                for c in range(nl):
                    y = g_ref[c, bm:bm + HALO, :]
                    g_ref[c, 0:HALO, :] = y
                    out += _vregs(y)
                return out

            def task(r):
                out = []
                for c in range(nl):
                    y = gn_ref[c, r:r + 32, :]
                    g_ref[c, HALO + r:HALO + r + 32, :] = y
                    out += _vregs(y)
                return out
            return [(head, 8)] + [(functools.partial(task, r), 16) for r in range(0, bm, 32)]

        def key_tasks(base, r0, n, gate=lambda w: w):
            def task(r):
                parts = [_ln(_unzip(x_rows(base + a * kw + r0 + r), gate)) for a in range(na)]
                zs = [_zip(z) for z in _ops(jnp.concatenate(parts, axis=0), LA, "b")]
                for j, z in enumerate(zs):
                    kv_ref[j, pl.ds(pl.multiple_of((r0 + r) // 2, 8), 8), :] = z
                return [v for z in (zs if ktok else zs[6::7]) for v in _vregs(z)]
            return [(functools.partial(task, r), kcost2) for r in range(0, n, 16)]

        def proj(pacer, src, w, dst, cols, skip=0):
            for n, c in enumerate(cols):
                lhs = _unpack(src[0:bm // 2, :]) if n < skip else pacer.tie(src[0:bm // 2, :])
                y = pacer.seen(_dot(lhs, _unpack(wp_ref[w, :, c * 128:(c + 1) * 128])))
                if len(dst.shape) == 3:
                    dst[c, 0:bm, :] = y
                else:
                    dst[0:bm, c * 128:(c + 1) * 128] = y
            return y

        copies = []

        def fetch(src, dst):
            copies.append(pltpu.make_async_copy(src, dst, sems.at[len(copies)]))
            return copies[-1]

        def fetch_x(b, r0, r1):
            return fetch(x_hbm.at[b, pl.ds(r0, r1 - r0)], x_ref.at[pl.ds(b * Tp + r0, r1 - r0)])

        pre = R * rpre
        halves = [(slice(None), pl.ds(n * D, D)) for n in range(2)]
        group = [
            [fetch_x(0, 0, bm)],
            [fetch(wup_hbm.at[halves[1]], wup_ref.at[halves[1]])],
            [fetch(wup_hbm.at[halves[0]], wup_ref.at[halves[0]])],
            [fetch(wq_hbm, wq_ref), fetch(wk_hbm, wk_ref)],
            [fetch(wv_hbm, wv_ref), fetch(wao_hbm, wao_ref), fetch_x(0, bm, kw)]
            + [fetch_x(0, a * kw, a * kw + pre) for a in range(1, na)],
            [fetch(wdn_hbm, wdn_ref), fetch(wm_hbm, wm_ref), fetch(dw_hbm, dw_ref)],
            [fetch_x(0, a * kw + pre, min(T, (a + 1) * kw)) for a in range(1, na)],
        ]
        batches = {b: fetch_x(b, 0, T) for b in range(1, B)}

        def start(group):
            for c in group:
                c.start()

        def wait(group):
            for c in group:
                c.wait()

        @pl.when(step == 0)
        def _():
            start(group[0] + group[1])
            for b in range(B):
                x_ref[b * Tp + T:(b + 1) * Tp, :] = jnp.zeros((Tp - T, D), BF16)
            for c in range(nl):
                g_ref[c, bm:bm + HALO, :] = jnp.zeros((HALO, 128), F32)
            wait(group[0])
            start(group[2] + group[3])
            early = Pacer(zero, arity)

            def mm(lhs, rhs_ref, r0):
                cols = [_dot(early.tie(lhs), rhs_ref[r0:r0 + D, c:c + 128]) for c in range(0, D, 128)]
                return jnp.concatenate([early.seen(y) for y in cols], axis=1)
            for t, _ in norm_tasks(0):
                t()
            wait(group[1])
            start(group[4])
            wp_ref[2] = pltpu.bitcast(wup_ref[:, D:2 * D], U32)
            fence(hg_ref, proj(early, xa_ref, 2, hg_ref, range(nl)))
            wait(group[2])
            wp_ref[1] = pltpu.bitcast(wup_ref[:, 0:D], U32)
            early.spread(gate_tasks(early.after), nl * (bm // 16), 14, 0, 2)
            fence(hu_ref, proj(early, xa_ref, 1, hu_ref, range(nl)))
            wait(group[3])
            start(group[5])
            early.spread(u_tasks(early.after) + shift_tasks(), D // 16 + nl * (bm // 16), 14, 0, 2)
            m = _dot_nt(early.tie(pltpu.bitcast(wq_ref[...], U32)), wk_ref[...])
            wp_ref[0] = _pack_rows(m * (LOG2E * float(D) ** -0.5))
            fence(hq_ref, proj(early, xa_ref, 0, hq_ref, range(nl)))
            wait(group[4])
            start(group[6])
            early.spread(q_tasks() + norm_tasks(bm, early.after) + key_tasks(0, 0, pre, early.after),
                         3 * nl * (D // 16), 14, 0, kparts)
            t = mm(pltpu.bitcast(wv_ref[...], U32), wao_ref, 0)
            wait(group[5])
            dwf_ref[0:K, :] = dw_ref[...].astype(F32)
            wp_ref[4] = _pack_rows(mm(pltpu.bitcast(wdn_ref[...], U32), wm_ref, D))
            wp_ref[3] = _pack_rows(mm(_pack_rows(t), wm_ref, 0))
            wait(group[6])
            start(batches.values())

        for b in range(1, B):
            @pl.when(step == b * nq - 2)
            def _():
                batches[b].wait()

        @pl.when(i == 0)
        def _():
            def body(j, carry):
                for t, _ in key_tasks(block_row(step), j * R, R):
                    t()
                return carry
            lax.fori_loop(jnp.where(step == 0, rpre, 0), kw // R, body, 0)

        pace = Pacer(zero, arity)
        gates = gate_tasks(pace.after)

        def conv_task(c, r):
            lanes = slice(c * 128, (c + 1) * 128)
            acc = None
            steps = []
            for s in range(8):
                if s and s % (8 // cparts) == 0:
                    steps.append(acc[0:8])
                taps = [k for k in range(K) if (HALO - pad + k) % 8 == s]
                lo = HALO - pad + taps[0] + r
                win = g_ref[c, lo:lo + rc + 8 * (len(taps) - 1), :]
                for n, k in enumerate(taps):
                    t = win[8 * n:8 * n + rc] * dwf_ref[k:k + 1, lanes]
                    acc = t if acc is None else acc + t
            y = _pack_rows(u_ref[r:r + rc, lanes] * acc)
            uc_ref[r // 2:(r + rc) // 2, lanes] = y
            return steps + _vregs(y)
        convs = [(functools.partial(conv_task, c, r), 2 * rc) for r in range(0, bm, rc) for c in range(nl)]
        nlate = nl * pl.cdiv(pad, rc)
        pace.spread(convs[:-nlate], int(qk_frac * nprod * (kw // wq) * (bq // 16)), parts=cparts)
        pace.credit += phase

        mx = None
        for c0 in range(0, kw, wq):
            def prod(j):
                return pace.seen(_dot_nt(pace.tie(q_ref[j]), _unpack(kv_ref[_a_as_b(j, LA), c0 // 2:(c0 + wq) // 2, :])))
            s = _combine(prod, LA, True)
            ts = []
            for a in range(na):
                for c in range(0, wq, 128):
                    t = s[:, a * wq + c:a * wq + c + 128]
                    col0 = a * kw + c0 + c
                    if col0 + 128 > T:
                        col = col0 + lax.broadcasted_iota(jnp.int32, t.shape, 1)
                        t = jnp.where(col < T, t, -jnp.inf)
                    s_ref[0:bm, col0:col0 + 128] = t
                    ts.append(t)
            for n in range(0, len(ts) if qkmax else 0, len(ts) // 2):
                t = functools.reduce(jnp.maximum, ts[n:n + len(ts) // 2])
                mx = t if mx is None else jnp.maximum(mx, t)
        fence(s_ref, ts[-1])
        if qkmax:
            m_ref[0, 0:bm, :] = mx
            fence(m_ref, mx)

        rowmax, rowsum = {}, {}

        def max_task(r):
            if qkmax:
                mx = m_ref[0, r:r + rs, :]
            else:
                part = [s_ref[pl.ds(zero + r, rs), c:c + 128] for c in range(0, Tp, 128)]
                part = [pace.after(t) if n < 2 and relmax else t for n, t in enumerate(part)]
                part = [functools.reduce(jnp.maximum, part[n::2]) for n in range(2)]
                mx = jnp.maximum(*part)
            rowmax[r] = jnp.broadcast_to(jnp.max(mx, axis=-1, keepdims=True), (rs, 128))
            return _vregs(rowmax[r])

        def sum_task(r):
            part = [None] * chains
            mx = pace.after(rowmax[r]) if relsum else rowmax[r]
            for n, c in enumerate(range(0, Tp, 128)):
                e = jnp.exp2(s_ref[r:r + rs, c:c + 128] - mx)
                part[n % chains] = e if part[n % chains] is None else part[n % chains] + e
            rowsum[r] = functools.reduce(jnp.add, part)
            return _vregs(rowsum[r])

        def scale_task(r):
            rl = jnp.broadcast_to(1.0 / jnp.sum(pace.after(rowsum[r]) if relscale else rowsum[r], axis=-1, keepdims=True), (rs, 128))
            m_ref[0, r:r + rs, :] = rowmax[r]
            m_ref[1, r:r + rs, :] = rl
            if r + rs == bm:
                fence(s_ref, rl)
                fence(m_ref, rl)
            return _vregs(rl)

        def prob_task(p_ref, c0, r, c):
            rows = []
            for a in range(na):
                rr = slice(a * bq + r, a * bq + r + 16)
                mx, rl = (pace.after if rel else lambda v: v)(m_ref[0, rr, :]), m_ref[1, rr, :]
                rows.append(jnp.concatenate(
                    [jnp.exp2(s_ref[rr, b * kw + c:b * kw + c + 128] - mx) * rl for b in range(na)], axis=1))
            zs = [_zip(z) for z in _ops(jnp.concatenate(rows, axis=0), LA, "a")]
            for j, z in enumerate(zs):
                p_ref[j, r // 2:r // 2 + 8, c - c0:c - c0 + 128] = z
            return zs if ptok == 49 else [zs[j] for j in range(6, 49, 7)] if ptok == 7 else [zs[j] for j in (40, 41, 47, 48)]

        def prob_tasks(n):
            p_ref, c0, w = p_refs[n], sum(chunks[:n]), chunks[n]

            def last():
                out = prob_task(p_ref, c0, bq - 16, c0 + w - 128)
                fence(p_ref, out[-1])
                return out
            fns = [functools.partial(prob_task, p_ref, c0, r, c) for r in range(0, bq, 16) for c in range(c0, c0 + w, 128)]
            return [(f, pcost) for f in fns[:-1] + [last]]

        rows = list(range(0, bm, rs))
        maxes = [(functools.partial(max_task, r), mcost) for r in rows]
        sums = [(functools.partial(sum_task, r), scost) for r in rows]
        stats = maxes[:ahead]
        for n, t in enumerate(sums):
            stats += [t] + maxes[ahead + n:ahead + n + 1]
        stats += [(functools.partial(scale_task, r), kcost) for r in rows]
        pace.spread(stats + gates[:1] + convs[-nlate:] + prob_tasks(0),
                    (3 * nl + nmid - skip) * (bm // 16), lag[0], back[0], parts[0])
        fence(hg_ref, proj(pace, xa_ref, 2, hg_ref, range(nl), skip))
        proj(pace, xa_ref, 0, hq_ref, range(nl))
        fence(hq_ref, pace.recent[-1])
        proj(pace, xa_ref, 1, hu_ref, range(nl))
        fence(hu_ref, pace.recent[-1])
        assert len(pace.tasks) <= len(prob_tasks(0))
        fence(uc_ref, pace.recent[-1])
        if nmid:
            proj(pace, uc_ref, 4, yc_ref, range(nmid))

        norms = norm_tasks(block_row(jnp.minimum(step + 2, B * nq - 1)), pace.after)
        later = (act_tasks(pace.after) if split else []) + norms + _merge(gates[1:], q_tasks()) + shift_tasks() + ([] if tailu else u_tasks(pace.after))
        c0 = 0
        cut = 0
        for n, w in enumerate(chunks):
            if n + 1 < len(chunks):
                nxt = cut + int(gsplit[n] * len(later))
                pace.spread(_merge(prob_tasks(n + 1), later[cut:nxt]), int(pv_frac * nprod * (bq // 16)), lag[1], back[1], parts[1])
                cut = nxt
            else:
                pace.spread(later[cut:], nprod * (bq // 16), lag[2], back[2], parts[2])
            for j in _order(LA):
                t = pace.seen(_dot(pace.tie(p_refs[n][j]), _unpack(kv_ref[j, c0 // 2:(c0 + w) // 2, :])))
                t = t if c0 == 0 else acc_ref[j] + t
                acc_ref[j] = t
            fence(acc_ref, t)
            c0 += w

        def out_task(r):
            o = _combine(lambda j: acc_ref[j, r:r + 16, :], LA)
            toks = []
            for a in range(na):
                y = _zip(o[16 * a:16 * a + 16])
                ob_ref[(a * bq + r) // 2:(a * bq + r) // 2 + 8, :] = y
                toks += _vregs(y)
            if r + 16 == bq:
                fence(ob_ref, y)
            return toks
        pace.spread([(functools.partial(out_task, r), 1) for r in range(0, bq, 16)],
                    (nl - nmid) * (bm // 16), lag[4], 0, parts[4])
        fence(yc_ref, proj(pace, uc_ref, 4, yc_ref, range(nmid, nl)))
        if tailu:
            pace.spread(u_tasks(pace.after), (nl - 1) * (bm // 16), lag[3], back[3], parts[3])
        for c in range(nl):
            lanes = slice(c * 128, (c + 1) * 128)
            lhs = ob_ref[0:bm // 2, :]
            out = _dot(pace.tie(lhs) if c else _unpack(lhs), _unpack(wp_ref[3, :, lanes]))
            for r in range(0, bm, 16):
                yc = jnp.concatenate([yc_ref[c, pl.ds(r + n, 8, stride=2), :] for n in range(2)], axis=0)
                o_ref[r:r + 16, lanes] = _unpack(_zip(_unzip(x_rows(block_row(step) + r, lanes)) + (yc + out[r:r + 16])))

    @jax.jit
    def fn(x, w_q, w_k, w_v, w_ao, w_up, dw, w_dn, w_merge):
        B, T, D = x.shape
        Tp = pl.cdiv(T, 128 * na) * 128 * na
        nq = pl.cdiv(T, bm)
        ns = B * nq
        ws = (w_q, w_k, w_v, w_ao, w_up, dw, w_dn, w_merge)
        return pl.pallas_call(
            kernel,
            grid=(ns,),
            in_specs=[pl.BlockSpec(memory_space=pl.ANY)] * 9,
            out_specs=pl.BlockSpec((None, bm, D), lambda s: (s // nq, s % nq, 0)),
            out_shape=jax.ShapeDtypeStruct(x.shape, x.dtype),
            scratch_shapes=[pltpu.VMEM((B * Tp, D), x.dtype)] + [pltpu.VMEM(w.shape, w.dtype) for w in ws] + [
                pltpu.SemaphoreType.DMA((len(ws) + 2 * na + B,)),
                pltpu.VMEM((5, D // 2, D), U32),
                pltpu.VMEM((32, D), F32),
                pltpu.VMEM((nprod, Tp // na // 2, D // na), U32),
                pltpu.VMEM((bm // 2 + 8, D), U32),
                pltpu.VMEM((nprod + 1, bq // 2, D // na), U32),
                pltpu.VMEM((bm + 8, D), F32),
                pltpu.VMEM((bm // 2 + 8, D), U32),
                pltpu.VMEM((D // 128, bm + 2 * HALO, 128), F32),
                pltpu.VMEM((D // 128, bm + 8, 128), F32),
                pltpu.VMEM((bm + 8, Tp), F32),
                pltpu.VMEM((2, bm + 8, 128), F32),
                pltpu.VMEM((D // 128, bm + 8, 128), F32),
                pltpu.VMEM((bm + 8, D), F32),
                pltpu.VMEM((bm + 8, D), F32),
                pltpu.VMEM((bm + 8, D), F32),
                pltpu.VMEM((nprod + 1, bq, D // na), F32),
                pltpu.VMEM((bm // 2 + 8, D), U32),
                pltpu.VMEM((bm + 8, D), F32),
            ] + [pltpu.VMEM((nprod + 1, bq // 2, w), U32) for w in chunks],
            compiler_params=pltpu.CompilerParams(dimension_semantics=("arbitrary",), vmem_limit_bytes=120 * 2**20, flags=flags),
        )(x, w_q, w_k, w_v, w_ao, w_up, dw, w_dn, w_merge)
    return fn


_kernel = make()


def pallas_standalone__conformer_family_branchformer__speech_kernel(x, w_q, w_k, w_v, w_ao, w_up, dw, w_dn, w_merge):
    return _kernel(x, w_q, w_k, w_v, w_ao, w_up, dw, w_dn, w_merge)
```

```python
import functools
import math
import jax
import jax.numpy as jnp
from jax import lax
from jax.experimental import pallas as pl
from jax.experimental.pallas import tpu as pltpu

F32 = jnp.float32
BF16 = jnp.bfloat16
U32 = jnp.uint32
EPS = 1e-5
LOG2E = 1.4426950408889634
HALO = 16


def _ln(x):
    m = jnp.mean(x, axis=-1, keepdims=True)
    c = x - m
    v = jnp.mean(c * c, axis=-1, keepdims=True)
    return c * lax.rsqrt(v + EPS)


def _gelu(x):
    c0 = math.sqrt(2.0 / math.pi)
    inner = x * (c0 + (c0 * 0.044715) * (x * x))
    hx = 0.5 * x
    return hx + hx * jnp.tanh(inner)


def _dot(a, b):
    return jnp.dot(a, b, preferred_element_type=F32)


def _dot_nt(a, b):
    return lax.dot_general(a, b, (((1,), (1,)), ((), ())), preferred_element_type=F32)


def _pack(x):
    return pltpu.bitcast(x.astype(BF16), U32)


def _unpack(x):
    return pltpu.bitcast(x, BF16)


def _split(x):
    r, c = x.shape
    return x[:r // 2, :c // 2], x[:r // 2, c // 2:], x[r // 2:, :c // 2], x[r // 2:, c // 2:]


def _join(c11, c12, c21, c22):
    return jnp.concatenate([jnp.concatenate([c11, c12], axis=1),
                            jnp.concatenate([c21, c22], axis=1)], axis=0)


def _ops(x, level, kind):
    if level == 0:
        return [x]
    x11, x12, x21, x22 = _split(x)
    if kind == "a":
        ops = [x11 + x22, x21 + x22, x11, x22, x11 + x12, x21 - x11, x12 - x22]
    elif kind == "b":
        ops = [x11 + x22, x11, x12 - x22, x21 - x11, x22, x11 + x12, x21 + x22]
    else:
        ops = [x11 + x22, x11, x21 - x22, x12 - x11, x22, x11 + x21, x12 + x22]
    return [z for o in ops for z in _ops(o, level - 1, kind)]


_A_AS_B = (0, 6, 1, 4, 5, 3, 2)


def _a_as_b(i, level):
    if level == 0:
        return 0
    n = 7 ** (level - 1)
    return _A_AS_B[i // n] * n + _a_as_b(i % n, level - 1)


ORDER = (0, 3, 4, 6, 2, 1, 5)


def _order(level, order=ORDER):
    if level == 0:
        return [0]
    n = 7 ** (level - 1)
    return [j * n + k for j in order for k in _order(level - 1, order)]


def _combine(get, level, transposed=False, base=0):
    if level == 0:
        return get(base)
    n = 7 ** (level - 1)
    sub = lambda j: _combine(get, level - 1, transposed, base + j * n)
    m0 = sub(0)
    m3 = sub(3)
    t = m0 + m3
    m4 = sub(4)
    t = t - m4
    m6 = sub(6)
    c11 = t + m6
    m2 = sub(2)
    c12 = m2 + m4
    t = m0 + m2
    m1 = sub(1)
    c21 = m1 + m3
    t = t - m1
    m5 = sub(5)
    c22 = t + m5
    if transposed:
        c12, c21 = c21, c12
    return _join(c11, c12, c21, c22)


def _vregs(x):
    return [x[r:r + 8, c:c + 128] for r in range(0, x.shape[0], 8) for c in range(0, x.shape[1], 128)]


def _pack_rows(x):
    return pltpu.bitcast(x.astype(BF16), U32)


def _zip(x):
    return pltpu.pack_elementwise([x[0:8], x[8:16]], packed_dtype=BF16)


def _unzip(x, gate=lambda w: w):
    w = gate(pltpu.bitcast(x, U32))
    return jnp.concatenate([pltpu.unpack_elementwise(w, index=n, packed_dtype=BF16, unpacked_dtype=F32)
                            for n in range(2)], axis=0)


def _tree(xs, arity):
    part = [functools.reduce(lambda a, b: a | b, xs[n::arity]) for n in range(min(arity, len(xs)))]
    while len(part) > 1:
        part = [functools.reduce(lambda a, b: a | b, part[n:n + 2]) for n in range(0, len(part), 2)]
    return part[0]


_TERMS = (((0, 1), (3, 1), (4, -1), (6, 1)), ((2, 1), (4, 1)), ((1, 1), (3, 1)), ((0, 1), (1, -1), (2, 1), (5, 1)))


def _combine2(get, orders, transposed=False, base=0):
    if not orders:
        return get(base)
    n = 7 ** (len(orders) - 1)
    quads = [None] * 4
    for j in orders[0]:
        m = _combine2(get, orders[1:], transposed, base + j * n)
        for k, terms in enumerate(_TERMS):
            for i, sign in terms:
                if i == j and quads[k] is None:
                    quads[k] = (m, sign)
                elif i == j:
                    t, tsign = quads[k]
                    quads[k] = (t + m, sign) if sign == tsign else (t - m, 1) if tsign > 0 else (m - t, 1)
    c11, c12, c21, c22 = [t for t, _ in quads]
    return _join(c11, c21, c12, c22) if transposed else _join(c11, c12, c21, c22)


class Pacer:
    def __init__(self, zero, arity):
        self.arity = arity
        self.keep = lax.broadcasted_iota(jnp.int32, (8, 128), 0) >= zero
        self.tasks, self.due = [], []
        self.recent = []
        self.back = 0
        self.rate = self.credit = self.slot = 0

    def spread(self, tasks, nslots, lag=0, back=0, parts=1):
        assert not self.tasks and not self.due
        self.tasks = list(tasks)
        self.rate = sum(c for _, c in tasks) / (nslots - lag)
        self.end = nslots - 1
        self.credit = tasks[0][1]
        self.slot, self.lag, self.back, self.parts = 0, lag, back, parts

    def seen(self, y):
        self.recent.append(y[0:8, 0:128])
        return y

    def after(self, x):
        tok = pltpu.bitcast(self.recent[max(0, len(self.recent) - 1 - self.back)], x.dtype)
        return jnp.concatenate([jnp.concatenate(
            [jnp.where(self.keep, x[r:r + 8, c:c + 128], tok) for c in range(0, x.shape[1], 128)], axis=1)
            for r in range(0, x.shape[0], 8)], axis=0)

    def tie(self, lhs):
        rows = []
        for r in range(0, lhs.shape[0], 8):
            t = lhs[r:r + 8]
            while self.tasks and self.credit >= self.tasks[0][1] * (1 - 1e-6):
                fn, cost = self.tasks.pop(0)
                self.credit -= cost
                out = [pltpu.bitcast(v, U32) for v in fn()]
                n = min(len(out), self.parts)
                for m in range(n):
                    part = out[m * len(out) // n:(m + 1) * len(out) // n]
                    when = min(self.end, self.slot + self.lag + m * cost / self.rate / n)
                    self.due.append((when, _tree(part, self.arity)))
                self.due.sort(key=lambda d: d[0])
            mine = None
            while self.due and self.due[0][0] <= self.slot:
                tok = self.due.pop(0)[1]
                mine = tok if mine is None else mine | tok
            self.slot += 1
            self.credit += self.rate
            if mine is not None:
                t0 = jnp.where(self.keep, t[:, 0:128], mine)
                t = t0 if t.shape[1] == 128 else jnp.concatenate([t0, t[:, 128:]], axis=1)
            rows.append(t)
        return _unpack(jnp.concatenate(rows, axis=0))


def _merge(xs, ys):
    if not ys:
        return xs
    keyed = [((n + 0.5) / len(xs), 0, n) for n in range(len(xs))] + [((n + 0.5) / len(ys), 1, n) for n in range(len(ys))]
    return [(xs, ys)[w][n] for _, w, n in sorted(keyed)]


def make(bm=448, LA=2, wq=256, chunks=(512, 512), R=64, rpre=8, pvo=(0, 3, 4, 6, 2, 1, 5), pvi=(0, 3, 4, 6, 2, 1, 5), outer=(0, 3, 4, 6, 2, 1, 5), inner=(0, 3, 4, 6, 2, 1, 5), kcost2=160, ktok=True, kparts=7, kfine=True, rc=16, rs=16, nmid=2, flags=None, qk_frac=1.0,
         pv_frac=1.0, skip=1, pcost=80, scost=70, ptok=7, gsplit=(0.0, 0.0, 0.0), tailu=True, chains=1, phase=0.0, split=False, lag=(10, 30, 10, 6, 14), back=(1, 6, 2, 0), arity=3, parts=(4, 7, 4, 2, 4), rel=True, relscale=True, relsum=False, cparts=8, qkmax=False, ahead=3, relmax=False, mcost=30, kcost=4):
    na = 2 ** LA
    nprod = 7 ** LA
    bq = bm // na
    rg = 16

    def kernel(x_hbm, wq_hbm, wk_hbm, wv_hbm, wao_hbm, wup_hbm, dw_hbm, wdn_hbm, wm_hbm, o_ref,
               x_ref, wq_ref, wk_ref, wv_ref, wao_ref, wup_ref, dw_ref, wdn_ref, wm_ref, sems,
               wp_ref, dwf_ref, kv_ref, xa_ref, q_ref, u_ref, uc_ref, g_ref, gn_ref, s_ref,
               m_ref, yc_ref, hg_ref, hq_ref, hu_ref, acc_ref, ob_ref, ga_ref, *p_refs):
        step = pl.program_id(0)
        B, T, D = x_hbm.shape
        nq = pl.cdiv(T, bm)
        i = step % nq
        Tp = s_ref.shape[1]
        K = dw_ref.shape[0]
        pad = K // 2
        nl = D // 128
        kw = Tp // na
        block_row = lambda n: (n // nq) * Tp + (n % nq) * bm
        W = lambda w: _unpack(wp_ref[w])
        zero = pl.multiple_of(jnp.minimum(step, 0) * 8, 8)

        def fence(ref, val=None):
            idx = tuple(n - 1 for n in ref.shape[:-2]) + (pl.ds(zero + ref.shape[-2] - 8, 8), pl.ds(0, 128))
            ref[idx] = jnp.zeros((8, 128), ref.dtype) if val is None else pltpu.bitcast(val[-8:, -128:], ref.dtype)

        def x_rows(r, lanes=slice(None)):
            return x_ref[pl.ds(r if isinstance(r, int) else pl.multiple_of(r, 16), 16), lanes]

        def norm_tasks(r0, gate=lambda w: w):
            def task(r):
                y = _zip(_ln(_unzip(x_rows(r0 + r), gate)))
                xa_ref[r // 2:r // 2 + 8, :] = y
                if r + 16 == bm:
                    fence(xa_ref, y)
                return _vregs(y)
            return [(functools.partial(task, r), 40) for r in range(0, bm, 16)]

        def act_tasks(gate=lambda w: w):
            def task(r):
                y = _gelu(gate(hg_ref[r:r + 16, :]))
                ga_ref[r:r + 16, :] = y
                if r + 16 == bm:
                    fence(ga_ref, y)
                return _vregs(y)
            return [(functools.partial(task, r), 24) for r in range(HALO, bm, 16)]

        def gate_tasks(gate=lambda w: w):
            def task(r):
                y = _gelu(gate(hg_ref[r:r + 16, :])) if r < HALO or not split else gate(ga_ref[r:r + 16, :])
                g = _ln(y)
                for c in range(nl):
                    gn_ref[c, r:r + 16, :] = g[:, c * 128:(c + 1) * 128]
                    if r < HALO:
                        g_ref[c, HALO + bm + r:HALO + bm + r + 16, :] = g[:, c * 128:(c + 1) * 128]
                if r + 16 == bm:
                    fence(gn_ref, g)
                return _vregs(g)
            return [(functools.partial(task, r), 30) for r in range(0, bm, 16)]

        def u_tasks(gate=lambda w: w):
            def task(r):
                y = _gelu(gate(hu_ref[r:r + 16, :]))
                u_ref[r:r + 16, :] = y
                return _vregs(y)
            return [(functools.partial(task, r), 24) for r in range(0, bm, 16)]

        def q_tasks():
            def task(r):
                x = jnp.concatenate([hq_ref[a * bq + r:a * bq + r + 16, :] for a in range(na)], axis=0)
                zs = [_zip(z) for z in _ops(x, LA, "bt")]
                for j, z in enumerate(zs):
                    q_ref[j, r // 2:r // 2 + 8, :] = z
                return [v for z in zs for v in _vregs(z)]
            return [(functools.partial(task, r), 55) for r in range(0, bq, 16)]

        def shift_tasks():
            def head():
                out = []
                for c in range(nl):
                    y = g_ref[c, bm:bm + HALO, :]
                    g_ref[c, 0:HALO, :] = y
                    out += _vregs(y)
                return out

            def task(r):
                out = []
                for c in range(nl):
                    y = gn_ref[c, r:r + 32, :]
                    g_ref[c, HALO + r:HALO + r + 32, :] = y
                    out += _vregs(y)
                return out
            return [(head, 8)] + [(functools.partial(task, r), 16) for r in range(0, bm, 32)]

        def key_tasks(base, r0, n, gate=lambda w: w):
            def task(r):
                parts = [_ln(_unzip(x_rows(base + a * kw + r0 + r), gate)) for a in range(na)]
                zs = [_zip(z) for z in _ops(jnp.concatenate(parts, axis=0), LA, "b")]
                for j, z in enumerate(zs):
                    kv_ref[j, pl.ds(pl.multiple_of((r0 + r) // 2, 8), 8), :] = z
                return [v for z in (zs if ktok else zs[6::7]) for v in _vregs(z)]
            return [(functools.partial(task, r), kcost2) for r in range(0, n, 16)]

        def proj(pacer, src, w, dst, cols, skip=0):
            for n, c in enumerate(cols):
                lhs = _unpack(src[0:bm // 2, :]) if n < skip else pacer.tie(src[0:bm // 2, :])
                y = pacer.seen(_dot(lhs, _unpack(wp_ref[w, :, c * 128:(c + 1) * 128])))
                if len(dst.shape) == 3:
                    dst[c, 0:bm, :] = y
                else:
                    dst[0:bm, c * 128:(c + 1) * 128] = y
            return y

        copies = []

        def fetch(src, dst):
            copies.append(pltpu.make_async_copy(src, dst, sems.at[len(copies)]))
            return copies[-1]

        def fetch_x(b, r0, r1):
            return fetch(x_hbm.at[b, pl.ds(r0, r1 - r0)], x_ref.at[pl.ds(b * Tp + r0, r1 - r0)])

        pre = R * rpre
        halves = [(slice(None), pl.ds(n * D, D)) for n in range(2)]
        group = [
            [fetch_x(0, 0, bm)],
            [fetch(wup_hbm.at[halves[1]], wup_ref.at[halves[1]])],
            [fetch(wup_hbm.at[halves[0]], wup_ref.at[halves[0]])],
            [fetch(wq_hbm, wq_ref), fetch(wk_hbm, wk_ref)],
            [fetch(wv_hbm, wv_ref), fetch(wao_hbm, wao_ref), fetch_x(0, bm, kw)]
            + [fetch_x(0, a * kw, a * kw + pre) for a in range(1, na)],
            [fetch(wdn_hbm, wdn_ref), fetch(wm_hbm, wm_ref), fetch(dw_hbm, dw_ref)],
            [fetch_x(0, a * kw + pre, min(T, (a + 1) * kw)) for a in range(1, na)],
        ]
        batches = {b: fetch_x(b, 0, T) for b in range(1, B)}

        def start(group):
            for c in group:
                c.start()

        def wait(group):
            for c in group:
                c.wait()

        @pl.when(step == 0)
        def _():
            start(group[0] + group[1])
            for b in range(B):
                x_ref[b * Tp + T:(b + 1) * Tp, :] = jnp.zeros((Tp - T, D), BF16)
            for c in range(nl):
                g_ref[c, bm:bm + HALO, :] = jnp.zeros((HALO, 128), F32)
            wait(group[0])
            start(group[2] + group[3])
            early = Pacer(zero, arity)

            def mm(lhs, rhs_ref, r0):
                cols = [_dot(early.tie(lhs), rhs_ref[r0:r0 + D, c:c + 128]) for c in range(0, D, 128)]
                return jnp.concatenate([early.seen(y) for y in cols], axis=1)
            for t, _ in norm_tasks(0):
                t()
            wait(group[1])
            start(group[4])
            wp_ref[2] = pltpu.bitcast(wup_ref[:, D:2 * D], U32)
            fence(hg_ref, proj(early, xa_ref, 2, hg_ref, range(nl)))
            wait(group[2])
            wp_ref[1] = pltpu.bitcast(wup_ref[:, 0:D], U32)
            early.spread(gate_tasks(early.after), nl * (bm // 16), 14, 0, 2)
            fence(hu_ref, proj(early, xa_ref, 1, hu_ref, range(nl)))
            wait(group[3])
            start(group[5])
            early.spread(u_tasks(early.after) + shift_tasks(), D // 16 + nl * (bm // 16), 14, 0, 2)
            m = _dot_nt(early.tie(pltpu.bitcast(wq_ref[...], U32)), wk_ref[...])
            wp_ref[0] = _pack_rows(m * (LOG2E * float(D) ** -0.5))
            fence(hq_ref, proj(early, xa_ref, 0, hq_ref, range(nl)))
            wait(group[4])
            start(group[6])
            early.spread(q_tasks() + norm_tasks(bm, early.after) + key_tasks(0, 0, pre, early.after),
                         3 * nl * (D // 16), 14, 0, kparts)
            t = mm(pltpu.bitcast(wv_ref[...], U32), wao_ref, 0)
            wait(group[5])
            dwf_ref[0:K, :] = dw_ref[...].astype(F32)
            wp_ref[4] = _pack_rows(mm(pltpu.bitcast(wdn_ref[...], U32), wm_ref, D))
            wp_ref[3] = _pack_rows(mm(_pack_rows(t), wm_ref, 0))
            wait(group[6])
            start(batches.values())

        for b in range(1, B):
            @pl.when(step == b * nq - 2)
            def _():
                batches[b].wait()

        @pl.when(i == 0)
        def _():
            def body(j, carry):
                for t, _ in key_tasks(block_row(step), j * R, R):
                    t()
                return carry
            lax.fori_loop(jnp.where(step == 0, rpre, 0), kw // R, body, 0)

        pace = Pacer(zero, arity)
        gates = gate_tasks(pace.after)

        def conv_task(c, r):
            lanes = slice(c * 128, (c + 1) * 128)
            acc = None
            steps = []
            for s in range(8):
                if s and s % (8 // cparts) == 0:
                    steps.append(acc[0:8])
                taps = [k for k in range(K) if (HALO - pad + k) % 8 == s]
                lo = HALO - pad + taps[0] + r
                win = g_ref[c, lo:lo + rc + 8 * (len(taps) - 1), :]
                for n, k in enumerate(taps):
                    t = win[8 * n:8 * n + rc] * dwf_ref[k:k + 1, lanes]
                    acc = t if acc is None else acc + t
            y = _pack_rows(u_ref[r:r + rc, lanes] * acc)
            uc_ref[r // 2:(r + rc) // 2, lanes] = y
            return steps + _vregs(y)
        convs = [(functools.partial(conv_task, c, r), 2 * rc) for r in range(0, bm, rc) for c in range(nl)]
        nlate = nl * pl.cdiv(pad, rc)
        pace.spread(convs[:-nlate], int(qk_frac * nprod * (kw // wq) * (bq // 16)), parts=cparts)
        pace.credit += phase

        mx = None
        for c0 in range(0, kw, wq):
            def prod(j):
                return pace.seen(_dot_nt(pace.tie(q_ref[j]), _unpack(kv_ref[_a_as_b(j, LA), c0 // 2:(c0 + wq) // 2, :])))
            s = _combine2(prod, (outer, inner), True)
            ts = []
            for a in range(na):
                for c in range(0, wq, 128):
                    t = s[:, a * wq + c:a * wq + c + 128]
                    col0 = a * kw + c0 + c
                    if col0 + 128 > T:
                        col = col0 + lax.broadcasted_iota(jnp.int32, t.shape, 1)
                        t = jnp.where(col < T, t, -jnp.inf)
                    s_ref[0:bm, col0:col0 + 128] = t
                    ts.append(t)
            for n in range(0, len(ts) if qkmax else 0, len(ts) // 2):
                t = functools.reduce(jnp.maximum, ts[n:n + len(ts) // 2])
                mx = t if mx is None else jnp.maximum(mx, t)
        fence(s_ref, ts[-1])
        if qkmax:
            m_ref[0, 0:bm, :] = mx
            fence(m_ref, mx)

        rowmax, rowsum = {}, {}

        def max_task(r):
            if qkmax:
                mx = m_ref[0, r:r + rs, :]
            else:
                part = [s_ref[pl.ds(zero + r, rs), c:c + 128] for c in range(0, Tp, 128)]
                part = [pace.after(t) if n < 2 and relmax else t for n, t in enumerate(part)]
                part = [functools.reduce(jnp.maximum, part[n::2]) for n in range(2)]
                mx = jnp.maximum(*part)
            rowmax[r] = jnp.broadcast_to(jnp.max(mx, axis=-1, keepdims=True), (rs, 128))
            return _vregs(rowmax[r])

        def sum_task(r):
            part = [None] * chains
            mx = pace.after(rowmax[r]) if relsum else rowmax[r]
            for n, c in enumerate(range(0, Tp, 128)):
                e = jnp.exp2(s_ref[r:r + rs, c:c + 128] - mx)
                part[n % chains] = e if part[n % chains] is None else part[n % chains] + e
            rowsum[r] = functools.reduce(jnp.add, part)
            return _vregs(rowsum[r])

        def scale_task(r):
            rl = jnp.broadcast_to(1.0 / jnp.sum(pace.after(rowsum[r]) if relscale else rowsum[r], axis=-1, keepdims=True), (rs, 128))
            m_ref[0, r:r + rs, :] = rowmax[r]
            m_ref[1, r:r + rs, :] = rl
            if r + rs == bm:
                fence(s_ref, rl)
                fence(m_ref, rl)
            return _vregs(rl)

        def prob_task(p_ref, c0, r, c):
            rows = []
            for a in range(na):
                rr = slice(a * bq + r, a * bq + r + 16)
                mx, rl = (pace.after if rel else lambda v: v)(m_ref[0, rr, :]), m_ref[1, rr, :]
                rows.append(jnp.concatenate(
                    [jnp.exp2(s_ref[rr, b * kw + c:b * kw + c + 128] - mx) * rl for b in range(na)], axis=1))
            zs = [_zip(z) for z in _ops(jnp.concatenate(rows, axis=0), LA, "a")]
            for j, z in enumerate(zs):
                p_ref[j, r // 2:r // 2 + 8, c - c0:c - c0 + 128] = z
            return zs if ptok == 49 else [zs[j] for j in range(6, 49, 7)] if ptok == 7 else [zs[j] for j in (40, 41, 47, 48)]

        def prob_tasks(n):
            p_ref, c0, w = p_refs[n], sum(chunks[:n]), chunks[n]

            def last():
                out = prob_task(p_ref, c0, bq - 16, c0 + w - 128)
                fence(p_ref, out[-1])
                return out
            fns = [functools.partial(prob_task, p_ref, c0, r, c) for r in range(0, bq, 16) for c in range(c0, c0 + w, 128)]
            return [(f, pcost) for f in fns[:-1] + [last]]

        rows = list(range(0, bm, rs))
        maxes = [(functools.partial(max_task, r), mcost) for r in rows]
        sums = [(functools.partial(sum_task, r), scost) for r in rows]
        stats = maxes[:ahead]
        for n, t in enumerate(sums):
            stats += [t] + maxes[ahead + n:ahead + n + 1]
        stats += [(functools.partial(scale_task, r), kcost) for r in rows]
        pace.spread(stats + gates[:1] + convs[-nlate:] + prob_tasks(0),
                    (3 * nl + nmid - skip) * (bm // 16), lag[0], back[0], parts[0])
        fence(hg_ref, proj(pace, xa_ref, 2, hg_ref, range(nl), skip))
        proj(pace, xa_ref, 0, hq_ref, range(nl))
        fence(hq_ref, pace.recent[-1])
        proj(pace, xa_ref, 1, hu_ref, range(nl))
        fence(hu_ref, pace.recent[-1])
        assert len(pace.tasks) <= len(prob_tasks(0))
        fence(uc_ref, pace.recent[-1])
        if nmid:
            proj(pace, uc_ref, 4, yc_ref, range(nmid))

        norms = norm_tasks(block_row(jnp.minimum(step + 2, B * nq - 1)), pace.after)
        later = (act_tasks(pace.after) if split else []) + norms + _merge(gates[1:], q_tasks()) + shift_tasks() + ([] if tailu else u_tasks(pace.after))
        c0 = 0
        cut = 0
        for n, w in enumerate(chunks):
            if n + 1 < len(chunks):
                nxt = cut + int(gsplit[n] * len(later))
                pace.spread(_merge(prob_tasks(n + 1), later[cut:nxt]), int(pv_frac * nprod * (bq // 16)), lag[1], back[1], parts[1])
                cut = nxt
            else:
                pace.spread(later[cut:], nprod * (bq // 16), lag[2], back[2], parts[2])
            for j in [a * 7 + b for a in pvo for b in pvi]:
                t = pace.seen(_dot(pace.tie(p_refs[n][j]), _unpack(kv_ref[j, c0 // 2:(c0 + w) // 2, :])))
                t = t if c0 == 0 else acc_ref[j] + t
                acc_ref[j] = t
            fence(acc_ref, t)
            c0 += w

        def out_task(r):
            o = _combine(lambda j: acc_ref[j, r:r + 16, :], LA)
            toks = []
            for a in range(na):
                y = _zip(o[16 * a:16 * a + 16])
                ob_ref[(a * bq + r) // 2:(a * bq + r) // 2 + 8, :] = y
                toks += _vregs(y)
            if r + 16 == bq:
                fence(ob_ref, y)
            return toks
        pace.spread([(functools.partial(out_task, r), 1) for r in range(0, bq, 16)],
                    (nl - nmid) * (bm // 16), lag[4], 0, parts[4])
        fence(yc_ref, proj(pace, uc_ref, 4, yc_ref, range(nmid, nl)))
        if tailu:
            pace.spread(u_tasks(pace.after), (nl - 1) * (bm // 16), lag[3], back[3], parts[3])
        for c in range(nl):
            lanes = slice(c * 128, (c + 1) * 128)
            lhs = ob_ref[0:bm // 2, :]
            out = _dot(pace.tie(lhs) if c else _unpack(lhs), _unpack(wp_ref[3, :, lanes]))
            for r in range(0, bm, 16):
                yc = jnp.concatenate([yc_ref[c, pl.ds(r + n, 8, stride=2), :] for n in range(2)], axis=0)
                o_ref[r:r + 16, lanes] = _unpack(_zip(_unzip(x_rows(block_row(step) + r, lanes)) + (yc + out[r:r + 16])))

    @jax.jit
    def fn(x, w_q, w_k, w_v, w_ao, w_up, dw, w_dn, w_merge):
        B, T, D = x.shape
        Tp = pl.cdiv(T, 128 * na) * 128 * na
        nq = pl.cdiv(T, bm)
        ns = B * nq
        ws = (w_q, w_k, w_v, w_ao, w_up, dw, w_dn, w_merge)
        return pl.pallas_call(
            kernel,
            grid=(ns,),
            in_specs=[pl.BlockSpec(memory_space=pl.ANY)] * 9,
            out_specs=pl.BlockSpec((None, bm, D), lambda s: (s // nq, s % nq, 0)),
            out_shape=jax.ShapeDtypeStruct(x.shape, x.dtype),
            scratch_shapes=[pltpu.VMEM((B * Tp, D), x.dtype)] + [pltpu.VMEM(w.shape, w.dtype) for w in ws] + [
                pltpu.SemaphoreType.DMA((len(ws) + 2 * na + B,)),
                pltpu.VMEM((5, D // 2, D), U32),
                pltpu.VMEM((32, D), F32),
                pltpu.VMEM((nprod, Tp // na // 2, D // na), U32),
                pltpu.VMEM((bm // 2 + 8, D), U32),
                pltpu.VMEM((nprod + 1, bq // 2, D // na), U32),
                pltpu.VMEM((bm + 8, D), F32),
                pltpu.VMEM((bm // 2 + 8, D), U32),
                pltpu.VMEM((D // 128, bm + 2 * HALO, 128), F32),
                pltpu.VMEM((D // 128, bm + 8, 128), F32),
                pltpu.VMEM((bm + 8, Tp), F32),
                pltpu.VMEM((2, bm + 8, 128), F32),
                pltpu.VMEM((D // 128, bm + 8, 128), F32),
                pltpu.VMEM((bm + 8, D), F32),
                pltpu.VMEM((bm + 8, D), F32),
                pltpu.VMEM((bm + 8, D), F32),
                pltpu.VMEM((nprod + 1, bq, D // na), F32),
                pltpu.VMEM((bm // 2 + 8, D), U32),
                pltpu.VMEM((bm + 8, D), F32),
            ] + [pltpu.VMEM((nprod + 1, bq // 2, w), U32) for w in chunks],
            compiler_params=pltpu.CompilerParams(dimension_semantics=("arbitrary",), vmem_limit_bytes=120 * 2**20, flags=flags),
        )(x, w_q, w_k, w_v, w_ao, w_up, dw, w_dn, w_merge)
    return fn


_kernel = make(outer=(1,3,2,4,0,5,6),inner=(4,2,1,3,0,5,6),wq=128,lag=(10,30,14,6,14),qkmax=True,mcost=3,scost=70,pcost=80,tailu=False)


def pallas_standalone__conformer_family_branchformer__speech_kernel(x, w_q, w_k, w_v, w_ao, w_up, dw, w_dn, w_merge):
    return _kernel(x, w_q, w_k, w_v, w_ao, w_up, dw, w_dn, w_merge)
```

```python
import functools
import math

import jax
import jax.numpy as jnp
from jax import lax
from jax.experimental import pallas as pl
from jax.experimental.pallas import tpu as pltpu

F32, BF16, U32 = jnp.float32, jnp.bfloat16, jnp.uint32
EPS = 1e-5
LOG2E = 1.4426950408889634
HALO = 16
LEVELS = 2
PARTS = 2 ** LEVELS
PRODUCTS = 7 ** LEVELS
BLOCK = 448
W_Q, W_U, W_G, W_ATT, W_CONV = range(5)


def _layernorm(x):
    c = x - jnp.mean(x, axis=-1, keepdims=True)
    return c * lax.rsqrt(jnp.mean(c * c, axis=-1, keepdims=True) + EPS)


def _gelu(x):
    c0 = math.sqrt(2.0 / math.pi)
    inner = x * (c0 + (c0 * 0.044715) * (x * x))
    half = 0.5 * x
    return half + half * jnp.tanh(inner)


def _dot(a, b):
    return jnp.dot(a, b, preferred_element_type=F32)


def _dot_nt(a, b):
    return lax.dot_general(a, b, (((1,), (1,)), ((), ())), preferred_element_type=F32)


def _rows(words):
    return pltpu.bitcast(words, BF16)


def _words(x):
    return pltpu.bitcast(x.astype(BF16), U32)


def _zip(x):
    return pltpu.pack_elementwise([x[0:8], x[8:16]], packed_dtype=BF16)


def _unzip(x, gate=lambda w: w):
    w = gate(pltpu.bitcast(x, U32))
    return jnp.concatenate([pltpu.unpack_elementwise(w, index=n, packed_dtype=BF16, unpacked_dtype=F32)
                            for n in range(2)], axis=0)


def _vregs(x):
    return [x[r:r + 8, c:c + 128] for r in range(0, x.shape[0], 8) for c in range(0, x.shape[1], 128)]


def _operands(x, kind, level=LEVELS):
    if level == 0:
        return [x]
    r, c = x.shape[0] // 2, x.shape[1] // 2
    x11, x12, x21, x22 = x[:r, :c], x[:r, c:], x[r:, :c], x[r:, c:]
    if kind == "a":
        sums = [x11 + x22, x21 + x22, x11, x22, x11 + x12, x21 - x11, x12 - x22]
    elif kind == "b":
        sums = [x11 + x22, x11, x12 - x22, x21 - x11, x22, x11 + x12, x21 + x22]
    else:
        sums = [x11 + x22, x11, x21 - x22, x12 - x11, x22, x11 + x21, x12 + x22]
    return [z for s in sums for z in _operands(s, kind, level - 1)]


def _a_as_b(j, level=LEVELS):
    if level == 0:
        return 0
    n = 7 ** (level - 1)
    return (0, 6, 1, 4, 5, 3, 2)[j // n] * n + _a_as_b(j % n, level - 1)


_TERMS = (((0, 1), (3, 1), (4, -1), (6, 1)), ((2, 1), (4, 1)), ((1, 1), (3, 1)), ((0, 1), (1, -1), (2, 1), (5, 1)))


def _assemble(product, orders, transposed=False, base=0):
    if not orders:
        return product(base)
    n = 7 ** (len(orders) - 1)
    quads = [None] * 4
    for j in orders[0]:
        m = _assemble(product, orders[1:], transposed, base + j * n)
        for k, terms in enumerate(_TERMS):
            for i, sign in terms:
                if i == j and quads[k] is None:
                    quads[k] = (m, sign)
                elif i == j:
                    t, tsign = quads[k]
                    quads[k] = (t + m, sign) if sign == tsign else (t - m, 1) if tsign > 0 else (m - t, 1)
    assert all(sign > 0 for _, sign in quads)
    c11, c12, c21, c22 = [t for t, _ in quads]
    if transposed:
        c12, c21 = c21, c12
    return jnp.concatenate([jnp.concatenate([c11, c12], axis=1), jnp.concatenate([c21, c22], axis=1)], axis=0)


class _Pacer:
    def __init__(self, zero):
        self.keep = lax.broadcasted_iota(jnp.int32, (8, 128), 0) >= zero
        self.tasks, self.due, self.recent = [], [], []
        self.rate = self.credit = self.slot = self.back = 0

    def idle(self):
        return not self.tasks and not self.due

    def spread(self, tasks, slots, lag=0, back=0, parts=1):
        assert self.idle()
        self.tasks = list(tasks)
        self.rate = sum(c for _, c in tasks) / (slots - lag)
        self.credit = tasks[0][1]
        self.slot, self.end, self.lag, self.back, self.parts = 0, slots - 1, lag, back, parts

    def seen(self, y):
        self.recent.append(y[0:8, 0:128])
        return y

    def after(self, x):
        token = pltpu.bitcast(self.recent[max(0, len(self.recent) - 1 - self.back)], x.dtype)
        return jnp.concatenate([jnp.concatenate(
            [jnp.where(self.keep, x[r:r + 8, c:c + 128], token) for c in range(0, x.shape[1], 128)], axis=1)
            for r in range(0, x.shape[0], 8)], axis=0)

    @staticmethod
    def _any(xs):
        chains = [functools.reduce(lambda a, b: a | b, xs[n::2]) for n in range(min(2, len(xs)))]
        return functools.reduce(lambda a, b: a | b, chains)

    def tie(self, lhs):
        rows = []
        for r in range(0, lhs.shape[0], 8):
            while self.tasks and self.credit >= self.tasks[0][1] * (1 - 1e-6):
                fn, cost = self.tasks.pop(0)
                self.credit -= cost
                out = [pltpu.bitcast(v, U32) for v in fn()]
                n = min(len(out), self.parts)
                for m in range(n):
                    when = min(self.end, self.slot + self.lag + m * cost / self.rate / n)
                    self.due.append((when, self._any(out[m * len(out) // n:(m + 1) * len(out) // n])))
                self.due.sort(key=lambda d: d[0])
            token = None
            while self.due and self.due[0][0] <= self.slot:
                t = self.due.pop(0)[1]
                token = t if token is None else token | t
            self.slot += 1
            self.credit += self.rate
            t = lhs[r:r + 8]
            if token is not None:
                t0 = jnp.where(self.keep, t[:, 0:128], token)
                t = t0 if t.shape[1] == 128 else jnp.concatenate([t0, t[:, 128:]], axis=1)
            rows.append(t)
        return _rows(jnp.concatenate(rows, axis=0))


def _merge(xs, ys):
    keyed = [((n + 0.5) / len(xs), 0, n) for n in range(len(xs))] + [((n + 0.5) / len(ys), 1, n) for n in range(len(ys))]
    return [(xs, ys)[w][n] for _, w, n in sorted(keyed)]


def _run(tasks):
    for fn, _ in tasks:
        fn()


def _kernel(x_hbm, wq_hbm, wk_hbm, wv_hbm, wao_hbm, wup_hbm, dw_hbm, wdn_hbm, wm_hbm, o_ref,
            x_ref, wq_ref, wk_ref, wv_ref, wao_ref, wup_ref, dw_ref, wdn_ref, wm_ref, sems,
            w_ref, taps_ref, kv_ref, xn_ref, q_ref, u_ref, uc_ref, g_ref, gn_ref, s_ref,
            stat_ref, yc_ref, hg_ref, hq_ref, hu_ref, acc_ref, ob_ref, ln_ref, *p_refs):
    step = pl.program_id(0)
    B, T, D = x_hbm.shape
    K = dw_ref.shape[0]
    Tp = s_ref.shape[1]
    bm, bq = BLOCK, BLOCK // PARTS
    kw = Tp // PARTS
    nq = pl.cdiv(T, bm)
    nl = D // 128
    pad = K // 2
    i = step % nq
    zero = pl.multiple_of(jnp.minimum(step, 0) * 8, 8)

    def block_row(n):
        return (n // nq) * Tp + (n % nq) * bm

    def rows16(r):
        return pl.ds(r if isinstance(r, int) else pl.multiple_of(r, 16), 16)

    def fence(ref, val):
        idx = tuple(n - 1 for n in ref.shape[:-2]) + (pl.ds(zero + ref.shape[-2] - 8, 8), pl.ds(0, 128))
        ref[idx] = pltpu.bitcast(val[-8:, -128:], ref.dtype)


    def block_tasks(r0, normalise):
        def task(r):
            y = _zip(_layernorm(_unzip(x_ref[rows16(r0 + r), :], normalise)) if normalise else ln_ref[rows16(r0 + r), :])
            xn_ref[r // 2:r // 2 + 8, :] = y
            if r + 16 == bm:
                fence(xn_ref, y)
            return _vregs(y)
        return [(functools.partial(task, r), 40 if normalise else 4) for r in range(0, bm, 16)]

    def norm_tasks(r0, n, gate):
        def task(r):
            y = _layernorm(_unzip(x_ref[rows16(r0 + r), :], gate))
            ln_ref[rows16(r0 + r), :] = y
            return _vregs(y)
        return [(functools.partial(task, r), 40) for r in range(0, n, 16)]

    def gate_tasks(gate):
        def task(r):
            g = _layernorm(_gelu(gate(hg_ref[r:r + 16, :])))
            for c in range(nl):
                gn_ref[c, r:r + 16, :] = g[:, c * 128:(c + 1) * 128]
                if r < HALO:
                    g_ref[c, HALO + bm + r:HALO + bm + r + 16, :] = g[:, c * 128:(c + 1) * 128]
            if r + 16 == bm:
                fence(gn_ref, g)
            return _vregs(g)
        return [(functools.partial(task, r), 30) for r in range(0, bm, 16)]

    def shift_tasks():
        def move(src, r, dst, n):
            out = []
            for c in range(nl):
                y = src[c, r:r + n, :]
                g_ref[c, dst:dst + n, :] = y
                out += _vregs(y)
            return out
        return ([(functools.partial(move, g_ref, bm, 0, HALO), 8)]
                + [(functools.partial(move, gn_ref, r, HALO + r, 32), 16) for r in range(0, bm, 32)])

    def u_tasks(gate):
        def task(r):
            y = _gelu(gate(hu_ref[r:r + 16, :]))
            u_ref[r:r + 16, :] = y
            return _vregs(y)
        return [(functools.partial(task, r), 24) for r in range(0, bm, 16)]

    def query_tasks():
        def task(r):
            x = jnp.concatenate([hq_ref[a * bq + r:a * bq + r + 16, :] for a in range(PARTS)], axis=0)
            zs = [_zip(z) for z in _operands(x, "bt")]
            for j, z in enumerate(zs):
                q_ref[j, r // 2:r // 2 + 8, :] = z
            return zs
        return [(functools.partial(task, r), 55) for r in range(0, bq, 16)]

    def key_tasks(base, r0, n, normalise):
        def task(r):
            rows = [base + a * kw + r0 + r for a in range(PARTS)]
            if normalise:
                xs = [_layernorm(_unzip(x_ref[rows16(row), :], normalise)) for row in rows]
                for row, y in zip(rows, xs):
                    ln_ref[rows16(row), :] = y
            else:
                xs = [ln_ref[rows16(row), :] for row in rows]
            zs = [_zip(z) for z in _operands(jnp.concatenate(xs, axis=0), "b")]
            for j, z in enumerate(zs):
                kv_ref[j, pl.ds(pl.multiple_of((r0 + r) // 2, 8), 8), :] = z
            return zs
        return [(functools.partial(task, r), 160) for r in range(0, n, 16)]

    def project(pacer, src, w, dst, cols, untied=0):
        for n, c in enumerate(cols):
            lhs = _rows(src[0:bm // 2, :]) if n < untied else pacer.tie(src[0:bm // 2, :])
            y = pacer.seen(_dot(lhs, _rows(w_ref[w, :, c * 128:(c + 1) * 128])))
            if len(dst.shape) == 3:
                dst[c, 0:bm, :] = y
            else:
                dst[0:bm, c * 128:(c + 1) * 128] = y
        return y

    copies = []

    def fetch(src, dst):
        copies.append(pltpu.make_async_copy(src, dst, sems.at[len(copies)]))
        return copies[-1]

    def fetch_x(b, r0, r1):
        return fetch(x_hbm.at[b, pl.ds(r0, r1 - r0)], x_ref.at[pl.ds(b * Tp + r0, r1 - r0)])

    def start(group):
        for c in group:
            c.start()

    def wait(group):
        for c in group:
            c.wait()

    halves = [(slice(None), pl.ds(n * D, D)) for n in range(2)]
    group = [
        [fetch_x(0, 0, bm)],
        [fetch(wup_hbm.at[halves[1]], wup_ref.at[halves[1]])],
        [fetch(wup_hbm.at[halves[0]], wup_ref.at[halves[0]])],
        [fetch(wq_hbm, wq_ref), fetch(wk_hbm, wk_ref)],
        [fetch(wv_hbm, wv_ref), fetch(wao_hbm, wao_ref), fetch_x(0, bm, kw)]
        + [fetch_x(0, a * kw, a * kw + kw // 2) for a in range(1, PARTS)],
        [fetch(wdn_hbm, wdn_ref), fetch(wm_hbm, wm_ref), fetch(dw_hbm, dw_ref)],
        [fetch_x(0, a * kw + kw // 2, min(T, (a + 1) * kw)) for a in range(1, PARTS)],
    ]
    batches = [fetch_x(b, 0, T) for b in range(1, B)]

    @pl.when(step == 0)
    def _():
        start(group[0] + group[1])
        for b in range(B):
            x_ref[b * Tp + T:(b + 1) * Tp, :] = jnp.zeros((Tp - T, D), x_ref.dtype)
        for c in range(nl):
            g_ref[c, bm:bm + HALO, :] = jnp.zeros((HALO, 128), F32)
        wait(group[0])
        start(group[2] + group[3])
        early = _Pacer(zero)

        def weights(lhs, rhs_ref, r0):
            cols = [_dot(early.tie(lhs), rhs_ref[r0:r0 + D, c:c + 128]) for c in range(0, D, 128)]
            return jnp.concatenate([early.seen(y) for y in cols], axis=1)

        _run(block_tasks(0, lambda w: w))
        wait(group[1])
        start(group[4])
        w_ref[W_G] = pltpu.bitcast(wup_ref[:, D:2 * D], U32)
        fence(hg_ref, project(early, xn_ref, W_G, hg_ref, range(nl)))
        wait(group[2])
        w_ref[W_U] = pltpu.bitcast(wup_ref[:, 0:D], U32)
        early.spread(gate_tasks(early.after), nl * (bm // 16), lag=14, parts=2)
        fence(hu_ref, project(early, xn_ref, W_U, hu_ref, range(nl)))
        wait(group[3])
        start(group[5])
        early.spread(u_tasks(early.after) + shift_tasks(), D // 16 + nl * (bm // 16), lag=14, parts=2)
        qk = _dot_nt(early.tie(pltpu.bitcast(wq_ref[...], U32)), wk_ref[...])
        w_ref[W_Q] = _words(qk * (LOG2E * float(D) ** -0.5))
        fence(hq_ref, project(early, xn_ref, W_Q, hq_ref, range(nl)))
        wait(group[4])
        start(group[6])
        early.spread(query_tasks() + block_tasks(bm, early.after) + key_tasks(0, 0, kw // 2, early.after),
                     3 * nl * (D // 16), lag=14, parts=7)
        vo = weights(pltpu.bitcast(wv_ref[...], U32), wao_ref, 0)
        wait(group[5])
        taps_ref[0:K, :] = dw_ref[...].astype(F32)
        w_ref[W_CONV] = _words(weights(pltpu.bitcast(wdn_ref[...], U32), wm_ref, D))
        w_ref[W_ATT] = _words(weights(_words(vo), wm_ref, 0))
        assert early.idle()
        wait(group[6])
        start(batches)

        @pl.loop(kw // 128, kw // 64)
        def _(j):
            _run(key_tasks(0, j * 64, 64, lambda w: w))

    for n, copy in enumerate(batches):
        pl.when(step == n * nq + 1)(copy.wait)

    @pl.when(jnp.logical_and(i == 0, step > 0))
    def _():
        @pl.loop(0, kw // 16)
        def _(j):
            _run(key_tasks(block_row(step), j * 16, 16, None))

    pace = _Pacer(zero)
    gates = gate_tasks(pace.after)

    def conv_task(c, r):
        lanes = slice(c * 128, (c + 1) * 128)
        acc, partial = None, []
        for shift in range(8):
            if shift:
                partial.append(acc[0:8])
            taps = [k for k in range(K) if (HALO - pad + k) % 8 == shift]
            lo = HALO - pad + taps[0] + r
            window = g_ref[c, lo:lo + 16 + 8 * (len(taps) - 1), :]
            for n, k in enumerate(taps):
                t = window[8 * n:8 * n + 16] * taps_ref[k:k + 1, lanes]
                acc = t if acc is None else acc + t
        y = _words(u_ref[r:r + 16, lanes] * acc)
        uc_ref[r // 2:r // 2 + 8, lanes] = y
        return partial + _vregs(y)
    convs = [(functools.partial(conv_task, c, r), 32) for r in range(0, bm, 16) for c in range(nl)]
    late = nl * pl.cdiv(pad, 16)
    pace.spread(convs[:-late], PRODUCTS * (kw // 128) * (bq // 16), parts=8)

    peak = None
    for c0 in range(0, kw, 128):
        def product(j):
            return pace.seen(_dot_nt(pace.tie(q_ref[j]), _rows(kv_ref[_a_as_b(j), c0 // 2:(c0 + 128) // 2, :])))
        s = _assemble(product, ((1, 3, 2, 4, 0, 5, 6), (2, 5, 4, 0, 1, 3, 6)), transposed=True)
        tiles = []
        for a in range(PARTS):
            t = s[:, a * 128:(a + 1) * 128]
            col0 = a * kw + c0
            if col0 + 128 > T:
                t = jnp.where(col0 + lax.broadcasted_iota(jnp.int32, t.shape, 1) < T, t, -jnp.inf)
            s_ref[0:bm, col0:col0 + 128] = t
            tiles.append(t)
        for n in range(0, PARTS, 2):
            t = jnp.maximum(tiles[n], tiles[n + 1])
            peak = t if peak is None else jnp.maximum(peak, t)
    fence(s_ref, tiles[-1])
    stat_ref[0, 0:bm, :] = peak
    fence(stat_ref, peak)

    rowmax, rowsum = {}, {}

    def max_task(r):
        rowmax[r] = jnp.broadcast_to(jnp.max(stat_ref[0, r:r + 16, :], axis=-1, keepdims=True), (16, 128))
        return _vregs(rowmax[r])

    def sum_task(r):
        total = None
        for c in range(0, Tp, 128):
            e = jnp.exp2(s_ref[r:r + 16, c:c + 128] - rowmax[r])
            total = e if total is None else total + e
        rowsum[r] = total
        return _vregs(total)

    def scale_task(r):
        scale = jnp.broadcast_to(1.0 / jnp.sum(pace.after(rowsum[r]), axis=-1, keepdims=True), (16, 128))
        stat_ref[0, r:r + 16, :] = rowmax[r]
        stat_ref[1, r:r + 16, :] = scale
        if r + 16 == bm:
            fence(s_ref, scale)
            fence(stat_ref, scale)
        return _vregs(scale)

    span = kw // len(p_refs)

    def prob_tasks(n):
        def task(r, c):
            rows = []
            for a in range(PARTS):
                rr = slice(a * bq + r, a * bq + r + 16)
                m, scale = pace.after(stat_ref[0, rr, :]), stat_ref[1, rr, :]
                cols = [b * kw + n * span + c for b in range(PARTS)]
                rows.append(jnp.concatenate([jnp.exp2(s_ref[rr, col:col + 128] - m) * scale for col in cols], axis=1))
            zs = [_zip(z) for z in _operands(jnp.concatenate(rows, axis=0), "a")]
            for j, z in enumerate(zs):
                p_refs[n][j, r // 2:r // 2 + 8, c:c + 128] = z
            if r + 16 == bq and c + 128 == span:
                fence(p_refs[n], zs[-1])
            return zs[6::7]
        return [(functools.partial(task, r, c), 80) for r in range(0, bq, 16) for c in range(0, span, 128)]

    maxes = [(functools.partial(max_task, r), 3) for r in range(0, bm, 16)]
    stats = maxes[:3]
    for n, r in enumerate(range(0, bm, 16)):
        stats += [(functools.partial(sum_task, r), 70)] + maxes[n + 3:n + 4]
    stats += [(functools.partial(scale_task, r), 4) for r in range(0, bm, 16)]
    probs = prob_tasks(0)
    pace.spread(stats + gates[:1] + convs[-late:] + probs, (3 * nl + nl // 2 - 1) * (bm // 16), lag=10, back=1, parts=4)
    fence(hg_ref, project(pace, xn_ref, W_G, hg_ref, range(nl), untied=1))
    assert len(pace.tasks) >= 1 + late + len(probs)
    project(pace, xn_ref, W_Q, hq_ref, range(nl))
    fence(hq_ref, pace.recent[-1])
    project(pace, xn_ref, W_U, hu_ref, range(nl))
    fence(hu_ref, pace.recent[-1])
    assert len(pace.tasks) <= len(probs)
    fence(uc_ref, pace.recent[-1])
    project(pace, uc_ref, W_CONV, yc_ref, range(nl // 2))

    share = Tp // (nq - 1)
    assert share * (nq - 1) == Tp and share % 16 == 0 and 2 * bm <= share * (nq - 3)
    batch = jnp.where(i == 0, step // nq, jnp.minimum(step // nq + 1, B - 1))
    norms = norm_tasks(batch * Tp + jnp.maximum(i - 1, 0) * share, share, pace.after)
    later = (block_tasks(block_row(jnp.minimum(step + 2, B * nq - 1)), None) + norms[8:]
             + _merge(gates[1:], query_tasks()) + shift_tasks())
    cut = int(0.28 * len(later))
    for n, p_ref in enumerate(p_refs):
        if n == 0:
            pace.spread(_merge(prob_tasks(1), later[:cut] + norms[:8]), PRODUCTS * (bq // 16), lag=30, back=6, parts=7)
        else:
            pace.spread(later[cut:], PRODUCTS * (bq // 16), lag=14, back=2, parts=4)
        for j in [a * 7 + b for a in (0, 3, 4, 6, 2, 1, 5) for b in (6, 5, 4, 3, 2, 1, 0)]:
            t = pace.seen(_dot(pace.tie(p_ref[j]), _rows(kv_ref[j, n * span // 2:(n + 1) * span // 2, :])))
            t = t if n == 0 else acc_ref[j] + t
            acc_ref[j] = t
        fence(acc_ref, t)

    def out_task(r):
        o = _assemble(lambda j: acc_ref[j, r:r + 16, :], ((0, 3, 4, 6, 2, 1, 5),) * LEVELS)
        out = []
        for a in range(PARTS):
            y = _zip(o[16 * a:16 * a + 16])
            ob_ref[(a * bq + r) // 2:(a * bq + r) // 2 + 8, :] = y
            out += _vregs(y)
        if r + 16 == bq:
            fence(ob_ref, y)
        return out
    pace.spread([(functools.partial(out_task, r), 1) for r in range(0, bq, 16)], (nl - nl // 2) * (bm // 16), lag=14, parts=4)
    fence(yc_ref, project(pace, uc_ref, W_CONV, yc_ref, range(nl // 2, nl)))
    pace.spread(u_tasks(pace.after), (nl - 1) * (bm // 16), lag=6, parts=2)
    for c in range(nl):
        lanes = slice(c * 128, (c + 1) * 128)
        lhs = ob_ref[0:bm // 2, :]
        ya = _dot(pace.tie(lhs) if c else _rows(lhs), _rows(w_ref[W_ATT, :, lanes]))
        for r in range(0, bm, 16):
            yc = jnp.concatenate([yc_ref[c, pl.ds(r + n, 8, stride=2), :] for n in range(2)], axis=0)
            x = _unzip(x_ref[rows16(block_row(step) + r), lanes])
            o_ref[r:r + 16, lanes] = _rows(_zip(x + (yc + ya[r:r + 16])))
    assert pace.idle()


@jax.jit
def pallas_standalone__conformer_family_branchformer__speech_kernel(
    x: jax.Array,
    w_q: jax.Array,
    w_k: jax.Array,
    w_v: jax.Array,
    w_ao: jax.Array,
    w_up: jax.Array,
    dw: jax.Array,
    w_dn: jax.Array,
    w_merge: jax.Array,
):
    B, T, D = x.shape
    assert x.dtype == BF16 and D == 128 * PARTS and dw.shape[0] < 2 * HALO
    bm, bq = BLOCK, BLOCK // PARTS
    Tp = pl.cdiv(T, 256 * PARTS) * 256 * PARTS
    nq = pl.cdiv(T, bm)
    weights = (w_q, w_k, w_v, w_ao, w_up, dw, w_dn, w_merge)
    return pl.pallas_call(
        _kernel,
        grid=(B * nq,),
        in_specs=[pl.BlockSpec(memory_space=pl.ANY)] * (1 + len(weights)),
        out_specs=pl.BlockSpec((None, bm, D), lambda s: (s // nq, s % nq, 0)),
        out_shape=jax.ShapeDtypeStruct(x.shape, x.dtype),
        scratch_shapes=[pltpu.VMEM((B * Tp, D), x.dtype)] + [pltpu.VMEM(w.shape, w.dtype) for w in weights] + [
            pltpu.SemaphoreType.DMA((len(weights) + 2 * PARTS + B,)),
            pltpu.VMEM((5, D // 2, D), U32),
            pltpu.VMEM((2 * HALO, D), F32),
            pltpu.VMEM((PRODUCTS, Tp // PARTS // 2, 128), U32),
            pltpu.VMEM((bm // 2 + 8, D), U32),
            pltpu.VMEM((PRODUCTS, bq // 2, 128), U32),
            pltpu.VMEM((bm, D), F32),
            pltpu.VMEM((bm // 2 + 8, D), U32),
            pltpu.VMEM((D // 128, bm + 2 * HALO, 128), F32),
            pltpu.VMEM((D // 128, bm + 8, 128), F32),
            pltpu.VMEM((bm + 8, Tp), F32),
            pltpu.VMEM((2, bm + 8, 128), F32),
            pltpu.VMEM((D // 128, bm + 8, 128), F32),
            pltpu.VMEM((bm + 8, D), F32),
            pltpu.VMEM((bm + 8, D), F32),
            pltpu.VMEM((bm + 8, D), F32),
            pltpu.VMEM((PRODUCTS + 1, bq, 128), F32),
            pltpu.VMEM((bm // 2 + 8, D), U32),
            pltpu.VMEM((B * Tp, D), F32),
        ] + [pltpu.VMEM((PRODUCTS + 1, bq // 2, Tp // PARTS // 2), U32)] * 2,
        compiler_params=pltpu.CompilerParams(dimension_semantics=("arbitrary",), vmem_limit_bytes=110 * 2**20),
    )(x, *weights)
```

```python
import functools
import math

import jax
import jax.numpy as jnp
from jax import lax
from jax.experimental import pallas as pl
from jax.experimental.pallas import tpu as pltpu

F32, BF16, U32 = jnp.float32, jnp.bfloat16, jnp.uint32
EPS = 1e-5
LOG2E = 1.4426950408889634
HALO = 16
LEVELS = 2
PARTS = 2 ** LEVELS
PRODUCTS = 7 ** LEVELS
BLOCK = 448
W_Q, W_U, W_G, W_ATT, W_CONV = range(5)


def _layernorm(x):
    c = x - jnp.mean(x, axis=-1, keepdims=True)
    return c * lax.rsqrt(jnp.mean(c * c, axis=-1, keepdims=True) + EPS)


def _gelu(x):
    c0 = math.sqrt(2.0 / math.pi)
    inner = x * (c0 + (c0 * 0.044715) * (x * x))
    half = 0.5 * x
    return half + half * jnp.tanh(inner)


def _dot(a, b):
    return jnp.dot(a, b, preferred_element_type=F32)


def _dot_nt(a, b):
    return lax.dot_general(a, b, (((1,), (1,)), ((), ())), preferred_element_type=F32)


def _rows(words):
    return pltpu.bitcast(words, BF16)


def _words(x):
    return pltpu.bitcast(x.astype(BF16), U32)


def _zip(x):
    return pltpu.pack_elementwise([x[0:8], x[8:16]], packed_dtype=BF16)


def _unzip(x, gate=lambda w: w):
    w = gate(pltpu.bitcast(x, U32))
    return jnp.concatenate([pltpu.unpack_elementwise(w, index=n, packed_dtype=BF16, unpacked_dtype=F32)
                            for n in range(2)], axis=0)


def _vregs(x):
    return [x[r:r + 8, c:c + 128] for r in range(0, x.shape[0], 8) for c in range(0, x.shape[1], 128)]


def _operands(x, kind, level=LEVELS):
    if level == 0:
        return [x]
    r, c = x.shape[0] // 2, x.shape[1] // 2
    x11, x12, x21, x22 = x[:r, :c], x[:r, c:], x[r:, :c], x[r:, c:]
    if kind == "a":
        sums = [x11 + x22, x21 + x22, x11, x22, x11 + x12, x21 - x11, x12 - x22]
    elif kind == "b":
        sums = [x11 + x22, x11, x12 - x22, x21 - x11, x22, x11 + x12, x21 + x22]
    else:
        sums = [x11 + x22, x11, x21 - x22, x12 - x11, x22, x11 + x21, x12 + x22]
    return [z for s in sums for z in _operands(s, kind, level - 1)]


def _a_as_b(j, level=LEVELS):
    if level == 0:
        return 0
    n = 7 ** (level - 1)
    return (0, 6, 1, 4, 5, 3, 2)[j // n] * n + _a_as_b(j % n, level - 1)


_TERMS = (((0, 1), (3, 1), (4, -1), (6, 1)), ((2, 1), (4, 1)), ((1, 1), (3, 1)), ((0, 1), (1, -1), (2, 1), (5, 1)))


def _assemble(product, orders, transposed=False, base=0):
    if not orders:
        return product(base)
    n = 7 ** (len(orders) - 1)
    quads = [None] * 4
    for j in orders[0]:
        m = _assemble(product, orders[1:], transposed, base + j * n)
        for k, terms in enumerate(_TERMS):
            for i, sign in terms:
                if i == j and quads[k] is None:
                    quads[k] = (m, sign)
                elif i == j:
                    t, tsign = quads[k]
                    quads[k] = (t + m, sign) if sign == tsign else (t - m, 1) if tsign > 0 else (m - t, 1)
    assert all(sign > 0 for _, sign in quads)
    c11, c12, c21, c22 = [t for t, _ in quads]
    if transposed:
        c12, c21 = c21, c12
    return jnp.concatenate([jnp.concatenate([c11, c12], axis=1), jnp.concatenate([c21, c22], axis=1)], axis=0)


class _Pacer:
    def __init__(self, zero):
        self.keep = lax.broadcasted_iota(jnp.int32, (8, 128), 0) >= zero
        self.tasks, self.due, self.recent = [], [], []
        self.rate = self.credit = self.slot = self.back = 0

    def idle(self):
        return not self.tasks and not self.due

    def spread(self, tasks, slots, lag=0, back=0, parts=1):
        assert self.idle()
        self.tasks = list(tasks)
        self.rate = sum(c for _, c in tasks) / (slots - lag)
        self.credit = tasks[0][1]
        self.slot, self.end, self.lag, self.back, self.parts = 0, slots - 1, lag, back, parts

    def seen(self, y):
        self.recent.append(y[0:8, 0:128])
        return y

    def after(self, x):
        token = pltpu.bitcast(self.recent[max(0, len(self.recent) - 1 - self.back)], x.dtype)
        return jnp.concatenate([jnp.concatenate(
            [jnp.where(self.keep, x[r:r + 8, c:c + 128], token) for c in range(0, x.shape[1], 128)], axis=1)
            for r in range(0, x.shape[0], 8)], axis=0)

    @staticmethod
    def _any(xs):
        chains = [functools.reduce(lambda a, b: a | b, xs[n::2]) for n in range(min(2, len(xs)))]
        return functools.reduce(lambda a, b: a | b, chains)

    def tie(self, lhs):
        rows = []
        for r in range(0, lhs.shape[0], 8):
            while self.tasks and self.credit >= self.tasks[0][1] * (1 - 1e-6):
                fn, cost = self.tasks.pop(0)
                self.credit -= cost
                out = [pltpu.bitcast(v, U32) for v in fn()]
                n = min(len(out), self.parts)
                for m in range(n):
                    when = min(self.end, self.slot + self.lag + m * cost / self.rate / n)
                    self.due.append((when, self._any(out[m * len(out) // n:(m + 1) * len(out) // n])))
                self.due.sort(key=lambda d: d[0])
            token = None
            while self.due and self.due[0][0] <= self.slot:
                t = self.due.pop(0)[1]
                token = t if token is None else token | t
            self.slot += 1
            self.credit += self.rate
            t = lhs[r:r + 8]
            if token is not None:
                t0 = jnp.where(self.keep, t[:, 0:128], token)
                t = t0 if t.shape[1] == 128 else jnp.concatenate([t0, t[:, 128:]], axis=1)
            rows.append(t)
        return _rows(jnp.concatenate(rows, axis=0))


def _merge(xs, ys):
    keyed = [((n + 0.5) / len(xs), 0, n) for n in range(len(xs))] + [((n + 0.5) / len(ys), 1, n) for n in range(len(ys))]
    return [(xs, ys)[w][n] for _, w, n in sorted(keyed)]


def _run(tasks):
    for fn, _ in tasks:
        fn()


def _kernel(x_hbm, wq_hbm, wk_hbm, wv_hbm, wao_hbm, wup_hbm, dw_hbm, wdn_hbm, wm_hbm, o_ref,
            x_ref, wq_ref, wk_ref, wv_ref, wao_ref, wup_ref, dw_ref, wdn_ref, wm_ref, sems,
            w_ref, taps_ref, kv_ref, xn_ref, q_ref, u_ref, uc_ref, g_ref, gn_ref, s_ref,
            stat_ref, yc_ref, hg_ref, hq_ref, hu_ref, acc_ref, ob_ref, ln_ref, *p_refs):
    step = pl.program_id(0)
    B, T, D = x_hbm.shape
    K = dw_ref.shape[0]
    Tp = s_ref.shape[1]
    bm, bq = BLOCK, BLOCK // PARTS
    kw = Tp // PARTS
    nq = pl.cdiv(T, bm)
    nl = D // 128
    pad = K // 2
    i = step % nq
    zero = pl.multiple_of(jnp.minimum(step, 0) * 8, 8)

    def block_row(n):
        return (n // nq) * Tp + (n % nq) * bm

    def rows16(r):
        return pl.ds(r if isinstance(r, int) else pl.multiple_of(r, 16), 16)

    def fence(ref, val):
        idx = tuple(n - 1 for n in ref.shape[:-2]) + (pl.ds(zero + ref.shape[-2] - 8, 8), pl.ds(0, 128))
        ref[idx] = pltpu.bitcast(val[-8:, -128:], ref.dtype)


    def block_tasks(r0, normalise):
        def task(r):
            y = _zip(_layernorm(_unzip(x_ref[rows16(r0 + r), :], normalise)) if normalise else ln_ref[rows16(r0 + r), :])
            xn_ref[r // 2:r // 2 + 8, :] = y
            if r + 16 == bm:
                fence(xn_ref, y)
            return _vregs(y)
        return [(functools.partial(task, r), 40 if normalise else 4) for r in range(0, bm, 16)]

    def norm_tasks(r0, n, gate):
        def task(r):
            y = _layernorm(_unzip(x_ref[rows16(r0 + r), :], gate))
            ln_ref[rows16(r0 + r), :] = y
            return _vregs(y)
        return [(functools.partial(task, r), 40) for r in range(0, n, 16)]

    def gate_tasks(gate):
        def task(r):
            g = _layernorm(_gelu(gate(hg_ref[r:r + 16, :])))
            for c in range(nl):
                gn_ref[c, r:r + 16, :] = g[:, c * 128:(c + 1) * 128]
                if r < HALO:
                    g_ref[c, HALO + bm + r:HALO + bm + r + 16, :] = g[:, c * 128:(c + 1) * 128]
            if r + 16 == bm:
                fence(gn_ref, g)
            return _vregs(g)
        return [(functools.partial(task, r), 30) for r in range(0, bm, 16)]

    def shift_tasks():
        def move(src, r, dst, n):
            out = []
            for c in range(nl):
                y = src[c, r:r + n, :]
                g_ref[c, dst:dst + n, :] = y
                out += _vregs(y)
            return out
        return ([(functools.partial(move, g_ref, bm, 0, HALO), 8)]
                + [(functools.partial(move, gn_ref, r, HALO + r, 32), 16) for r in range(0, bm, 32)])

    def u_tasks(gate):
        def task(r):
            y = _gelu(gate(hu_ref[r:r + 16, :]))
            u_ref[r:r + 16, :] = y
            return _vregs(y)
        return [(functools.partial(task, r), 24) for r in range(0, bm, 16)]

    def query_tasks():
        def task(r):
            x = jnp.concatenate([hq_ref[a * bq + r:a * bq + r + 16, :] for a in range(PARTS)], axis=0)
            zs = [_zip(z) for z in _operands(x, "bt")]
            for j, z in enumerate(zs):
                q_ref[j, r // 2:r // 2 + 8, :] = z
            return zs
        return [(functools.partial(task, r), 55) for r in range(0, bq, 16)]

    def key_tasks(base, r0, n, normalise):
        def task(r):
            rows = [base + a * kw + r0 + r for a in range(PARTS)]
            if normalise:
                xs = [_layernorm(_unzip(x_ref[rows16(row), :], normalise)) for row in rows]
                for row, y in zip(rows, xs):
                    ln_ref[rows16(row), :] = y
            else:
                xs = [ln_ref[rows16(row), :] for row in rows]
            zs = [_zip(z) for z in _operands(jnp.concatenate(xs, axis=0), "b")]
            for j, z in enumerate(zs):
                kv_ref[j, pl.ds(pl.multiple_of((r0 + r) // 2, 8), 8), :] = z
            return zs
        return [(functools.partial(task, r), 160) for r in range(0, n, 16)]

    def project(pacer, src, w, dst, cols, untied=0):
        for n, c in enumerate(cols):
            lhs = _rows(src[0:bm // 2, :]) if n < untied else pacer.tie(src[0:bm // 2, :])
            y = pacer.seen(_dot(lhs, _rows(w_ref[w, :, c * 128:(c + 1) * 128])))
            if len(dst.shape) == 3:
                dst[c, 0:bm, :] = y
            else:
                dst[0:bm, c * 128:(c + 1) * 128] = y
        return y

    copies = []

    def fetch(src, dst):
        copies.append(pltpu.make_async_copy(src, dst, sems.at[len(copies)]))
        return copies[-1]

    def fetch_x(b, r0, r1):
        return fetch(x_hbm.at[b, pl.ds(r0, r1 - r0)], x_ref.at[pl.ds(b * Tp + r0, r1 - r0)])

    def start(group):
        for c in group:
            c.start()

    def wait(group):
        for c in group:
            c.wait()

    halves = [(slice(None), pl.ds(n * D, D)) for n in range(2)]
    cuts = (192, 704)

    def fetch_keys(r0, r1):
        return [fetch_x(0, a * kw + r0, min(T, a * kw + r1)) for a in range(1, PARTS)]

    group = [
        [fetch_x(0, 0, bm)],
        [fetch(wup_hbm.at[halves[1]], wup_ref.at[halves[1]])],
        [fetch(wup_hbm.at[halves[0]], wup_ref.at[halves[0]])],
        [fetch(wq_hbm, wq_ref), fetch(wk_hbm, wk_ref)] + fetch_keys(0, cuts[0]),
        [fetch(wv_hbm, wv_ref), fetch(wao_hbm, wao_ref), fetch_x(0, bm, kw)] + fetch_keys(*cuts),
        [fetch(wdn_hbm, wdn_ref), fetch(wm_hbm, wm_ref), fetch(dw_hbm, dw_ref)],
        fetch_keys(cuts[1], kw),
    ]
    assert cuts[0] <= bm and 2 * bm <= kw
    batches = [fetch_x(b, 0, T) for b in range(1, B)]

    @pl.when(step == 0)
    def _():
        start(group[0] + group[1])
        for b in range(B):
            x_ref[b * Tp + T:(b + 1) * Tp, :] = jnp.zeros((Tp - T, D), x_ref.dtype)
        for c in range(nl):
            g_ref[c, bm:bm + HALO, :] = jnp.zeros((HALO, 128), F32)
        wait(group[0])
        start(group[2] + group[3])
        early = _Pacer(zero)

        def weights(lhs, rhs_ref, r0):
            cols = [_dot(early.tie(lhs), rhs_ref[r0:r0 + D, c:c + 128]) for c in range(0, D, 128)]
            return jnp.concatenate([early.seen(y) for y in cols], axis=1)

        _run(block_tasks(0, lambda w: w))
        wait(group[1])
        start(group[4])
        w_ref[W_G] = pltpu.bitcast(wup_ref[:, D:2 * D], U32)
        fence(hg_ref, project(early, xn_ref, W_G, hg_ref, range(nl)))
        wait(group[2])
        w_ref[W_U] = pltpu.bitcast(wup_ref[:, 0:D], U32)
        early.spread(gate_tasks(early.after), nl * (bm // 16), lag=14, parts=2)
        fence(hu_ref, project(early, xn_ref, W_U, hu_ref, range(nl)))
        wait(group[3])
        start(group[5])
        early.spread(u_tasks(early.after) + shift_tasks() + key_tasks(0, 0, cuts[0], early.after),
                     D // 16 + nl * (bm // 16), lag=14, parts=7)
        qk = _dot_nt(early.tie(pltpu.bitcast(wq_ref[...], U32)), wk_ref[...])
        w_ref[W_Q] = _words(qk * (LOG2E * float(D) ** -0.5))
        fence(hq_ref, project(early, xn_ref, W_Q, hq_ref, range(nl)))
        wait(group[4])
        start(group[6])
        early.spread(query_tasks() + block_tasks(bm, early.after) + key_tasks(0, cuts[0], cuts[1] - cuts[0], early.after),
                     3 * nl * (D // 16), lag=14, parts=7)
        vo = weights(pltpu.bitcast(wv_ref[...], U32), wao_ref, 0)
        wait(group[5])
        taps_ref[0:K, :] = dw_ref[...].astype(F32)
        w_ref[W_CONV] = _words(weights(pltpu.bitcast(wdn_ref[...], U32), wm_ref, D))
        w_ref[W_ATT] = _words(weights(_words(vo), wm_ref, 0))
        assert early.idle()
        wait(group[6])
        start(batches)

        @pl.loop(cuts[1] // 64, kw // 64)
        def _(j):
            _run(key_tasks(0, j * 64, 64, lambda w: w))

    for n, copy in enumerate(batches):
        pl.when(step == n * nq + 1)(copy.wait)

    @pl.when(jnp.logical_and(i == 0, step > 0))
    def _():
        @pl.loop(0, kw // 16)
        def _(j):
            _run(key_tasks(block_row(step), j * 16, 16, None))

    pace = _Pacer(zero)
    gates = gate_tasks(pace.after)

    def conv_task(c, r):
        lanes = slice(c * 128, (c + 1) * 128)
        acc, partial = None, []
        for shift in range(8):
            if shift:
                partial.append(acc[0:8])
            taps = [k for k in range(K) if (HALO - pad + k) % 8 == shift]
            lo = HALO - pad + taps[0] + r
            window = g_ref[c, lo:lo + 16 + 8 * (len(taps) - 1), :]
            for n, k in enumerate(taps):
                t = window[8 * n:8 * n + 16] * taps_ref[k:k + 1, lanes]
                acc = t if acc is None else acc + t
        y = _words(u_ref[r:r + 16, lanes] * acc)
        uc_ref[r // 2:r // 2 + 8, lanes] = y
        return partial + _vregs(y)
    convs = [(functools.partial(conv_task, c, r), 32) for r in range(0, bm, 16) for c in range(nl)]
    late = nl * pl.cdiv(pad, 16)
    pace.spread(convs[:-late], PRODUCTS * (kw // 128) * (bq // 16), parts=8)

    peak = None
    for c0 in range(0, kw, 128):
        def product(j):
            return pace.seen(_dot_nt(pace.tie(q_ref[j]), _rows(kv_ref[_a_as_b(j), c0 // 2:(c0 + 128) // 2, :])))
        s = _assemble(product, ((1, 3, 2, 4, 0, 5, 6), (2, 5, 4, 0, 1, 3, 6)), transposed=True)
        tiles = []
        for a in range(PARTS):
            t = s[:, a * 128:(a + 1) * 128]
            col0 = a * kw + c0
            if col0 + 128 > T:
                t = jnp.where(col0 + lax.broadcasted_iota(jnp.int32, t.shape, 1) < T, t, -jnp.inf)
            s_ref[0:bm, col0:col0 + 128] = t
            tiles.append(t)
        for n in range(0, PARTS, 2):
            t = jnp.maximum(tiles[n], tiles[n + 1])
            peak = t if peak is None else jnp.maximum(peak, t)
    fence(s_ref, tiles[-1])
    stat_ref[0, 0:bm, :] = peak
    fence(stat_ref, peak)

    rowmax, rowsum = {}, {}

    def max_task(r):
        rowmax[r] = jnp.broadcast_to(jnp.max(stat_ref[0, r:r + 16, :], axis=-1, keepdims=True), (16, 128))
        return _vregs(rowmax[r])

    def sum_task(r):
        total = None
        for c in range(0, Tp, 128):
            e = jnp.exp2(s_ref[r:r + 16, c:c + 128] - rowmax[r])
            total = e if total is None else total + e
        rowsum[r] = total
        return _vregs(total)

    def scale_task(r):
        scale = jnp.broadcast_to(1.0 / jnp.sum(pace.after(rowsum[r]), axis=-1, keepdims=True), (16, 128))
        stat_ref[0, r:r + 16, :] = rowmax[r]
        stat_ref[1, r:r + 16, :] = scale
        if r + 16 == bm:
            fence(s_ref, scale)
            fence(stat_ref, scale)
        return _vregs(scale)

    span = kw // len(p_refs)

    def prob_tasks(n):
        def task(r, c):
            rows = []
            for a in range(PARTS):
                rr = slice(a * bq + r, a * bq + r + 16)
                m, scale = pace.after(stat_ref[0, rr, :]), stat_ref[1, rr, :]
                cols = [b * kw + n * span + c for b in range(PARTS)]
                rows.append(jnp.concatenate([jnp.exp2(s_ref[rr, col:col + 128] - m) * scale for col in cols], axis=1))
            zs = [_zip(z) for z in _operands(jnp.concatenate(rows, axis=0), "a")]
            for j, z in enumerate(zs):
                p_refs[n][j, r // 2:r // 2 + 8, c:c + 128] = z
            if r + 16 == bq and c + 128 == span:
                fence(p_refs[n], zs[-1])
            return zs[6::7]
        return [(functools.partial(task, r, c), 80) for r in range(0, bq, 16) for c in range(0, span, 128)]

    maxes = [(functools.partial(max_task, r), 3) for r in range(0, bm, 16)]
    stats = maxes[:3]
    for n, r in enumerate(range(0, bm, 16)):
        stats += [(functools.partial(sum_task, r), 70)] + maxes[n + 3:n + 4]
    stats += [(functools.partial(scale_task, r), 4) for r in range(0, bm, 16)]
    probs = prob_tasks(0)
    pace.spread(stats + gates[:1] + convs[-late:] + probs, (3 * nl + nl // 2 - 1) * (bm // 16), lag=10, parts=4)
    fence(hg_ref, project(pace, xn_ref, W_G, hg_ref, range(nl), untied=1))
    assert len(pace.tasks) >= 1 + late + len(probs)
    project(pace, xn_ref, W_Q, hq_ref, range(nl))
    fence(hq_ref, pace.recent[-1])
    project(pace, xn_ref, W_U, hu_ref, range(nl))
    fence(hu_ref, pace.recent[-1])
    assert len(pace.tasks) <= len(probs)
    fence(uc_ref, pace.recent[-1])
    project(pace, uc_ref, W_CONV, yc_ref, range(nl // 2))

    share = Tp // (nq - 1)
    assert share * (nq - 1) == Tp and share % 16 == 0 and 2 * bm <= share * (nq - 3)
    batch = jnp.where(i == 0, step // nq, jnp.minimum(step // nq + 1, B - 1))
    norms = norm_tasks(batch * Tp + jnp.maximum(i - 1, 0) * share, share, pace.after)
    later = (block_tasks(block_row(jnp.minimum(step + 2, B * nq - 1)), None) + norms[8:]
             + _merge(gates[1:], query_tasks()) + shift_tasks())
    cut = int(0.22 * len(later))
    for n, p_ref in enumerate(p_refs):
        if n == 0:
            pace.spread(_merge(prob_tasks(1), later[:cut] + norms[:8]), PRODUCTS * (bq // 16), lag=30, back=3, parts=7)
        else:
            pace.spread(later[cut:], PRODUCTS * (bq // 16), lag=20, back=2, parts=4)
        for j in [a * 7 + b for a in (0, 3, 4, 6, 2, 1, 5) for b in (4, 6, 5, 3, 2, 1, 0)]:
            t = pace.seen(_dot(pace.tie(p_ref[j]), _rows(kv_ref[j, n * span // 2:(n + 1) * span // 2, :])))
            t = t if n == 0 else acc_ref[j] + t
            acc_ref[j] = t
        fence(acc_ref, t)

    def out_task(r):
        o = _assemble(lambda j: acc_ref[j, r:r + 16, :], ((0, 3, 4, 6, 2, 1, 5),) * LEVELS)
        out = []
        for a in range(PARTS):
            y = _zip(o[16 * a:16 * a + 16])
            ob_ref[(a * bq + r) // 2:(a * bq + r) // 2 + 8, :] = y
            out += _vregs(y)
        if r + 16 == bq:
            fence(ob_ref, y)
        return out
    pace.spread([(functools.partial(out_task, r), 1) for r in range(0, bq, 16)], (nl - nl // 2) * (bm // 16), lag=14, parts=8)
    fence(yc_ref, project(pace, uc_ref, W_CONV, yc_ref, range(nl // 2, nl)))
    pace.spread(u_tasks(pace.after), (nl - 1) * (bm // 16), lag=3, parts=2)
    for c in range(nl):
        lanes = slice(c * 128, (c + 1) * 128)
        lhs = ob_ref[0:bm // 2, :]
        ya = _dot(pace.tie(lhs) if c else _rows(lhs), _rows(w_ref[W_ATT, :, lanes]))
        for r in range(0, bm, 16):
            yc = jnp.concatenate([yc_ref[c, pl.ds(r + n, 8, stride=2), :] for n in range(2)], axis=0)
            x = _unzip(x_ref[rows16(block_row(step) + r), lanes])
            o_ref[r:r + 16, lanes] = _rows(_zip(x + (yc + ya[r:r + 16])))
    assert pace.idle()


@jax.jit
def pallas_standalone__conformer_family_branchformer__speech_kernel(
    x: jax.Array,
    w_q: jax.Array,
    w_k: jax.Array,
    w_v: jax.Array,
    w_ao: jax.Array,
    w_up: jax.Array,
    dw: jax.Array,
    w_dn: jax.Array,
    w_merge: jax.Array,
):
    B, T, D = x.shape
    assert x.dtype == BF16 and D == 128 * PARTS and dw.shape[0] < 2 * HALO
    bm, bq = BLOCK, BLOCK // PARTS
    Tp = pl.cdiv(T, 256 * PARTS) * 256 * PARTS
    nq = pl.cdiv(T, bm)
    weights = (w_q, w_k, w_v, w_ao, w_up, dw, w_dn, w_merge)
    return pl.pallas_call(
        _kernel,
        grid=(B * nq,),
        in_specs=[pl.BlockSpec(memory_space=pl.ANY)] * (1 + len(weights)),
        out_specs=pl.BlockSpec((None, bm, D), lambda s: (s // nq, s % nq, 0)),
        out_shape=jax.ShapeDtypeStruct(x.shape, x.dtype),
        scratch_shapes=[pltpu.VMEM((B * Tp, D), x.dtype)] + [pltpu.VMEM(w.shape, w.dtype) for w in weights] + [
            pltpu.SemaphoreType.DMA((len(weights) + 3 * PARTS + B - 1,)),
            pltpu.VMEM((5, D // 2, D), U32),
            pltpu.VMEM((2 * HALO, D), F32),
            pltpu.VMEM((PRODUCTS, Tp // PARTS // 2, 128), U32),
            pltpu.VMEM((bm // 2 + 8, D), U32),
            pltpu.VMEM((PRODUCTS, bq // 2, 128), U32),
            pltpu.VMEM((bm, D), F32),
            pltpu.VMEM((bm // 2 + 8, D), U32),
            pltpu.VMEM((D // 128, bm + 2 * HALO, 128), F32),
            pltpu.VMEM((D // 128, bm + 8, 128), F32),
            pltpu.VMEM((bm + 8, Tp), F32),
            pltpu.VMEM((2, bm + 8, 128), F32),
            pltpu.VMEM((D // 128, bm + 8, 128), F32),
            pltpu.VMEM((bm + 8, D), F32),
            pltpu.VMEM((bm + 8, D), F32),
            pltpu.VMEM((bm + 8, D), F32),
            pltpu.VMEM((PRODUCTS + 1, bq, 128), F32),
            pltpu.VMEM((bm // 2 + 8, D), U32),
            pltpu.VMEM((B * Tp, D), F32),
        ] + [pltpu.VMEM((PRODUCTS + 1, bq // 2, Tp // PARTS // 2), U32)] * 2,
        compiler_params=pltpu.CompilerParams(dimension_semantics=("arbitrary",), vmem_limit_bytes=110 * 2**20),
    )(x, *weights)
```

```python
import functools
import math

import jax
import jax.numpy as jnp
from jax import lax
from jax.experimental import pallas as pl
from jax.experimental.pallas import tpu as pltpu

F32, BF16, U32 = jnp.float32, jnp.bfloat16, jnp.uint32
EPS = 1e-5
LOG2E = 1.4426950408889634
HALO = 16
LEVELS = 2
PARTS = 2 ** LEVELS
PRODUCTS = 7 ** LEVELS
BLOCK = 448
W_Q, W_U, W_G, W_ATT, W_CONV = range(5)


def _layernorm(x):
    c = x - jnp.mean(x, axis=-1, keepdims=True)
    return c * lax.rsqrt(jnp.mean(c * c, axis=-1, keepdims=True) + EPS)


def _gelu(x):
    c0 = math.sqrt(2.0 / math.pi)
    inner = x * (c0 + (c0 * 0.044715) * (x * x))
    half = 0.5 * x
    return half + half * jnp.tanh(inner)


def _dot(a, b):
    return jnp.dot(a, b, preferred_element_type=F32)


def _dot_nt(a, b):
    return lax.dot_general(a, b, (((1,), (1,)), ((), ())), preferred_element_type=F32)


def _rows(words):
    return pltpu.bitcast(words, BF16)


def _words(x):
    return pltpu.bitcast(x.astype(BF16), U32)


def _zip(x):
    return pltpu.pack_elementwise([x[0:8], x[8:16]], packed_dtype=BF16)


def _unzip(x, gate=lambda w: w):
    w = gate(pltpu.bitcast(x, U32))
    return jnp.concatenate([pltpu.unpack_elementwise(w, index=n, packed_dtype=BF16, unpacked_dtype=F32)
                            for n in range(2)], axis=0)


def _vregs(x):
    return [x[r:r + 8, c:c + 128] for r in range(0, x.shape[0], 8) for c in range(0, x.shape[1], 128)]


def _operands(x, kind, level=LEVELS):
    if level == 0:
        return [x]
    r, c = x.shape[0] // 2, x.shape[1] // 2
    x11, x12, x21, x22 = x[:r, :c], x[:r, c:], x[r:, :c], x[r:, c:]
    if kind == "a":
        sums = [x11 + x22, x21 + x22, x11, x22, x11 + x12, x21 - x11, x12 - x22]
    elif kind == "b":
        sums = [x11 + x22, x11, x12 - x22, x21 - x11, x22, x11 + x12, x21 + x22]
    else:
        sums = [x11 + x22, x11, x21 - x22, x12 - x11, x22, x11 + x21, x12 + x22]
    return [z for s in sums for z in _operands(s, kind, level - 1)]


def _a_as_b(j, level=LEVELS):
    if level == 0:
        return 0
    n = 7 ** (level - 1)
    return (0, 6, 1, 4, 5, 3, 2)[j // n] * n + _a_as_b(j % n, level - 1)


_TERMS = (((0, 1), (3, 1), (4, -1), (6, 1)), ((2, 1), (4, 1)), ((1, 1), (3, 1)), ((0, 1), (1, -1), (2, 1), (5, 1)))


def _assemble(product, orders, transposed=False, base=0):
    if not orders:
        return product(base)
    n = 7 ** (len(orders) - 1)
    quads = [None] * 4
    for j in orders[0]:
        m = _assemble(product, orders[1:], transposed, base + j * n)
        for k, terms in enumerate(_TERMS):
            for i, sign in terms:
                if i == j and quads[k] is None:
                    quads[k] = (m, sign)
                elif i == j:
                    t, tsign = quads[k]
                    quads[k] = (t + m, sign) if sign == tsign else (t - m, 1) if tsign > 0 else (m - t, 1)
    assert all(sign > 0 for _, sign in quads)
    c11, c12, c21, c22 = [t for t, _ in quads]
    if transposed:
        c12, c21 = c21, c12
    return jnp.concatenate([jnp.concatenate([c11, c12], axis=1), jnp.concatenate([c21, c22], axis=1)], axis=0)


class _Pacer:
    def __init__(self, zero):
        self.keep = lax.broadcasted_iota(jnp.int32, (8, 128), 0) >= zero
        self.tasks, self.due, self.recent = [], [], []
        self.rate = self.credit = self.slot = self.back = 0

    def idle(self):
        return not self.tasks and not self.due

    def spread(self, tasks, slots, lag=0, back=0, parts=1):
        assert self.idle()
        self.tasks = list(tasks)
        self.rate = sum(c for _, c in tasks) / (slots - lag)
        self.credit = tasks[0][1]
        self.slot, self.end, self.lag, self.back, self.parts = 0, slots - 1, lag, back, parts

    def seen(self, y):
        self.recent.append(y[0:8, 0:128])
        return y

    def after(self, x):
        token = pltpu.bitcast(self.recent[max(0, len(self.recent) - 1 - self.back)], x.dtype)
        return jnp.concatenate([jnp.concatenate(
            [jnp.where(self.keep, x[r:r + 8, c:c + 128], token) for c in range(0, x.shape[1], 128)], axis=1)
            for r in range(0, x.shape[0], 8)], axis=0)

    @staticmethod
    def _any(xs):
        chains = [functools.reduce(lambda a, b: a | b, xs[n::2]) for n in range(min(2, len(xs)))]
        return functools.reduce(lambda a, b: a | b, chains)

    def tie(self, lhs):
        rows = []
        for r in range(0, lhs.shape[0], 8):
            while self.tasks and self.credit >= self.tasks[0][1] * (1 - 1e-6):
                fn, cost = self.tasks.pop(0)
                self.credit -= cost
                out = [pltpu.bitcast(v, U32) for v in fn()]
                n = min(len(out), self.parts)
                for m in range(n):
                    when = min(self.end, self.slot + self.lag + m * cost / self.rate / n)
                    self.due.append((when, self._any(out[m * len(out) // n:(m + 1) * len(out) // n])))
                self.due.sort(key=lambda d: d[0])
            token = None
            while self.due and self.due[0][0] <= self.slot:
                t = self.due.pop(0)[1]
                token = t if token is None else token | t
            self.slot += 1
            self.credit += self.rate
            t = lhs[r:r + 8]
            if token is not None:
                t0 = jnp.where(self.keep, t[:, 0:128], token)
                t = t0 if t.shape[1] == 128 else jnp.concatenate([t0, t[:, 128:]], axis=1)
            rows.append(t)
        return _rows(jnp.concatenate(rows, axis=0))


def _merge(xs, ys):
    keyed = [((n + 0.5) / len(xs), 0, n) for n in range(len(xs))] + [((n + 0.5) / len(ys), 1, n) for n in range(len(ys))]
    return [(xs, ys)[w][n] for _, w, n in sorted(keyed)]


def _run(tasks):
    for fn, _ in tasks:
        fn()


def _kernel(x_hbm, wq_hbm, wk_hbm, wv_hbm, wao_hbm, wup_hbm, dw_hbm, wdn_hbm, wm_hbm, o_ref,
            x_ref, wq_ref, wk_ref, wv_ref, wao_ref, wu_ref, wg_ref, wdn_ref, dw_ref, wm_ref, sems,
            w_ref, taps_ref, kv_ref, xn_ref, q_ref, u_ref, uc_ref, g_ref, gn_ref, s_ref,
            stat_ref, yc_ref, hg_ref, hq_ref, hu_ref, acc_ref, ob_ref, ln_ref, *p_refs):
    step = pl.program_id(0)
    B, T, D = x_hbm.shape
    K = dw_ref.shape[0]
    Tp = s_ref.shape[1]
    bm, bq = BLOCK, BLOCK // PARTS
    kw = Tp // PARTS
    nq = pl.cdiv(T, bm)
    nl = D // 128
    pad = K // 2
    i = step % nq
    zero = pl.multiple_of(jnp.minimum(step, 0) * 8, 8)

    def block_row(n):
        return (n // nq) * Tp + (n % nq) * bm

    def rows16(r):
        return pl.ds(r if isinstance(r, int) else pl.multiple_of(r, 16), 16)

    def fence(ref, val):
        idx = tuple(n - 1 for n in ref.shape[:-2]) + (pl.ds(zero + ref.shape[-2] - 8, 8), pl.ds(0, 128))
        ref[idx] = pltpu.bitcast(val[-8:, -128:], ref.dtype)


    def block_tasks(r0, normalise):
        def task(r):
            y = _zip(_layernorm(_unzip(x_ref[rows16(r0 + r), :], normalise)) if normalise else ln_ref[rows16(r0 + r), :])
            xn_ref[r // 2:r // 2 + 8, :] = y
            if r + 16 == bm:
                fence(xn_ref, y)
            return _vregs(y)
        return [(functools.partial(task, r), 40 if normalise else 4) for r in range(0, bm, 16)]

    def norm_tasks(r0, n, gate):
        def task(r):
            y = _layernorm(_unzip(x_ref[rows16(r0 + r), :], gate))
            ln_ref[rows16(r0 + r), :] = y
            return _vregs(y)
        return [(functools.partial(task, r), 40) for r in range(0, n, 16)]

    def gate_tasks(gate):
        def task(r):
            g = _layernorm(_gelu(gate(hg_ref[r:r + 16, :])))
            for c in range(nl):
                gn_ref[c, r:r + 16, :] = g[:, c * 128:(c + 1) * 128]
                if r < HALO:
                    g_ref[c, HALO + bm + r:HALO + bm + r + 16, :] = g[:, c * 128:(c + 1) * 128]
            if r + 16 == bm:
                fence(gn_ref, g)
            return _vregs(g)
        return [(functools.partial(task, r), 30) for r in range(0, bm, 16)]

    def shift_tasks():
        def move(src, r, dst, n):
            out = []
            for c in range(nl):
                y = src[c, r:r + n, :]
                g_ref[c, dst:dst + n, :] = y
                out += _vregs(y)
            return out
        return ([(functools.partial(move, g_ref, bm, 0, HALO), 8)]
                + [(functools.partial(move, gn_ref, r, HALO + r, 32), 16) for r in range(0, bm, 32)])

    def u_tasks(gate):
        def task(r):
            y = _gelu(gate(hu_ref[r:r + 16, :]))
            u_ref[r:r + 16, :] = y
            return _vregs(y)
        return [(functools.partial(task, r), 24) for r in range(0, bm, 16)]

    def query_tasks():
        def task(r):
            x = jnp.concatenate([hq_ref[a * bq + r:a * bq + r + 16, :] for a in range(PARTS)], axis=0)
            zs = [_zip(z) for z in _operands(x, "bt")]
            for j, z in enumerate(zs):
                q_ref[j, r // 2:r // 2 + 8, :] = z
            return zs
        return [(functools.partial(task, r), 55) for r in range(0, bq, 16)]

    def key_tasks(base, r0, n, normalise):
        def task(r):
            rows = [base + a * kw + r0 + r for a in range(PARTS)]
            if normalise:
                xs = [_layernorm(_unzip(x_ref[rows16(row), :], normalise)) for row in rows]
                for row, y in zip(rows, xs):
                    ln_ref[rows16(row), :] = y
            else:
                xs = [ln_ref[rows16(row), :] for row in rows]
            zs = [_zip(z) for z in _operands(jnp.concatenate(xs, axis=0), "b")]
            for j, z in enumerate(zs):
                kv_ref[j, pl.ds(pl.multiple_of((r0 + r) // 2, 8), 8), :] = z
            return zs
        return [(functools.partial(task, r), 160) for r in range(0, n, 16)]

    def project(pacer, src, w, dst, cols, untied=0):
        for n, c in enumerate(cols):
            lhs = _rows(src[0:bm // 2, :]) if n < untied else pacer.tie(src[0:bm // 2, :])
            y = pacer.seen(_dot(lhs, _rows(w_ref[w, :, c * 128:(c + 1) * 128])))
            if len(dst.shape) == 3:
                dst[c, 0:bm, :] = y
            else:
                dst[0:bm, c * 128:(c + 1) * 128] = y
        return y

    copies = []

    def fetch(src, dst):
        copies.append(pltpu.make_async_copy(src, dst, sems.at[len(copies)]))
        return copies[-1]

    def fetch_x(b, r0, r1):
        return fetch(x_hbm.at[b, pl.ds(r0, r1 - r0)], x_ref.at[pl.ds(b * Tp + r0, r1 - r0)])

    def start(group):
        for c in group:
            c.start()

    def wait(group):
        for c in group:
            c.wait()

    cuts = (192, 704)

    def fetch_keys(r0, r1):
        return [fetch_x(0, a * kw + r0, min(T, a * kw + r1)) for a in range(1, PARTS)]

    group = [
        [fetch_x(0, 0, bm)],
        [fetch(wup_hbm.at[:, pl.ds(D, D)], wg_ref)],
        [fetch(wup_hbm.at[:, pl.ds(0, D)], wu_ref)],
        [fetch(wq_hbm, wq_ref), fetch(wk_hbm, wk_ref)] + fetch_keys(0, cuts[0]),
        [fetch(wv_hbm, wv_ref), fetch(wao_hbm, wao_ref), fetch_x(0, bm, kw)] + fetch_keys(*cuts),
        [fetch(wdn_hbm, wdn_ref), fetch(wm_hbm, wm_ref), fetch(dw_hbm, dw_ref)],
        fetch_keys(cuts[1], kw),
    ]
    assert cuts[0] <= bm and 2 * bm <= kw
    batches = [fetch_x(b, 0, T) for b in range(1, B)]

    @pl.when(step == 0)
    def _():
        start(group[0] + group[1])
        for b in range(B):
            x_ref[b * Tp + T:(b + 1) * Tp, :] = jnp.zeros((Tp - T, D), x_ref.dtype)
        for c in range(nl):
            g_ref[c, bm:bm + HALO, :] = jnp.zeros((HALO, 128), F32)
        wait(group[0])
        start(group[2] + group[3])
        early = _Pacer(zero)

        def weights(lhs, rhs_ref, r0):
            cols = [_dot(early.tie(lhs), rhs_ref[r0:r0 + D, c:c + 128]) for c in range(0, D, 128)]
            return jnp.concatenate([early.seen(y) for y in cols], axis=1)

        _run(block_tasks(0, lambda w: w))
        wait(group[1])
        start(group[4])
        w_ref[W_G] = pltpu.bitcast(wg_ref[...], U32)
        fence(hg_ref, project(early, xn_ref, W_G, hg_ref, range(nl)))
        wait(group[2])
        w_ref[W_U] = pltpu.bitcast(wu_ref[...], U32)
        early.spread(gate_tasks(early.after), nl * (bm // 16), lag=14, parts=2)
        fence(hu_ref, project(early, xn_ref, W_U, hu_ref, range(nl)))
        wait(group[3])
        start(group[5])
        early.spread(u_tasks(early.after) + shift_tasks() + key_tasks(0, 0, cuts[0], early.after),
                     D // 16 + nl * (bm // 16), lag=14, parts=7)
        qk = _dot_nt(early.tie(pltpu.bitcast(wq_ref[...], U32)), wk_ref[...])
        w_ref[W_Q] = _words(qk * (LOG2E * float(D) ** -0.5))
        fence(hq_ref, project(early, xn_ref, W_Q, hq_ref, range(nl)))
        wait(group[4])
        start(group[6])
        early.spread(query_tasks() + block_tasks(bm, early.after) + key_tasks(0, cuts[0], cuts[1] - cuts[0], early.after),
                     3 * nl * (D // 16), lag=14, parts=7)
        vo = weights(pltpu.bitcast(wv_ref[...], U32), wao_ref, 0)
        wait(group[5])
        taps_ref[0:K, :] = dw_ref[...].astype(F32)
        w_ref[W_CONV] = _words(weights(pltpu.bitcast(wdn_ref[...], U32), wm_ref, D))
        w_ref[W_ATT] = _words(weights(_words(vo), wm_ref, 0))
        assert early.idle()
        wait(group[6])
        start(batches)

        @pl.loop(cuts[1] // 64, kw // 64)
        def _(j):
            _run(key_tasks(0, j * 64, 64, lambda w: w))

    for n, copy in enumerate(batches):
        pl.when(step == n * nq + 1)(copy.wait)

    @pl.when(jnp.logical_and(i == 0, step > 0))
    def _():
        @pl.loop(0, kw // 16)
        def _(j):
            _run(key_tasks(block_row(step), j * 16, 16, None))

    pace = _Pacer(zero)
    gates = gate_tasks(pace.after)

    def conv_task(c, r):
        lanes = slice(c * 128, (c + 1) * 128)
        acc, partial = None, []
        for shift in range(8):
            if shift:
                partial.append(acc[0:8])
            taps = [k for k in range(K) if (HALO - pad + k) % 8 == shift]
            lo = HALO - pad + taps[0] + r
            window = g_ref[c, lo:lo + 16 + 8 * (len(taps) - 1), :]
            for n, k in enumerate(taps):
                t = window[8 * n:8 * n + 16] * taps_ref[k:k + 1, lanes]
                acc = t if acc is None else acc + t
        y = _words(u_ref[r:r + 16, lanes] * acc)
        uc_ref[r // 2:r // 2 + 8, lanes] = y
        return partial + _vregs(y)
    convs = [(functools.partial(conv_task, c, r), 32) for r in range(0, bm, 16) for c in range(nl)]
    late = nl * pl.cdiv(pad, 16)
    pace.spread(convs[:-late], PRODUCTS * (kw // 128) * (bq // 16), parts=8)

    peak = None
    for c0 in range(0, kw, 128):
        def product(j):
            return pace.seen(_dot_nt(pace.tie(q_ref[j]), _rows(kv_ref[_a_as_b(j), c0 // 2:(c0 + 128) // 2, :])))
        s = _assemble(product, ((1, 3, 2, 4, 0, 5, 6), (2, 5, 4, 0, 1, 3, 6)), transposed=True)
        tiles = []
        for a in range(PARTS):
            t = s[:, a * 128:(a + 1) * 128]
            col0 = a * kw + c0
            if col0 + 128 > T:
                t = jnp.where(col0 + lax.broadcasted_iota(jnp.int32, t.shape, 1) < T, t, -jnp.inf)
            s_ref[0:bm, col0:col0 + 128] = t
            tiles.append(t)
        for n in range(0, PARTS, 2):
            t = jnp.maximum(tiles[n], tiles[n + 1])
            peak = t if peak is None else jnp.maximum(peak, t)
    fence(s_ref, tiles[-1])
    stat_ref[0, 0:bm, :] = peak
    fence(stat_ref, peak)

    rowmax, rowsum = {}, {}

    def max_task(r):
        rowmax[r] = jnp.broadcast_to(jnp.max(stat_ref[0, r:r + 16, :], axis=-1, keepdims=True), (16, 128))
        return _vregs(rowmax[r])

    def sum_task(r):
        total = None
        for c in range(0, Tp, 128):
            e = jnp.exp2(s_ref[r:r + 16, c:c + 128] - rowmax[r])
            total = e if total is None else total + e
        rowsum[r] = total
        return _vregs(total)

    def scale_task(r):
        scale = jnp.broadcast_to(1.0 / jnp.sum(pace.after(rowsum[r]), axis=-1, keepdims=True), (16, 128))
        stat_ref[0, r:r + 16, :] = rowmax[r]
        stat_ref[1, r:r + 16, :] = scale
        if r + 16 == bm:
            fence(s_ref, scale)
            fence(stat_ref, scale)
        return _vregs(scale)

    span = kw // len(p_refs)

    def prob_tasks(n):
        def task(r, c):
            rows = []
            for a in range(PARTS):
                rr = slice(a * bq + r, a * bq + r + 16)
                m, scale = pace.after(stat_ref[0, rr, :]), stat_ref[1, rr, :]
                cols = [b * kw + n * span + c for b in range(PARTS)]
                rows.append(jnp.concatenate([jnp.exp2(s_ref[rr, col:col + 128] - m) * scale for col in cols], axis=1))
            zs = [_zip(z) for z in _operands(jnp.concatenate(rows, axis=0), "a")]
            for j, z in enumerate(zs):
                p_refs[n][j, r // 2:r // 2 + 8, c:c + 128] = z
            if r + 16 == bq and c + 128 == span:
                fence(p_refs[n], zs[-1])
            return zs[6::7]
        return [(functools.partial(task, r, c), 80) for r in range(0, bq, 16) for c in range(0, span, 128)]

    maxes = [(functools.partial(max_task, r), 3) for r in range(0, bm, 16)]
    stats = maxes[:3]
    for n, r in enumerate(range(0, bm, 16)):
        stats += [(functools.partial(sum_task, r), 70)] + maxes[n + 3:n + 4]
    stats += [(functools.partial(scale_task, r), 4) for r in range(0, bm, 16)]
    probs = prob_tasks(0)
    pace.spread(stats + gates[:1] + convs[-late:] + probs, (3 * nl + nl // 2 - 1) * (bm // 16), lag=10, parts=4)
    fence(hg_ref, project(pace, xn_ref, W_G, hg_ref, range(nl), untied=1))
    assert len(pace.tasks) >= 1 + late + len(probs)
    project(pace, xn_ref, W_Q, hq_ref, range(nl))
    fence(hq_ref, pace.recent[-1])
    project(pace, xn_ref, W_U, hu_ref, range(nl))
    fence(hu_ref, pace.recent[-1])
    assert len(pace.tasks) <= len(probs)
    fence(uc_ref, pace.recent[-1])
    project(pace, uc_ref, W_CONV, yc_ref, range(nl // 2))

    share = Tp // (nq - 1)
    assert share * (nq - 1) == Tp and share % 16 == 0 and 2 * bm <= share * (nq - 3)
    batch = jnp.where(i == 0, step // nq, jnp.minimum(step // nq + 1, B - 1))
    norms = norm_tasks(batch * Tp + jnp.maximum(i - 1, 0) * share, share, pace.after)
    later = (block_tasks(block_row(jnp.minimum(step + 2, B * nq - 1)), None) + norms[8:]
             + _merge(gates[1:], query_tasks()) + shift_tasks())
    cut = int(0.22 * len(later))
    for n, p_ref in enumerate(p_refs):
        if n == 0:
            pace.spread(_merge(prob_tasks(1), later[:cut] + norms[:8]), PRODUCTS * (bq // 16), lag=30, back=3, parts=7)
        else:
            pace.spread(later[cut:], PRODUCTS * (bq // 16), lag=20, back=2, parts=4)
        for j in [a * 7 + b for a in (0, 3, 4, 6, 2, 1, 5) for b in (4, 6, 5, 3, 2, 1, 0)]:
            t = pace.seen(_dot(pace.tie(p_ref[j]), _rows(kv_ref[j, n * span // 2:(n + 1) * span // 2, :])))
            t = t if n == 0 else acc_ref[j] + t
            acc_ref[j] = t
        fence(acc_ref, t)

    def out_task(r):
        o = _assemble(lambda j: acc_ref[j, r:r + 16, :], ((0, 3, 4, 6, 2, 1, 5),) * LEVELS)
        out = []
        for a in range(PARTS):
            y = _zip(o[16 * a:16 * a + 16])
            ob_ref[(a * bq + r) // 2:(a * bq + r) // 2 + 8, :] = y
            out += _vregs(y)
        if r + 16 == bq:
            fence(ob_ref, y)
        return out
    pace.spread([(functools.partial(out_task, r), 1) for r in range(0, bq, 16)], (nl - nl // 2) * (bm // 16), lag=14, parts=8)
    fence(yc_ref, project(pace, uc_ref, W_CONV, yc_ref, range(nl // 2, nl)))
    pace.spread(u_tasks(pace.after), (nl - 1) * (bm // 16), lag=3, parts=2)
    for c in range(nl):
        lanes = slice(c * 128, (c + 1) * 128)
        lhs = ob_ref[0:bm // 2, :]
        ya = _dot(pace.tie(lhs) if c else _rows(lhs), _rows(w_ref[W_ATT, :, lanes]))
        for r in range(0, bm, 16):
            yc = jnp.concatenate([yc_ref[c, pl.ds(r + n, 8, stride=2), :] for n in range(2)], axis=0)
            x = _unzip(x_ref[rows16(block_row(step) + r), lanes])
            o_ref[r:r + 16, lanes] = _rows(_zip(x + (yc + ya[r:r + 16])))
    assert pace.idle()


@jax.jit
def pallas_standalone__conformer_family_branchformer__speech_kernel(
    x: jax.Array,
    w_q: jax.Array,
    w_k: jax.Array,
    w_v: jax.Array,
    w_ao: jax.Array,
    w_up: jax.Array,
    dw: jax.Array,
    w_dn: jax.Array,
    w_merge: jax.Array,
):
    B, T, D = x.shape
    weights = (w_q, w_k, w_v, w_ao, w_up, dw, w_dn, w_merge)
    assert all(a.dtype == BF16 for a in (x, *weights)) and D == 128 * PARTS and dw.shape[0] < 2 * HALO
    bm, bq = BLOCK, BLOCK // PARTS
    Tp = pl.cdiv(T, 256 * PARTS) * 256 * PARTS
    nq = pl.cdiv(T, bm)
    return pl.pallas_call(
        _kernel,
        grid=(B * nq,),
        in_specs=[pl.BlockSpec(memory_space=pl.ANY)] * (1 + len(weights)),
        out_specs=pl.BlockSpec((None, bm, D), lambda s: (s // nq, s % nq, 0)),
        out_shape=jax.ShapeDtypeStruct(x.shape, x.dtype),
        scratch_shapes=[pltpu.VMEM((B * Tp, D), BF16)] + [pltpu.VMEM((D, D), BF16)] * 7 + [
            pltpu.VMEM(dw.shape, BF16),
            pltpu.VMEM(w_merge.shape, BF16),
            pltpu.SemaphoreType.DMA((len(weights) + 3 * PARTS + B - 1,)),
            pltpu.VMEM((5, D // 2, D), U32),
            pltpu.VMEM((2 * HALO, D), F32),
            pltpu.VMEM((PRODUCTS, Tp // PARTS // 2, 128), U32),
            pltpu.VMEM((bm // 2 + 8, D), U32),
            pltpu.VMEM((PRODUCTS, bq // 2, 128), U32),
            pltpu.VMEM((bm, D), F32),
            pltpu.VMEM((bm // 2 + 8, D), U32),
            pltpu.VMEM((D // 128, bm + 2 * HALO, 128), F32),
            pltpu.VMEM((D // 128, bm + 8, 128), F32),
            pltpu.VMEM((bm + 8, Tp), F32),
            pltpu.VMEM((2, bm + 8, 128), F32),
            pltpu.VMEM((D // 128, bm + 8, 128), F32),
            pltpu.VMEM((bm + 8, D), F32),
            pltpu.VMEM((bm + 8, D), F32),
            pltpu.VMEM((bm + 8, D), F32),
            pltpu.VMEM((PRODUCTS + 1, bq, 128), F32),
            pltpu.VMEM((bm // 2 + 8, D), U32),
            pltpu.VMEM((B * Tp, D), F32),
        ] + [pltpu.VMEM((PRODUCTS + 1, bq // 2, Tp // PARTS // 2), U32)] * 2,
        compiler_params=pltpu.CompilerParams(dimension_semantics=("arbitrary",), vmem_limit_bytes=110 * 2**20),
    )(x, *weights)
```

```python
import functools
import math

import jax
import jax.numpy as jnp
from jax import lax
from jax.experimental import pallas as pl
from jax.experimental.pallas import tpu as pltpu

F32, BF16, U32 = jnp.float32, jnp.bfloat16, jnp.uint32
EPS = 1e-5
LOG2E = 1.4426950408889634
HALO = 16
LEVELS = 2
PARTS = 2 ** LEVELS
PRODUCTS = 7 ** LEVELS
BLOCK = 448
W_Q, W_U, W_G, W_ATT, W_CONV = range(5)


def _layernorm(x):
    c = x - jnp.mean(x, axis=-1, keepdims=True)
    return c * lax.rsqrt(jnp.mean(c * c, axis=-1, keepdims=True) + EPS)


def _gelu(x):
    c0 = math.sqrt(2.0 / math.pi)
    inner = x * (c0 + (c0 * 0.044715) * (x * x))
    half = 0.5 * x
    return half + half * jnp.tanh(inner)


def _dot(a, b):
    return jnp.dot(a, b, preferred_element_type=F32)


def _dot_nt(a, b):
    return lax.dot_general(a, b, (((1,), (1,)), ((), ())), preferred_element_type=F32)


def _rows(words):
    return pltpu.bitcast(words, BF16)


def _words(x):
    return pltpu.bitcast(x.astype(BF16), U32)


def _zip(x):
    return pltpu.pack_elementwise([x[0:8], x[8:16]], packed_dtype=BF16)


def _unzip(x, gate=lambda w: w):
    w = gate(pltpu.bitcast(x, U32))
    return jnp.concatenate([pltpu.unpack_elementwise(w, index=n, packed_dtype=BF16, unpacked_dtype=F32)
                            for n in range(2)], axis=0)


def _vregs(x):
    return [x[r:r + 8, c:c + 128] for r in range(0, x.shape[0], 8) for c in range(0, x.shape[1], 128)]


def _operands(x, kind, level=LEVELS):
    if level == 0:
        return [x]
    r, c = x.shape[0] // 2, x.shape[1] // 2
    x11, x12, x21, x22 = x[:r, :c], x[:r, c:], x[r:, :c], x[r:, c:]
    if kind == "a":
        sums = [x11 + x22, x21 + x22, x11, x22, x11 + x12, x21 - x11, x12 - x22]
    elif kind == "b":
        sums = [x11 + x22, x11, x12 - x22, x21 - x11, x22, x11 + x12, x21 + x22]
    else:
        sums = [x11 + x22, x11, x21 - x22, x12 - x11, x22, x11 + x21, x12 + x22]
    return [z for s in sums for z in _operands(s, kind, level - 1)]


def _a_as_b(j, level=LEVELS):
    if level == 0:
        return 0
    n = 7 ** (level - 1)
    return (0, 6, 1, 4, 5, 3, 2)[j // n] * n + _a_as_b(j % n, level - 1)


_TERMS = (((0, 1), (3, 1), (4, -1), (6, 1)), ((2, 1), (4, 1)), ((1, 1), (3, 1)), ((0, 1), (1, -1), (2, 1), (5, 1)))


def _assemble(product, orders, transposed=False, base=0):
    if not orders:
        return product(base)
    n = 7 ** (len(orders) - 1)
    quads = [None] * 4
    for j in orders[0]:
        m = _assemble(product, orders[1:], transposed, base + j * n)
        for k, terms in enumerate(_TERMS):
            for i, sign in terms:
                if i == j and quads[k] is None:
                    quads[k] = (m, sign)
                elif i == j:
                    t, tsign = quads[k]
                    quads[k] = (t + m, sign) if sign == tsign else (t - m, 1) if tsign > 0 else (m - t, 1)
    assert all(sign > 0 for _, sign in quads)
    c11, c12, c21, c22 = [t for t, _ in quads]
    if transposed:
        c12, c21 = c21, c12
    return jnp.concatenate([jnp.concatenate([c11, c12], axis=1), jnp.concatenate([c21, c22], axis=1)], axis=0)


class _Pacer:
    def __init__(self, zero):
        self.keep = lax.broadcasted_iota(jnp.int32, (8, 128), 0) >= zero
        self.tasks, self.due, self.recent = [], [], []
        self.rate = self.credit = self.slot = self.back = 0

    def idle(self):
        return not self.tasks and not self.due

    def spread(self, tasks, slots, lag=0, back=0, parts=1):
        assert self.idle()
        self.tasks = list(tasks)
        self.rate = sum(c for _, c in tasks) / (slots - lag)
        self.credit = tasks[0][1]
        self.slot, self.end, self.lag, self.back, self.parts = 0, slots - 1, lag, back, parts

    def seen(self, y):
        self.recent.append(y[0:8, 0:128])
        return y

    def after(self, x):
        token = pltpu.bitcast(self.recent[max(0, len(self.recent) - 1 - self.back)], x.dtype)
        return jnp.concatenate([jnp.concatenate(
            [jnp.where(self.keep, x[r:r + 8, c:c + 128], token) for c in range(0, x.shape[1], 128)], axis=1)
            for r in range(0, x.shape[0], 8)], axis=0)

    @staticmethod
    def _any(xs):
        chains = [functools.reduce(lambda a, b: a | b, xs[n::2]) for n in range(min(2, len(xs)))]
        return functools.reduce(lambda a, b: a | b, chains)

    def tie(self, lhs):
        rows = []
        for r in range(0, lhs.shape[0], 8):
            while self.tasks and self.credit >= self.tasks[0][1] * (1 - 1e-6):
                fn, cost = self.tasks.pop(0)
                self.credit -= cost
                out = [pltpu.bitcast(v, U32) for v in fn()]
                n = min(len(out), self.parts)
                for m in range(n):
                    when = min(self.end, self.slot + self.lag + m * cost / self.rate / n)
                    self.due.append((when, self._any(out[m * len(out) // n:(m + 1) * len(out) // n])))
                self.due.sort(key=lambda d: d[0])
            token = None
            while self.due and self.due[0][0] <= self.slot:
                t = self.due.pop(0)[1]
                token = t if token is None else token | t
            self.slot += 1
            self.credit += self.rate
            t = lhs[r:r + 8]
            if token is not None:
                t0 = jnp.where(self.keep, t[:, 0:128], token)
                t = t0 if t.shape[1] == 128 else jnp.concatenate([t0, t[:, 128:]], axis=1)
            rows.append(t)
        return _rows(jnp.concatenate(rows, axis=0))


def _merge(xs, ys):
    keyed = [((n + 0.5) / len(xs), 0, n) for n in range(len(xs))] + [((n + 0.5) / len(ys), 1, n) for n in range(len(ys))]
    return [(xs, ys)[w][n] for _, w, n in sorted(keyed)]


def _run(tasks):
    for fn, _ in tasks:
        fn()


def _kernel(x_hbm, wq_hbm, wk_hbm, wv_hbm, wao_hbm, wup_hbm, dw_hbm, wdn_hbm, wm_hbm, o_ref,
            x_ref, wq_ref, wk_ref, wv_ref, wao_ref, wu_ref, wg_ref, wdn_ref, dw_ref, wm_ref, sems,
            w_ref, taps_ref, kv_ref, xn_ref, q_ref, u_ref, uc_ref, g_ref, gn_ref, s_ref,
            stat_ref, yc_ref, hg_ref, hq_ref, hu_ref, acc_ref, ob_ref, ln_ref, *p_refs):
    step = pl.program_id(0)
    B, T, D = x_hbm.shape
    K = dw_ref.shape[0]
    Tp = s_ref.shape[1]
    bm, bq = BLOCK, BLOCK // PARTS
    kw = Tp // PARTS
    nq = pl.cdiv(T, bm)
    nl = D // 128
    pad = K // 2
    i = step % nq
    zero = pl.multiple_of(jnp.minimum(step, 0) * 8, 8)

    def block_row(n):
        return (n // nq) * Tp + (n % nq) * bm

    def rows16(r):
        return pl.ds(r if isinstance(r, int) else pl.multiple_of(r, 16), 16)

    def fence(ref, val):
        idx = tuple(n - 1 for n in ref.shape[:-2]) + (pl.ds(zero + ref.shape[-2] - 8, 8), pl.ds(0, 128))
        ref[idx] = pltpu.bitcast(val[-8:, -128:], ref.dtype)


    def block_tasks(r0, normalise):
        def task(r):
            y = _zip(_layernorm(_unzip(x_ref[rows16(r0 + r), :], normalise)) if normalise else ln_ref[rows16(r0 + r), :])
            xn_ref[r // 2:r // 2 + 8, :] = y
            if r + 16 == bm:
                fence(xn_ref, y)
            return _vregs(y)
        return [(functools.partial(task, r), 40 if normalise else 4) for r in range(0, bm, 16)]

    def norm_tasks(r0, n, gate):
        def task(r):
            y = _layernorm(_unzip(x_ref[rows16(r0 + r), :], gate))
            ln_ref[rows16(r0 + r), :] = y
            return _vregs(y)
        return [(functools.partial(task, r), 40) for r in range(0, n, 16)]

    def gate_tasks(gate):
        def task(r):
            g = _layernorm(_gelu(gate(hg_ref[r:r + 16, :])))
            for c in range(nl):
                gn_ref[c, r:r + 16, :] = g[:, c * 128:(c + 1) * 128]
                if r < HALO:
                    g_ref[c, HALO + bm + r:HALO + bm + r + 16, :] = g[:, c * 128:(c + 1) * 128]
            if r + 16 == bm:
                fence(gn_ref, g)
            return _vregs(g)
        return [(functools.partial(task, r), 30) for r in range(0, bm, 16)]

    def shift_tasks():
        def move(src, r, dst, n):
            out = []
            for c in range(nl):
                y = src[c, r:r + n, :]
                g_ref[c, dst:dst + n, :] = y
                out += _vregs(y)
            return out
        return ([(functools.partial(move, g_ref, bm, 0, HALO), 8)]
                + [(functools.partial(move, gn_ref, r, HALO + r, 32), 16) for r in range(0, bm, 32)])

    def u_tasks(gate):
        def task(r):
            y = _gelu(gate(hu_ref[r:r + 16, :]))
            u_ref[r:r + 16, :] = y
            return _vregs(y)
        return [(functools.partial(task, r), 24) for r in range(0, bm, 16)]

    def query_tasks():
        def task(r):
            x = jnp.concatenate([hq_ref[a * bq + r:a * bq + r + 16, :] for a in range(PARTS)], axis=0)
            zs = [_zip(z) for z in _operands(x, "bt")]
            for j, z in enumerate(zs):
                q_ref[j, r // 2:r // 2 + 8, :] = z
            return zs
        return [(functools.partial(task, r), 40) for r in range(0, bq, 16)]

    def key_tasks(base, r0, n, normalise):
        def task(r):
            rows = [base + a * kw + r0 + r for a in range(PARTS)]
            if normalise:
                xs = [_layernorm(_unzip(x_ref[rows16(row), :], normalise)) for row in rows]
                for row, y in zip(rows, xs):
                    ln_ref[rows16(row), :] = y
            else:
                xs = [ln_ref[rows16(row), :] for row in rows]
            zs = [_zip(z) for z in _operands(jnp.concatenate(xs, axis=0), "b")]
            for j, z in enumerate(zs):
                kv_ref[j, pl.ds(pl.multiple_of((r0 + r) // 2, 8), 8), :] = z
            return zs
        return [(functools.partial(task, r), 160) for r in range(0, n, 16)]

    def project(pacer, src, w, dst, cols, untied=0):
        for n, c in enumerate(cols):
            lhs = _rows(src[0:bm // 2, :]) if n < untied else pacer.tie(src[0:bm // 2, :])
            y = pacer.seen(_dot(lhs, _rows(w_ref[w, :, c * 128:(c + 1) * 128])))
            if len(dst.shape) == 3:
                dst[c, 0:bm, :] = y
            else:
                dst[0:bm, c * 128:(c + 1) * 128] = y
        return y

    copies = []

    def fetch(src, dst):
        copies.append(pltpu.make_async_copy(src, dst, sems.at[len(copies)]))
        return copies[-1]

    def fetch_x(b, r0, r1):
        return fetch(x_hbm.at[b, pl.ds(r0, r1 - r0)], x_ref.at[pl.ds(b * Tp + r0, r1 - r0)])

    def start(group):
        for c in group:
            c.start()

    def wait(group):
        for c in group:
            c.wait()

    cuts = (192, 704)

    def fetch_keys(r0, r1):
        return [fetch_x(0, a * kw + r0, min(T, a * kw + r1)) for a in range(1, PARTS)]

    group = [
        [fetch_x(0, 0, bm)],
        [fetch(wup_hbm.at[:, pl.ds(D, D)], wg_ref)],
        [fetch(wup_hbm.at[:, pl.ds(0, D)], wu_ref)],
        [fetch(wq_hbm, wq_ref), fetch(wk_hbm, wk_ref)] + fetch_keys(0, cuts[0]),
        [fetch(wv_hbm, wv_ref), fetch(wao_hbm, wao_ref), fetch_x(0, bm, kw)] + fetch_keys(*cuts),
        [fetch(wdn_hbm, wdn_ref), fetch(wm_hbm, wm_ref), fetch(dw_hbm, dw_ref)],
        fetch_keys(cuts[1], kw),
    ]
    assert cuts[0] <= bm and 2 * bm <= kw
    batches = [fetch_x(b, 0, T) for b in range(1, B)]

    @pl.when(step == 0)
    def _():
        start(group[0] + group[1])
        for b in range(B):
            x_ref[b * Tp + T:(b + 1) * Tp, :] = jnp.zeros((Tp - T, D), x_ref.dtype)
        for c in range(nl):
            g_ref[c, bm:bm + HALO, :] = jnp.zeros((HALO, 128), F32)
        wait(group[0])
        start(group[2] + group[3])
        early = _Pacer(zero)

        def weights(lhs, rhs_ref, r0):
            cols = [_dot(early.tie(lhs), rhs_ref[r0:r0 + D, c:c + 128]) for c in range(0, D, 128)]
            return jnp.concatenate([early.seen(y) for y in cols], axis=1)

        _run(block_tasks(0, lambda w: w))
        wait(group[1])
        start(group[4])
        w_ref[W_G] = pltpu.bitcast(wg_ref[...], U32)
        fence(hg_ref, project(early, xn_ref, W_G, hg_ref, range(nl)))
        wait(group[2])
        w_ref[W_U] = pltpu.bitcast(wu_ref[...], U32)
        early.spread(gate_tasks(early.after), nl * (bm // 16), lag=14, parts=2)
        fence(hu_ref, project(early, xn_ref, W_U, hu_ref, range(nl)))
        wait(group[3])
        start(group[5])
        early.spread(u_tasks(early.after) + shift_tasks() + key_tasks(0, 0, cuts[0], early.after),
                     D // 16 + nl * (bm // 16), lag=14, parts=7)
        qk = _dot_nt(early.tie(pltpu.bitcast(wq_ref[...], U32)), wk_ref[...])
        w_ref[W_Q] = _words(qk * (LOG2E * float(D) ** -0.5))
        fence(hq_ref, project(early, xn_ref, W_Q, hq_ref, range(nl)))
        wait(group[4])
        start(group[6])
        early.spread(query_tasks() + block_tasks(bm, early.after) + key_tasks(0, cuts[0], cuts[1] - cuts[0], early.after),
                     3 * nl * (D // 16), lag=14, parts=7)
        vo = weights(pltpu.bitcast(wv_ref[...], U32), wao_ref, 0)
        wait(group[5])
        taps_ref[0:K, :] = dw_ref[...].astype(F32)
        w_ref[W_CONV] = _words(weights(pltpu.bitcast(wdn_ref[...], U32), wm_ref, D))
        w_ref[W_ATT] = _words(weights(_words(vo), wm_ref, 0))
        assert early.idle()
        wait(group[6])
        start(batches)

        @pl.loop(cuts[1] // 64, kw // 64)
        def _(j):
            _run(key_tasks(0, j * 64, 64, lambda w: w))

    for n, copy in enumerate(batches):
        pl.when(step == n * nq + 1)(copy.wait)

    @pl.when(jnp.logical_and(i == 0, step > 0))
    def _():
        @pl.loop(0, kw // 16)
        def _(j):
            _run(key_tasks(block_row(step), j * 16, 16, None))

    pace = _Pacer(zero)
    gates = gate_tasks(pace.after)

    def conv_task(c, r):
        lanes = slice(c * 128, (c + 1) * 128)
        acc, partial = None, []
        for shift in range(8):
            if shift:
                partial.append(acc[0:8])
            taps = [k for k in range(K) if (HALO - pad + k) % 8 == shift]
            lo = HALO - pad + taps[0] + r
            window = g_ref[c, lo:lo + 16 + 8 * (len(taps) - 1), :]
            for n, k in enumerate(taps):
                t = window[8 * n:8 * n + 16] * taps_ref[k:k + 1, lanes]
                acc = t if acc is None else acc + t
        y = _words(u_ref[r:r + 16, lanes] * acc)
        uc_ref[r // 2:r // 2 + 8, lanes] = y
        return partial + _vregs(y)
    convs = [(functools.partial(conv_task, c, r), 48) for r in range(0, bm, 16) for c in range(nl)]
    late = nl * pl.cdiv(pad, 16)
    pace.spread(convs[:-late], PRODUCTS * (kw // 128) * (bq // 16), parts=8)

    peak = None
    for c0 in range(0, kw, 128):
        def product(j):
            return pace.seen(_dot_nt(pace.tie(q_ref[j]), _rows(kv_ref[_a_as_b(j), c0 // 2:(c0 + 128) // 2, :])))
        s = _assemble(product, ((1, 3, 2, 4, 0, 5, 6), (2, 5, 4, 1, 0, 3, 6)), transposed=True)
        tiles = []
        for a in range(PARTS):
            t = s[:, a * 128:(a + 1) * 128]
            col0 = a * kw + c0
            if col0 + 128 > T:
                t = jnp.where(col0 + lax.broadcasted_iota(jnp.int32, t.shape, 1) < T, t, -jnp.inf)
            s_ref[0:bm, col0:col0 + 128] = t
            tiles.append(t)
        for n in range(0, PARTS, 2):
            t = jnp.maximum(tiles[n], tiles[n + 1])
            peak = t if peak is None else jnp.maximum(peak, t)
    fence(s_ref, tiles[-1])
    stat_ref[0, 0:bm, :] = peak
    fence(stat_ref, peak)

    rowmax, rowsum = {}, {}

    def max_task(r):
        rowmax[r] = jnp.broadcast_to(jnp.max(stat_ref[0, r:r + 16, :], axis=-1, keepdims=True), (16, 128))
        return _vregs(rowmax[r])

    def sum_task(r):
        total = None
        for c in range(0, Tp, 128):
            e = jnp.exp2(s_ref[r:r + 16, c:c + 128] - rowmax[r])
            total = e if total is None else total + e
        rowsum[r] = total
        return _vregs(total)

    def scale_task(r):
        scale = jnp.broadcast_to(1.0 / jnp.sum(pace.after(rowsum[r]), axis=-1, keepdims=True), (16, 128))
        stat_ref[0, r:r + 16, :] = rowmax[r]
        stat_ref[1, r:r + 16, :] = scale
        if r + 16 == bm:
            fence(s_ref, scale)
            fence(stat_ref, scale)
        return _vregs(scale)

    span = kw // len(p_refs)

    def prob_tasks(n):
        def task(r, c):
            rows = []
            for a in range(PARTS):
                rr = slice(a * bq + r, a * bq + r + 16)
                m, scale = pace.after(stat_ref[0, rr, :]), stat_ref[1, rr, :]
                cols = [b * kw + n * span + c for b in range(PARTS)]
                rows.append(jnp.concatenate([jnp.exp2(s_ref[rr, col:col + 128] - m) * scale for col in cols], axis=1))
            zs = [_zip(z) for z in _operands(jnp.concatenate(rows, axis=0), "a")]
            for j, z in enumerate(zs):
                p_refs[n][j, r // 2:r // 2 + 8, c:c + 128] = z
            if r + 16 == bq and c + 128 == span:
                fence(p_refs[n], zs[-1])
            return zs[6::7]
        return [(functools.partial(task, r, c), 80) for r in range(0, bq, 16) for c in range(0, span, 128)]

    maxes = [(functools.partial(max_task, r), 3) for r in range(0, bm, 16)]
    stats = maxes[:2]
    for n, r in enumerate(range(0, bm, 16)):
        stats += [(functools.partial(sum_task, r), 70)] + maxes[n + 2:n + 3]
    stats += [(functools.partial(scale_task, r), 4) for r in range(0, bm, 16)]
    probs = prob_tasks(0)
    pace.spread(stats + gates[:1] + convs[-late:] + probs, (3 * nl + nl // 2 - 1) * (bm // 16), lag=10, parts=4)
    fence(hg_ref, project(pace, xn_ref, W_G, hg_ref, range(nl), untied=1))
    assert len(pace.tasks) >= 1 + late + len(probs)
    project(pace, xn_ref, W_Q, hq_ref, range(nl))
    fence(hq_ref, pace.recent[-1])
    project(pace, xn_ref, W_U, hu_ref, range(nl))
    fence(hu_ref, pace.recent[-1])
    assert len(pace.tasks) <= len(probs)
    fence(uc_ref, pace.recent[-1])
    project(pace, uc_ref, W_CONV, yc_ref, range(nl // 2))

    share = Tp // (nq - 1)
    assert share * (nq - 1) == Tp and share % 16 == 0 and 2 * bm <= share * (nq - 3)
    batch = jnp.where(i == 0, step // nq, jnp.minimum(step // nq + 1, B - 1))
    norms = norm_tasks(batch * Tp + jnp.maximum(i - 1, 0) * share, share, pace.after)
    later = (block_tasks(block_row(jnp.minimum(step + 2, B * nq - 1)), None) + norms[8:]
             + _merge(gates[1:], query_tasks()) + shift_tasks())
    cut = int(0.22 * len(later))
    for n, p_ref in enumerate(p_refs):
        if n == 0:
            pace.spread(_merge(prob_tasks(1), later[:cut] + norms[:8]), PRODUCTS * (bq // 16), lag=36, back=3, parts=7)
        else:
            pace.spread(later[cut:], PRODUCTS * (bq // 16), lag=20, back=2, parts=4)
        for j in [a * 7 + b for a in (6, 0, 3, 4, 2, 1, 5) for b in (4, 6, 5, 3, 2, 1, 0)]:
            t = pace.seen(_dot(pace.tie(p_ref[j]), _rows(kv_ref[j, n * span // 2:(n + 1) * span // 2, :])))
            t = t if n == 0 else acc_ref[j] + t
            acc_ref[j] = t
        fence(acc_ref, t)

    def out_task(r):
        o = _assemble(lambda j: acc_ref[j, r:r + 16, :], ((0, 3, 4, 6, 2, 1, 5),) * LEVELS)
        out = []
        for a in range(PARTS):
            y = _zip(o[16 * a:16 * a + 16])
            ob_ref[(a * bq + r) // 2:(a * bq + r) // 2 + 8, :] = y
            out += _vregs(y)
        if r + 16 == bq:
            fence(ob_ref, y)
        return out
    pace.spread([(functools.partial(out_task, r), 1) for r in range(0, bq, 16)], (nl - nl // 2) * (bm // 16), lag=14, parts=8)
    fence(yc_ref, project(pace, uc_ref, W_CONV, yc_ref, range(nl // 2, nl)))
    pace.spread(u_tasks(pace.after), (nl - 1) * (bm // 16), lag=3, parts=2)
    for c in range(nl):
        lanes = slice(c * 128, (c + 1) * 128)
        lhs = ob_ref[0:bm // 2, :]
        ya = _dot(pace.tie(lhs) if c else _rows(lhs), _rows(w_ref[W_ATT, :, lanes]))
        for r in range(0, bm, 16):
            yc = jnp.concatenate([yc_ref[c, pl.ds(r + n, 8, stride=2), :] for n in range(2)], axis=0)
            x = _unzip(x_ref[rows16(block_row(step) + r), lanes])
            o_ref[r:r + 16, lanes] = _rows(_zip(x + (yc + ya[r:r + 16])))
    assert pace.idle()


@jax.jit
def pallas_standalone__conformer_family_branchformer__speech_kernel(
    x: jax.Array,
    w_q: jax.Array,
    w_k: jax.Array,
    w_v: jax.Array,
    w_ao: jax.Array,
    w_up: jax.Array,
    dw: jax.Array,
    w_dn: jax.Array,
    w_merge: jax.Array,
):
    B, T, D = x.shape
    weights = (w_q, w_k, w_v, w_ao, w_up, dw, w_dn, w_merge)
    assert all(a.dtype == BF16 for a in (x, *weights)) and D == 128 * PARTS and dw.shape[0] < 2 * HALO
    bm, bq = BLOCK, BLOCK // PARTS
    Tp = pl.cdiv(T, 256 * PARTS) * 256 * PARTS
    nq = pl.cdiv(T, bm)
    return pl.pallas_call(
        _kernel,
        grid=(B * nq,),
        in_specs=[pl.BlockSpec(memory_space=pl.ANY)] * (1 + len(weights)),
        out_specs=pl.BlockSpec((None, bm, D), lambda s: (s // nq, s % nq, 0)),
        out_shape=jax.ShapeDtypeStruct(x.shape, x.dtype),
        scratch_shapes=[pltpu.VMEM((B * Tp, D), BF16)] + [pltpu.VMEM((D, D), BF16)] * 7 + [
            pltpu.VMEM(dw.shape, BF16),
            pltpu.VMEM(w_merge.shape, BF16),
            pltpu.SemaphoreType.DMA((len(weights) + 3 * PARTS + B - 1,)),
            pltpu.VMEM((5, D // 2, D), U32),
            pltpu.VMEM((2 * HALO, D), F32),
            pltpu.VMEM((PRODUCTS, Tp // PARTS // 2, 128), U32),
            pltpu.VMEM((bm // 2 + 8, D), U32),
            pltpu.VMEM((PRODUCTS, bq // 2, 128), U32),
            pltpu.VMEM((bm, D), F32),
            pltpu.VMEM((bm // 2 + 8, D), U32),
            pltpu.VMEM((D // 128, bm + 2 * HALO, 128), F32),
            pltpu.VMEM((D // 128, bm + 8, 128), F32),
            pltpu.VMEM((bm + 8, Tp), F32),
            pltpu.VMEM((2, bm + 8, 128), F32),
            pltpu.VMEM((D // 128, bm + 8, 128), F32),
            pltpu.VMEM((bm + 8, D), F32),
            pltpu.VMEM((bm + 8, D), F32),
            pltpu.VMEM((bm + 8, D), F32),
            pltpu.VMEM((PRODUCTS + 1, bq, 128), F32),
            pltpu.VMEM((bm // 2 + 8, D), U32),
            pltpu.VMEM((B * Tp, D), F32),
        ] + [pltpu.VMEM((PRODUCTS + 1, bq // 2, Tp // PARTS // 2), U32)] * 2,
        compiler_params=pltpu.CompilerParams(dimension_semantics=("arbitrary",), vmem_limit_bytes=110 * 2**20),
    )(x, *weights)
```

```python
import functools
import math

import jax
import jax.numpy as jnp
from jax import lax
from jax.experimental import pallas as pl
from jax.experimental.pallas import tpu as pltpu

F32, BF16, U32 = jnp.float32, jnp.bfloat16, jnp.uint32
EPS = 1e-5
LOG2E = 1.4426950408889634
HALO = 16
LEVELS = 2
PARTS = 2 ** LEVELS
PRODUCTS = 7 ** LEVELS
BLOCK = 448
W_Q, W_U, W_G, W_ATT, W_CONV = range(5)


def _layernorm(x):
    c = x - jnp.mean(x, axis=-1, keepdims=True)
    return c * lax.rsqrt(jnp.mean(c * c, axis=-1, keepdims=True) + EPS)


def _gelu(x):
    c0 = math.sqrt(2.0 / math.pi)
    inner = x * (c0 + (c0 * 0.044715) * (x * x))
    half = 0.5 * x
    return half + half * jnp.tanh(inner)


def _dot(a, b):
    return jnp.dot(a, b, preferred_element_type=F32)


def _dot_nt(a, b):
    return lax.dot_general(a, b, (((1,), (1,)), ((), ())), preferred_element_type=F32)


def _words(x):
    return pltpu.bitcast(x, U32)


def _rows(words):
    return pltpu.bitcast(words, BF16)


def _put(ref, idx, r, x):
    for c in range(x.shape[1] // 128):
        ref[(*idx, c, slice(r, r + x.shape[0]))] = x[:, c * 128:(c + 1) * 128].astype(BF16)


def _tile(ref, idx, r, n):
    return ref.bitcast(U32)[(*idx, slice(r // 2, (r + n) // 2))]


def _get(ref, idx, n):
    return jnp.concatenate([_tile(ref, (*idx, c), 0, n) for c in range(ref.shape[-3])], axis=1)


def _vregs(x):
    return [x[r:r + 8, c:c + 128] for r in range(0, x.shape[0], 8) for c in range(0, x.shape[1], 128)]


def _operands(x, kind, level=LEVELS):
    if level == 0:
        return [x]
    r, c = x.shape[0] // 2, x.shape[1] // 2
    x11, x12, x21, x22 = x[:r, :c], x[:r, c:], x[r:, :c], x[r:, c:]
    if kind == "a":
        sums = [x11 + x22, x21 + x22, x11, x22, x11 + x12, x21 - x11, x12 - x22]
    elif kind == "b":
        sums = [x11 + x22, x11, x12 - x22, x21 - x11, x22, x11 + x12, x21 + x22]
    else:
        sums = [x11 + x22, x11, x21 - x22, x12 - x11, x22, x11 + x21, x12 + x22]
    return [z for s in sums for z in _operands(s, kind, level - 1)]


def _a_as_b(j, level=LEVELS):
    if level == 0:
        return 0
    n = 7 ** (level - 1)
    return (0, 6, 1, 4, 5, 3, 2)[j // n] * n + _a_as_b(j % n, level - 1)


_TERMS = (((0, 1), (3, 1), (4, -1), (6, 1)), ((2, 1), (4, 1)), ((1, 1), (3, 1)), ((0, 1), (1, -1), (2, 1), (5, 1)))


def _assemble(product, orders, transposed=False, base=0):
    if not orders:
        return product(base)
    n = 7 ** (len(orders) - 1)
    quads = [None] * 4
    for j in orders[0]:
        m = _assemble(product, orders[1:], transposed, base + j * n)
        for k, terms in enumerate(_TERMS):
            for i, sign in terms:
                if i == j and quads[k] is None:
                    quads[k] = (m, sign)
                elif i == j:
                    t, tsign = quads[k]
                    quads[k] = (t + m, sign) if sign == tsign else (t - m, 1) if tsign > 0 else (m - t, 1)
    assert all(sign > 0 for _, sign in quads)
    c11, c12, c21, c22 = [t for t, _ in quads]
    if transposed:
        c12, c21 = c21, c12
    return jnp.concatenate([jnp.concatenate([c11, c12], axis=1), jnp.concatenate([c21, c22], axis=1)], axis=0)


class _Pacer:
    def __init__(self, zero):
        self.keep = lax.broadcasted_iota(jnp.int32, (8, 128), 0) >= zero
        self.tasks, self.due, self.recent = [], [], []
        self.rate = self.credit = self.slot = self.back = 0

    def idle(self):
        return not self.tasks and not self.due

    def spread(self, tasks, slots, lag=0, back=0, parts=1):
        assert self.idle()
        self.tasks = list(tasks)
        self.rate = sum(c for _, c in tasks) / (slots - lag)
        self.credit = tasks[0][1]
        self.slot, self.end, self.lag, self.back, self.parts = 0, slots - 1, lag, back, parts

    def seen(self, y):
        self.recent.append(y[0:8, 0:128])
        return y

    def after(self, x):
        token = pltpu.bitcast(self.recent[max(0, len(self.recent) - 1 - self.back)], x.dtype)
        return jnp.concatenate([jnp.concatenate(
            [jnp.where(self.keep, x[r:r + 8, c:c + 128], token) for c in range(0, x.shape[1], 128)], axis=1)
            for r in range(0, x.shape[0], 8)], axis=0)

    @staticmethod
    def _any(xs):
        chains = [functools.reduce(lambda a, b: a | b, xs[n::2]) for n in range(min(2, len(xs)))]
        return functools.reduce(lambda a, b: a | b, chains)

    def tie(self, lhs):
        rows = []
        for r in range(0, lhs.shape[0], 8):
            while self.tasks and self.credit >= self.tasks[0][1] * (1 - 1e-6):
                fn, cost = self.tasks.pop(0)
                self.credit -= cost
                out = [pltpu.bitcast(v, U32) for v in fn()]
                n = min(len(out), self.parts)
                for m in range(n):
                    when = min(self.end, self.slot + self.lag + m * cost / self.rate / n)
                    self.due.append((when, self._any(out[m * len(out) // n:(m + 1) * len(out) // n])))
                self.due.sort(key=lambda d: d[0])
            token = None
            while self.due and self.due[0][0] <= self.slot:
                t = self.due.pop(0)[1]
                token = t if token is None else token | t
            self.slot += 1
            self.credit += self.rate
            t = lhs[r:r + 8]
            if token is not None:
                t0 = jnp.where(self.keep, t[:, 0:128], token)
                t = t0 if t.shape[1] == 128 else jnp.concatenate([t0, t[:, 128:]], axis=1)
            rows.append(t)
        return _rows(jnp.concatenate(rows, axis=0))


def _merge(xs, ys):
    keyed = [((n + 0.5) / len(xs), 0, n) for n in range(len(xs))] + [((n + 0.5) / len(ys), 1, n) for n in range(len(ys))]
    return [(xs, ys)[w][n] for _, w, n in sorted(keyed)]


def _run(tasks):
    for fn, _ in tasks:
        fn()


def _kernel(x_hbm, wq_hbm, wk_hbm, wv_hbm, wao_hbm, wup_hbm, dw_hbm, wdn_hbm, wm_hbm, o_ref,
            x_ref, wq_ref, wk_ref, wv_ref, wao_ref, wu_ref, wg_ref, wdn_ref, dw_ref, wm_ref, sems,
            w_ref, taps_ref, kv_ref, xn_ref, q_ref, u_ref, uc_ref, g_ref, gn_ref, s_ref,
            stat_ref, yc_ref, hg_ref, hq_ref, hu_ref, acc_ref, ob_ref, ln_ref, *p_refs):
    step = pl.program_id(0)
    B, T, D = x_hbm.shape
    K = dw_ref.shape[0]
    Tp = s_ref.shape[1]
    bm, bq = BLOCK, BLOCK // PARTS
    kw = Tp // PARTS
    nq = pl.cdiv(T, bm)
    nl = D // 128
    pad = K // 2
    i = step % nq
    zero = pl.multiple_of(jnp.minimum(step, 0) * 16, 16)

    def block_row(n):
        return (n // nq) * Tp + (n % nq) * bm

    def rows16(r):
        return pl.ds(r if isinstance(r, int) else pl.multiple_of(r, 16), 16)

    def fence(ref, val):
        val = pltpu.bitcast(val[-8:, -128:], ref.dtype)
        rows = val.shape[0]
        ref[tuple(n - 1 for n in ref.shape[:-2]) + (pl.ds(zero + ref.shape[-2] - rows, rows), pl.ds(0, 128))] = val

    def x_rows(r, gate):
        return _rows(gate(_words(x_ref[rows16(r), :]))).astype(F32)


    def block_tasks(r0, normalise):
        def task(r):
            y = _layernorm(x_rows(r0 + r, normalise)) if normalise else ln_ref[rows16(r0 + r), :]
            _put(xn_ref, (), r, y)
            if r + 16 == bm:
                fence(xn_ref, y)
            return _vregs(y[0:8])
        return [(functools.partial(task, r), 40 if normalise else 4) for r in range(0, bm, 16)]

    def norm_tasks(r0, n, gate):
        def task(r):
            y = _layernorm(x_rows(r0 + r, gate))
            ln_ref[rows16(r0 + r), :] = y
            return _vregs(y)
        return [(functools.partial(task, r), 40) for r in range(0, n, 16)]

    def gate_tasks(gate):
        def task(r):
            g = _layernorm(_gelu(gate(hg_ref[r:r + 16, :])))
            for c in range(nl):
                gn_ref[c, r:r + 16, :] = g[:, c * 128:(c + 1) * 128]
                if r < HALO:
                    g_ref[c, HALO + bm + r:HALO + bm + r + 16, :] = g[:, c * 128:(c + 1) * 128]
            if r + 16 == bm:
                fence(gn_ref, g)
            return _vregs(g)
        return [(functools.partial(task, r), 30) for r in range(0, bm, 16)]

    def shift_tasks():
        def move(src, r, dst, n):
            out = []
            for c in range(nl):
                y = src[c, r:r + n, :]
                g_ref[c, dst:dst + n, :] = y
                out += _vregs(y)
            return out
        return ([(functools.partial(move, g_ref, bm, 0, HALO), 8)]
                + [(functools.partial(move, gn_ref, r, HALO + r, 32), 16) for r in range(0, bm, 32)])

    def u_tasks(gate):
        def task(r):
            y = _gelu(gate(hu_ref[r:r + 16, :]))
            u_ref[r:r + 16, :] = y
            return _vregs(y)
        return [(functools.partial(task, r), 24) for r in range(0, bm, 16)]

    def query_tasks():
        def task(r):
            x = jnp.concatenate([hq_ref[a * bq + r:a * bq + r + 16, :] for a in range(PARTS)], axis=0)
            zs = _operands(x, "bt")
            for j, z in enumerate(zs):
                q_ref[j, r:r + 16, :] = z.astype(BF16)
            return [z[0:8] for z in zs]
        return [(functools.partial(task, r), 40) for r in range(0, bq, 16)]

    def key_tasks(base, r0, n, normalise):
        def task(r):
            rows = [base + a * kw + r0 + r for a in range(PARTS)]
            if normalise:
                xs = [_layernorm(x_rows(row, normalise)) for row in rows]
                for row, y in zip(rows, xs):
                    ln_ref[rows16(row), :] = y
            else:
                xs = [ln_ref[rows16(row), :] for row in rows]
            zs = _operands(jnp.concatenate(xs, axis=0), "b")
            for j, z in enumerate(zs):
                kv_ref[j, rows16(r0 + r), :] = z.astype(BF16)
            return [v for z in zs[::2] for v in _vregs(z)]
        return [(functools.partial(task, r), 160) for r in range(0, n, 16)]

    def project(pacer, src, w, dst, cols, untied=0):
        for n, c in enumerate(cols):
            lhs = _rows(_get(src, (), bm)) if n < untied else pacer.tie(_get(src, (), bm))
            y = pacer.seen(_dot(lhs, _rows(_tile(w_ref, (w, c), 0, D))))
            dst[0:bm, c * 128:(c + 1) * 128] = y
        return y

    copies = []

    def fetch(src, dst):
        copies.append(pltpu.make_async_copy(src, dst, sems.at[len(copies)]))
        return copies[-1]

    def fetch_x(b, r0, r1):
        return fetch(x_hbm.at[b, pl.ds(r0, r1 - r0)], x_ref.at[pl.ds(b * Tp + r0, r1 - r0)])

    def start(group):
        for c in group:
            c.start()

    def wait(group):
        for c in group:
            c.wait()

    cuts = (256, 704)

    def fetch_keys(r0, r1):
        return [fetch_x(0, a * kw + r0, min(T, a * kw + r1)) for a in range(1, PARTS)]

    group = [
        [fetch_x(0, 0, bm)],
        [fetch(wup_hbm.at[:, pl.ds(D, D)], wg_ref)],
        [fetch(wup_hbm.at[:, pl.ds(0, D)], wu_ref)],
        [fetch(wq_hbm, wq_ref), fetch(wk_hbm, wk_ref)] + fetch_keys(0, cuts[0]),
        [fetch(wv_hbm, wv_ref), fetch(wao_hbm, wao_ref), fetch_x(0, bm, kw)] + fetch_keys(*cuts),
        [fetch(wdn_hbm, wdn_ref), fetch(wm_hbm, wm_ref), fetch(dw_hbm, dw_ref)],
        fetch_keys(cuts[1], kw),
    ]
    assert cuts[0] <= bm and 2 * bm <= kw
    batches = [fetch_x(b, 0, T) for b in range(1, B)]

    @pl.when(step == 0)
    def _():
        start(group[0] + group[1])
        for b in range(B):
            x_ref[b * Tp + T:(b + 1) * Tp, :] = jnp.zeros((Tp - T, D), x_ref.dtype)
        for c in range(nl):
            g_ref[c, bm:bm + HALO, :] = jnp.zeros((HALO, 128), F32)
        wait(group[0])
        start(group[2] + group[3])
        early = _Pacer(zero)

        def weights(lhs, rhs_ref, r0):
            cols = [_dot(early.tie(lhs), rhs_ref[r0:r0 + D, c:c + 128]) for c in range(0, D, 128)]
            return jnp.concatenate([early.seen(y) for y in cols], axis=1)

        _run(block_tasks(0, lambda w: w))
        wait(group[1])
        start(group[4])
        _put(w_ref, (W_G,), 0, wg_ref[...])
        fence(hg_ref, project(early, xn_ref, W_G, hg_ref, range(nl)))
        wait(group[2])
        _put(w_ref, (W_U,), 0, wu_ref[...])
        early.spread(gate_tasks(early.after), nl * (bm // 16), lag=14, parts=2)
        fence(hu_ref, project(early, xn_ref, W_U, hu_ref, range(nl)))
        wait(group[3])
        start(group[5])
        early.spread(u_tasks(early.after) + shift_tasks() + key_tasks(0, 0, cuts[0], early.after),
                     D // 16 + nl * (bm // 16), lag=8, parts=7)
        qk = _dot_nt(early.tie(_words(wq_ref[...])), wk_ref[...])
        _put(w_ref, (W_Q,), 0, qk * (LOG2E * float(D) ** -0.5))
        fence(hq_ref, project(early, xn_ref, W_Q, hq_ref, range(nl)))
        wait(group[4])
        start(group[6])
        early.spread(query_tasks() + block_tasks(bm, early.after) + key_tasks(0, cuts[0], cuts[1] - cuts[0], early.after),
                     3 * nl * (D // 16), lag=8, parts=7)
        vo = weights(_words(wv_ref[...]), wao_ref, 0)
        wait(group[5])
        taps_ref[0:K, :] = dw_ref[...].astype(F32)
        _put(w_ref, (W_CONV,), 0, weights(_words(wdn_ref[...]), wm_ref, D))
        _put(w_ref, (W_ATT,), 0, weights(_words(vo.astype(BF16)), wm_ref, 0))
        assert early.idle()
        wait(group[6])
        start(batches)

        @pl.loop(cuts[1] // 64, kw // 64)
        def _(j):
            _run(key_tasks(0, j * 64, 64, lambda w: w))

    for n, copy in enumerate(batches):
        pl.when(step == n * nq + 1)(copy.wait)

    @pl.when(jnp.logical_and(i == 0, step > 0))
    def _():
        @pl.loop(0, kw // 16)
        def _(j):
            _run(key_tasks(block_row(step), j * 16, 16, None))

    pace = _Pacer(zero)
    gates = gate_tasks(pace.after)

    def conv_task(c, r):
        lanes = slice(c * 128, (c + 1) * 128)
        acc, partial = None, []
        for shift in range(8):
            if shift:
                partial.append(acc[0:8])
            taps = [k for k in range(K) if (HALO - pad + k) % 8 == shift]
            lo = HALO - pad + taps[0] + r
            window = g_ref[c, lo:lo + 16 + 8 * (len(taps) - 1), :]
            for n, k in enumerate(taps):
                t = window[8 * n:8 * n + 16] * taps_ref[k:k + 1, lanes]
                acc = t if acc is None else acc + t
        y = u_ref[r:r + 16, lanes] * acc
        uc_ref[c, r:r + 16, :] = y.astype(BF16)
        return partial + [y[0:8]]
    convs = [(functools.partial(conv_task, c, r), 48) for r in range(0, bm, 16) for c in range(nl)]
    late = nl * pl.cdiv(pad, 16)
    pace.spread(convs[:-late], PRODUCTS * (kw // 128) * (bq // 16), parts=8)

    peak = None
    for c0 in range(0, kw, 128):
        def product(j):
            return pace.seen(_dot_nt(pace.tie(_tile(q_ref, (j,), 0, bq)), _rows(_tile(kv_ref, (_a_as_b(j),), c0, 128))))
        s = _assemble(product, ((1, 3, 2, 4, 0, 5, 6), (2, 5, 4, 1, 0, 3, 6)), transposed=True)
        tiles = []
        for a in range(PARTS):
            t = s[:, a * 128:(a + 1) * 128]
            col0 = a * kw + c0
            if col0 + 128 > T:
                t = jnp.where(col0 + lax.broadcasted_iota(jnp.int32, t.shape, 1) < T, t, -jnp.inf)
            s_ref[0:bm, col0:col0 + 128] = t
            tiles.append(t)
        for n in range(0, PARTS, 2):
            t = jnp.maximum(tiles[n], tiles[n + 1])
            peak = t if peak is None else jnp.maximum(peak, t)
    fence(s_ref, tiles[-1])
    stat_ref[0, 0:bm, :] = peak
    fence(stat_ref, peak)

    rowmax, rowsum = {}, {}

    def max_task(r):
        rowmax[r] = jnp.broadcast_to(jnp.max(stat_ref[0, r:r + 16, :], axis=-1, keepdims=True), (16, 128))
        return _vregs(rowmax[r])

    def sum_task(r):
        total = None
        for c in range(0, Tp, 128):
            e = jnp.exp2(s_ref[r:r + 16, c:c + 128] - rowmax[r])
            total = e if total is None else total + e
        rowsum[r] = total
        return _vregs(total)

    def scale_task(r):
        scale = jnp.broadcast_to(1.0 / jnp.sum(pace.after(rowsum[r]), axis=-1, keepdims=True), (16, 128))
        stat_ref[0, r:r + 16, :] = rowmax[r]
        stat_ref[1, r:r + 16, :] = scale
        if r + 16 == bm:
            fence(s_ref, scale)
            fence(stat_ref, scale)
        return _vregs(scale)

    span = kw // len(p_refs)

    def prob_tasks(n):
        def task(r, c):
            rows = []
            for a in range(PARTS):
                rr = slice(a * bq + r, a * bq + r + 16)
                m, scale = pace.after(stat_ref[0, rr, :]), stat_ref[1, rr, :]
                cols = [b * kw + n * span + c for b in range(PARTS)]
                rows.append(jnp.concatenate([jnp.exp2(s_ref[rr, col:col + 128] - m) * scale for col in cols], axis=1))
            zs = _operands(jnp.concatenate(rows, axis=0), "a")
            for j, z in enumerate(zs):
                p_refs[n][j, c // 128, r:r + 16, :] = z.astype(BF16)
            if r + 16 == bq and c + 128 == span:
                fence(p_refs[n], zs[-1][0:8])
            return [z[0:8] for z in zs[6::7]]
        return [(functools.partial(task, r, c), 80) for r in range(0, bq, 16) for c in range(0, span, 128)]

    maxes = [(functools.partial(max_task, r), 3) for r in range(0, bm, 16)]
    stats = maxes[:2]
    for n, r in enumerate(range(0, bm, 16)):
        stats += [(functools.partial(sum_task, r), 70)] + maxes[n + 2:n + 3]
    stats += [(functools.partial(scale_task, r), 4) for r in range(0, bm, 16)]
    probs = prob_tasks(0)
    pace.spread(stats + gates[:1] + convs[-late:] + probs, (3 * nl + nl // 2 - 1) * (bm // 16), lag=10, parts=4)
    fence(hg_ref, project(pace, xn_ref, W_G, hg_ref, range(nl), untied=1))
    assert len(pace.tasks) >= 1 + late + len(probs)
    project(pace, xn_ref, W_Q, hq_ref, range(nl))
    fence(hq_ref, pace.recent[-1])
    project(pace, xn_ref, W_U, hu_ref, range(nl))
    fence(hu_ref, pace.recent[-1])
    assert len(pace.tasks) <= len(probs)
    fence(uc_ref, pace.recent[-1])
    project(pace, uc_ref, W_CONV, yc_ref, range(nl // 2))

    share = Tp // (nq - 1)
    assert share * (nq - 1) == Tp and share % 16 == 0 and 2 * bm <= share * (nq - 3)
    batch = jnp.where(i == 0, step // nq, jnp.minimum(step // nq + 1, B - 1))
    norms = norm_tasks(batch * Tp + jnp.maximum(i - 1, 0) * share, share, pace.after)
    later = (block_tasks(block_row(jnp.minimum(step + 2, B * nq - 1)), None) + norms[8:]
             + _merge(gates[1:], query_tasks()) + shift_tasks())
    cut = int(0.22 * len(later))
    for n, p_ref in enumerate(p_refs):
        if n == 0:
            pace.spread(_merge(prob_tasks(1), later[:cut] + norms[:8]), PRODUCTS * (bq // 16), lag=36, back=3, parts=7)
        else:
            pace.spread(later[cut:], PRODUCTS * (bq // 16), lag=20, back=2, parts=4)
        for j in [a * 7 + b for a in (6, 0, 3, 4, 2, 1, 5) for b in (4, 6, 5, 3, 2, 1, 0)]:
            t = pace.seen(_dot(pace.tie(_get(p_ref, (j,), bq)), _rows(_tile(kv_ref, (j,), n * span, span))))
            t = t if n == 0 else acc_ref[j] + t
            acc_ref[j] = t
        fence(acc_ref, t)

    def out_task(r):
        o = _assemble(lambda j: acc_ref[j, r:r + 16, :], ((0, 3, 4, 6, 2, 1, 5),) * LEVELS)
        out = []
        for a in range(PARTS):
            y = o[16 * a:16 * a + 16]
            _put(ob_ref, (), a * bq + r, y)
            out += _vregs(y[8:16])
        if r + 16 == bq:
            fence(ob_ref, y)
        return out
    pace.spread([(functools.partial(out_task, r), 1) for r in range(0, bq, 16)], (nl - nl // 2) * (bm // 16), lag=14, parts=8)
    fence(yc_ref, project(pace, uc_ref, W_CONV, yc_ref, range(nl // 2, nl)))
    pace.spread(u_tasks(pace.after), (nl - 1) * (bm // 16), lag=3, parts=2)
    for c in range(nl):
        lanes = slice(c * 128, (c + 1) * 128)
        lhs = _get(ob_ref, (), bm)
        ya = _dot(pace.tie(lhs) if c else _rows(lhs), _rows(_tile(w_ref, (W_ATT, c), 0, D)))
        for r in range(0, bm, 16):
            x = x_ref[rows16(block_row(step) + r), lanes].astype(F32)
            o_ref[r:r + 16, lanes] = (x + (yc_ref[r:r + 16, lanes] + ya[r:r + 16])).astype(o_ref.dtype)
    assert pace.idle()


@jax.jit
def pallas_standalone__conformer_family_branchformer__speech_kernel(
    x: jax.Array,
    w_q: jax.Array,
    w_k: jax.Array,
    w_v: jax.Array,
    w_ao: jax.Array,
    w_up: jax.Array,
    dw: jax.Array,
    w_dn: jax.Array,
    w_merge: jax.Array,
):
    B, T, D = x.shape
    weights = (w_q, w_k, w_v, w_ao, w_up, dw, w_dn, w_merge)
    assert all(a.dtype == BF16 for a in (x, *weights)) and D == 128 * PARTS and dw.shape[0] < 2 * HALO
    bm, bq = BLOCK, BLOCK // PARTS
    Tp = pl.cdiv(T, 256 * PARTS) * 256 * PARTS
    nq = pl.cdiv(T, bm)
    return pl.pallas_call(
        _kernel,
        grid=(B * nq,),
        in_specs=[pl.BlockSpec(memory_space=pl.ANY)] * (1 + len(weights)),
        out_specs=pl.BlockSpec((None, bm, D), lambda s: (s // nq, s % nq, 0)),
        out_shape=jax.ShapeDtypeStruct(x.shape, x.dtype),
        scratch_shapes=[pltpu.VMEM((B * Tp, D), BF16)] + [pltpu.VMEM((D, D), BF16)] * 7 + [
            pltpu.VMEM(dw.shape, BF16),
            pltpu.VMEM(w_merge.shape, BF16),
            pltpu.SemaphoreType.DMA((len(weights) + 3 * PARTS + B - 1,)),
            pltpu.VMEM((5, D // 128, D, 128), BF16),
            pltpu.VMEM((2 * HALO, D), F32),
            pltpu.VMEM((PRODUCTS, Tp // PARTS, 128), BF16),
            pltpu.VMEM((D // 128, bm + 16, 128), BF16),
            pltpu.VMEM((PRODUCTS, bq, 128), BF16),
            pltpu.VMEM((bm, D), F32),
            pltpu.VMEM((D // 128, bm + 16, 128), BF16),
            pltpu.VMEM((D // 128, bm + 2 * HALO, 128), F32),
            pltpu.VMEM((D // 128, bm + 8, 128), F32),
            pltpu.VMEM((bm + 8, Tp), F32),
            pltpu.VMEM((2, bm + 8, 128), F32),
            pltpu.VMEM((bm + 8, D), F32),
            pltpu.VMEM((bm + 8, D), F32),
            pltpu.VMEM((bm + 8, D), F32),
            pltpu.VMEM((bm + 8, D), F32),
            pltpu.VMEM((PRODUCTS + 1, bq, 128), F32),
            pltpu.VMEM((D // 128, bm + 16, 128), BF16),
            pltpu.VMEM((B * Tp, D), F32),
        ] + [pltpu.VMEM((PRODUCTS + 1, Tp // PARTS // 256, bq, 128), BF16)] * 2,
        compiler_params=pltpu.CompilerParams(dimension_semantics=("arbitrary",), vmem_limit_bytes=110 * 2**20),
    )(x, *weights)
```

```python
import functools
import math

import jax
import jax.numpy as jnp
from jax import lax
from jax.experimental import pallas as pl
from jax.experimental.pallas import tpu as pltpu

F32, BF16, U32 = jnp.float32, jnp.bfloat16, jnp.uint32
EPS = 1e-5
LOG2E = 1.4426950408889634
HALO = 16
LEVELS = 2
PARTS = 2 ** LEVELS
PRODUCTS = 7 ** LEVELS
BLOCK = 448
W_Q, W_U, W_G, W_ATT, W_CONV = range(5)


def _layernorm(x):
    c = x - jnp.mean(x, axis=-1, keepdims=True)
    return c * lax.rsqrt(jnp.mean(c * c, axis=-1, keepdims=True) + EPS)


def _gelu(x):
    c0 = math.sqrt(2.0 / math.pi)
    inner = x * (c0 + (c0 * 0.044715) * (x * x))
    half = 0.5 * x
    return half + half * jnp.tanh(inner)


def _dot(a, b):
    return jnp.dot(a, b, preferred_element_type=F32)


def _dot_nt(a, b):
    return lax.dot_general(a, b, (((1,), (1,)), ((), ())), preferred_element_type=F32)


def _words(x):
    return pltpu.bitcast(x, U32)


def _rows(words):
    return pltpu.bitcast(words, BF16)


def _put(ref, idx, r, x):
    for c in range(x.shape[1] // 128):
        ref[(*idx, c, slice(r, r + x.shape[0]))] = x[:, c * 128:(c + 1) * 128].astype(BF16)


def _tile(ref, idx, r, n):
    return ref.bitcast(U32)[(*idx, slice(r // 2, (r + n) // 2))]


def _get(ref, idx, n):
    return jnp.concatenate([_tile(ref, (*idx, c), 0, n) for c in range(ref.shape[-3])], axis=1)


def _vregs(x):
    return [x[r:r + 8, c:c + 128] for r in range(0, x.shape[0], 8) for c in range(0, x.shape[1], 128)]


def _operands(x, kind, level=LEVELS):
    if level == 0:
        return [x]
    r, c = x.shape[0] // 2, x.shape[1] // 2
    x11, x12, x21, x22 = x[:r, :c], x[:r, c:], x[r:, :c], x[r:, c:]
    if kind == "a":
        sums = [x11 + x22, x21 + x22, x11, x22, x11 + x12, x21 - x11, x12 - x22]
    elif kind == "b":
        sums = [x11 + x22, x11, x12 - x22, x21 - x11, x22, x11 + x12, x21 + x22]
    else:
        sums = [x11 + x22, x11, x21 - x22, x12 - x11, x22, x11 + x21, x12 + x22]
    return [z for s in sums for z in _operands(s, kind, level - 1)]


def _a_as_b(j, level=LEVELS):
    if level == 0:
        return 0
    n = 7 ** (level - 1)
    return (0, 6, 1, 4, 5, 3, 2)[j // n] * n + _a_as_b(j % n, level - 1)


_TERMS = (((0, 1), (3, 1), (4, -1), (6, 1)), ((2, 1), (4, 1)), ((1, 1), (3, 1)), ((0, 1), (1, -1), (2, 1), (5, 1)))


def _assemble(product, orders, transposed=False, base=0):
    if not orders:
        return product(base)
    n = 7 ** (len(orders) - 1)
    quads = [None] * 4
    for j in orders[0]:
        m = _assemble(product, orders[1:], transposed, base + j * n)
        for k, terms in enumerate(_TERMS):
            for i, sign in terms:
                if i == j and quads[k] is None:
                    quads[k] = (m, sign)
                elif i == j:
                    t, tsign = quads[k]
                    quads[k] = (t + m, sign) if sign == tsign else (t - m, 1) if tsign > 0 else (m - t, 1)
    assert all(sign > 0 for _, sign in quads)
    c11, c12, c21, c22 = [t for t, _ in quads]
    if transposed:
        c12, c21 = c21, c12
    return jnp.concatenate([jnp.concatenate([c11, c12], axis=1), jnp.concatenate([c21, c22], axis=1)], axis=0)


class _Pacer:
    def __init__(self, zero):
        self.keep = lax.broadcasted_iota(jnp.int32, (8, 128), 0) >= zero
        self.tasks, self.due, self.recent = [], [], []
        self.rate = self.credit = self.slot = self.back = 0

    def idle(self):
        return not self.tasks and not self.due

    def spread(self, tasks, slots, lag=0, back=0, parts=1):
        assert self.idle()
        self.tasks = list(tasks)
        self.rate = sum(c for _, c in tasks) / (slots - lag)
        self.credit = tasks[0][1]
        self.slot, self.end, self.lag, self.back, self.parts = 0, slots - 1, lag, back, parts

    def seen(self, y):
        self.recent.append(y[0:8, 0:128])
        return y

    def after(self, x):
        token = pltpu.bitcast(self.recent[max(0, len(self.recent) - 1 - self.back)], x.dtype)
        return jnp.concatenate([jnp.concatenate(
            [jnp.where(self.keep, x[r:r + 8, c:c + 128], token) for c in range(0, x.shape[1], 128)], axis=1)
            for r in range(0, x.shape[0], 8)], axis=0)

    @staticmethod
    def _any(xs):
        chains = [functools.reduce(lambda a, b: a | b, xs[n::2]) for n in range(min(2, len(xs)))]
        return functools.reduce(lambda a, b: a | b, chains)

    def tie(self, lhs):
        rows = []
        for r in range(0, lhs.shape[0], 8):
            while self.tasks and self.credit >= self.tasks[0][1] * (1 - 1e-6):
                fn, cost = self.tasks.pop(0)
                self.credit -= cost
                out = [pltpu.bitcast(v, U32) for v in fn()]
                n = min(len(out), self.parts)
                for m in range(n):
                    when = min(self.end, self.slot + self.lag + m * cost / self.rate / n)
                    self.due.append((when, self._any(out[m * len(out) // n:(m + 1) * len(out) // n])))
                self.due.sort(key=lambda d: d[0])
            token = None
            while self.due and self.due[0][0] <= self.slot:
                t = self.due.pop(0)[1]
                token = t if token is None else token | t
            self.slot += 1
            self.credit += self.rate
            t = lhs[r:r + 8]
            if token is not None:
                t0 = jnp.where(self.keep, t[:, 0:128], token)
                t = t0 if t.shape[1] == 128 else jnp.concatenate([t0, t[:, 128:]], axis=1)
            rows.append(t)
        return _rows(jnp.concatenate(rows, axis=0))


def _merge(xs, ys):
    keyed = [((n + 0.5) / len(xs), 0, n) for n in range(len(xs))] + [((n + 0.5) / len(ys), 1, n) for n in range(len(ys))]
    return [(xs, ys)[w][n] for _, w, n in sorted(keyed)]


def _run(tasks):
    for fn, _ in tasks:
        fn()


def _kernel(x_hbm, wq_hbm, wk_hbm, wv_hbm, wao_hbm, wup_hbm, dw_hbm, wdn_hbm, wm_hbm, o_ref,
            x_ref, wq_ref, wk_ref, wv_ref, wao_ref, wu_ref, wg_ref, wdn_ref, dw_ref, wm_ref, sems,
            w_ref, taps_ref, kv_ref, xn_ref, q_ref, u_ref, uc_ref, g_ref, gn_ref, s_ref,
            stat_ref, yc_ref, hg_ref, hq_ref, hu_ref, acc_ref, ob_ref, ln_ref, *p_refs):
    step = pl.program_id(0)
    B, T, D = x_hbm.shape
    K = dw_ref.shape[0]
    Tp = s_ref.shape[1]
    bm, bq = BLOCK, BLOCK // PARTS
    kw = Tp // PARTS
    nq = pl.cdiv(T, bm)
    nl = D // 128
    pad = K // 2
    i = step % nq
    zero = pl.multiple_of(jnp.minimum(step, 0) * 16, 16)

    def block_row(n):
        return (n // nq) * Tp + (n % nq) * bm

    def rows16(r):
        return pl.ds(r if isinstance(r, int) else pl.multiple_of(r, 16), 16)

    def fence(ref, val):
        val = pltpu.bitcast(val[-8:, -128:], ref.dtype)
        rows = val.shape[0]
        ref[tuple(n - 1 for n in ref.shape[:-2]) + (pl.ds(zero + ref.shape[-2] - rows, rows), pl.ds(0, 128))] = val

    def x_rows(r, gate):
        return _rows(gate(_words(x_ref[rows16(r), :]))).astype(F32)


    def block_tasks(r0, normalise):
        def task(r):
            y = _layernorm(x_rows(r0 + r, normalise)) if normalise else ln_ref[rows16(r0 + r), :]
            _put(xn_ref, (), r, y)
            if r + 16 == bm:
                fence(xn_ref, y)
            return _vregs(y[0:8])
        return [(functools.partial(task, r), 40 if normalise else 4) for r in range(0, bm, 16)]

    def norm_tasks(r0, n, gate):
        def task(r):
            y = _layernorm(x_rows(r0 + r, gate))
            ln_ref[rows16(r0 + r), :] = y
            return _vregs(y)
        return [(functools.partial(task, r), 50) for r in range(0, n, 16)]

    def gate_tasks(gate):
        def task(r):
            g = _layernorm(_gelu(gate(hg_ref[r:r + 16, :])))
            for c in range(nl):
                gn_ref[c, r:r + 16, :] = g[:, c * 128:(c + 1) * 128]
                if r < HALO:
                    g_ref[c, HALO + bm + r:HALO + bm + r + 16, :] = g[:, c * 128:(c + 1) * 128]
            if r + 16 == bm:
                fence(gn_ref, g)
            return _vregs(g)
        return [(functools.partial(task, r), 50) for r in range(0, bm, 16)]

    def shift_tasks():
        def move(src, r, dst, n):
            out = []
            for c in range(nl):
                y = src[c, r:r + n, :]
                g_ref[c, dst:dst + n, :] = y
                out += _vregs(y)
            return out
        return ([(functools.partial(move, g_ref, bm, 0, HALO), 8)]
                + [(functools.partial(move, gn_ref, r, HALO + r, 32), 16) for r in range(0, bm, 32)])

    def u_tasks(gate):
        def task(r):
            y = _gelu(gate(hu_ref[r:r + 16, :]))
            u_ref[r:r + 16, :] = y
            return _vregs(y)
        return [(functools.partial(task, r), 24) for r in range(0, bm, 16)]

    def query_tasks():
        def task(r):
            x = jnp.concatenate([hq_ref[a * bq + r:a * bq + r + 16, :] for a in range(PARTS)], axis=0)
            zs = _operands(x, "bt")
            for j, z in enumerate(zs):
                q_ref[j, r:r + 16, :] = z.astype(BF16)
            return [z[0:8] for z in zs[::2]]
        return [(functools.partial(task, r), 40) for r in range(0, bq, 16)]

    def key_tasks(base, r0, n, normalise):
        def task(r):
            rows = [base + a * kw + r0 + r for a in range(PARTS)]
            if normalise:
                xs = [_layernorm(x_rows(row, normalise)) for row in rows]
                for row, y in zip(rows, xs):
                    ln_ref[rows16(row), :] = y
            else:
                xs = [ln_ref[rows16(row), :] for row in rows]
            zs = _operands(jnp.concatenate(xs, axis=0), "b")
            for j, z in enumerate(zs):
                kv_ref[j, rows16(r0 + r), :] = z.astype(BF16)
            return [v for z in zs[::2] for v in _vregs(z)]
        return [(functools.partial(task, r), 160) for r in range(0, n, 16)]

    def project(pacer, src, w, dst, cols, untied=0):
        for n, c in enumerate(cols):
            lhs = _rows(_get(src, (), bm)) if n < untied else pacer.tie(_get(src, (), bm))
            y = pacer.seen(_dot(lhs, _rows(_tile(w_ref, (w, c), 0, D))))
            dst[0:bm, c * 128:(c + 1) * 128] = y
        return y

    copies = []

    def fetch(src, dst):
        copies.append(pltpu.make_async_copy(src, dst, sems.at[len(copies)]))
        return copies[-1]

    def fetch_x(b, r0, r1):
        return fetch(x_hbm.at[b, pl.ds(r0, r1 - r0)], x_ref.at[pl.ds(b * Tp + r0, r1 - r0)])

    def start(group):
        for c in group:
            c.start()

    def wait(group):
        for c in group:
            c.wait()

    cuts = (256, 704)

    def fetch_keys(r0, r1):
        return [fetch_x(0, a * kw + r0, min(T, a * kw + r1)) for a in range(1, PARTS)]

    group = [
        [fetch_x(0, 0, bm)],
        [fetch(wup_hbm.at[:, pl.ds(D, D)], wg_ref)],
        [fetch(wup_hbm.at[:, pl.ds(0, D)], wu_ref)],
        [fetch(wq_hbm, wq_ref), fetch(wk_hbm, wk_ref)] + fetch_keys(0, cuts[0]),
        [fetch(wv_hbm, wv_ref), fetch(wao_hbm, wao_ref), fetch_x(0, bm, kw)] + fetch_keys(*cuts),
        [fetch(wdn_hbm, wdn_ref), fetch(wm_hbm, wm_ref), fetch(dw_hbm, dw_ref)],
        fetch_keys(cuts[1], kw),
    ]
    assert cuts[0] <= bm and 2 * bm <= kw
    batches = [fetch_x(b, 0, T) for b in range(1, B)]

    @pl.when(step == 0)
    def _():
        start(group[0] + group[1])
        for b in range(B):
            x_ref[b * Tp + T:(b + 1) * Tp, :] = jnp.zeros((Tp - T, D), x_ref.dtype)
        for c in range(nl):
            g_ref[c, bm:bm + HALO, :] = jnp.zeros((HALO, 128), F32)
        wait(group[0])
        start(group[2] + group[3])
        early = _Pacer(zero)

        def weights(lhs, rhs_ref, r0):
            cols = [_dot(early.tie(lhs), rhs_ref[r0:r0 + D, c:c + 128]) for c in range(0, D, 128)]
            return jnp.concatenate([early.seen(y) for y in cols], axis=1)

        _run(block_tasks(0, lambda w: w))
        wait(group[1])
        start(group[4])
        _put(w_ref, (W_G,), 0, wg_ref[...])
        fence(hg_ref, project(early, xn_ref, W_G, hg_ref, range(nl)))
        wait(group[2])
        _put(w_ref, (W_U,), 0, wu_ref[...])
        early.spread(gate_tasks(early.after), nl * (bm // 16), lag=14, parts=2)
        fence(hu_ref, project(early, xn_ref, W_U, hu_ref, range(nl)))
        wait(group[3])
        start(group[5])
        early.spread(u_tasks(early.after) + shift_tasks() + key_tasks(0, 0, cuts[0], early.after),
                     D // 16 + nl * (bm // 16), lag=8, parts=7)
        qk = _dot_nt(early.tie(_words(wq_ref[...])), wk_ref[...])
        _put(w_ref, (W_Q,), 0, qk * (LOG2E * float(D) ** -0.5))
        fence(hq_ref, project(early, xn_ref, W_Q, hq_ref, range(nl)))
        wait(group[4])
        start(group[6])
        early.spread(query_tasks() + block_tasks(bm, early.after) + key_tasks(0, cuts[0], cuts[1] - cuts[0], early.after),
                     3 * nl * (D // 16), lag=8, parts=7)
        vo = weights(_words(wv_ref[...]), wao_ref, 0)
        wait(group[5])
        taps_ref[0:K, :] = dw_ref[...].astype(F32)
        _put(w_ref, (W_CONV,), 0, weights(_words(wdn_ref[...]), wm_ref, D))
        _put(w_ref, (W_ATT,), 0, weights(_words(vo.astype(BF16)), wm_ref, 0))
        assert early.idle()
        wait(group[6])
        start(batches)

        @pl.loop(cuts[1] // 64, kw // 64)
        def _(j):
            _run(key_tasks(0, j * 64, 64, lambda w: w))

    for n, copy in enumerate(batches):
        pl.when(step == n * nq + 1)(copy.wait)

    @pl.when(jnp.logical_and(i == 0, step > 0))
    def _():
        @pl.loop(0, kw // 16)
        def _(j):
            _run(key_tasks(block_row(step), j * 16, 16, None))

    pace = _Pacer(zero)
    gates = gate_tasks(pace.after)

    def conv_task(c, r):
        lanes = slice(c * 128, (c + 1) * 128)
        acc, partial = None, []
        for shift in range(8):
            if shift:
                partial.append(acc[0:8])
            taps = [k for k in range(K) if (HALO - pad + k) % 8 == shift]
            lo = HALO - pad + taps[0] + r
            window = g_ref[c, lo:lo + 16 + 8 * (len(taps) - 1), :]
            for n, k in enumerate(taps):
                t = window[8 * n:8 * n + 16] * taps_ref[k:k + 1, lanes]
                acc = t if acc is None else acc + t
        y = u_ref[r:r + 16, lanes] * acc
        uc_ref[c, r:r + 16, :] = y.astype(BF16)
        return partial + [y[0:8]]
    convs = [(functools.partial(conv_task, c, r), 48) for r in range(0, bm, 16) for c in range(nl)]
    late = nl * pl.cdiv(pad, 16)
    pace.spread(convs[:-late], PRODUCTS * (kw // 128) * (bq // 16), parts=8)

    peak = None
    for c0 in range(0, kw, 128):
        def product(j):
            return pace.seen(_dot_nt(pace.tie(_tile(q_ref, (j,), 0, bq)), _rows(_tile(kv_ref, (_a_as_b(j),), c0, 128))))
        s = _assemble(product, ((1, 3, 2, 4, 0, 5, 6), (2, 5, 4, 1, 0, 3, 6)), transposed=True)
        tiles = []
        for a in range(PARTS):
            t = s[:, a * 128:(a + 1) * 128]
            col0 = a * kw + c0
            if col0 + 128 > T:
                t = jnp.where(col0 + lax.broadcasted_iota(jnp.int32, t.shape, 1) < T, t, -jnp.inf)
            s_ref[0:bm, col0:col0 + 128] = t
            tiles.append(t)
        for n in range(0, PARTS, 2):
            t = jnp.maximum(tiles[n], tiles[n + 1])
            peak = t if peak is None else jnp.maximum(peak, t)
    fence(s_ref, tiles[-1])
    stat_ref[0, 0:bm, :] = peak
    fence(stat_ref, peak)

    rowmax, rowsum = {}, {}

    def max_task(r):
        rowmax[r] = jnp.broadcast_to(jnp.max(stat_ref[0, r:r + 16, :], axis=-1, keepdims=True), (16, 128))
        return _vregs(rowmax[r])

    def sum_task(r):
        total = None
        for c in range(0, Tp, 128):
            e = jnp.exp2(s_ref[r:r + 16, c:c + 128] - rowmax[r])
            total = e if total is None else total + e
        rowsum[r] = total
        return _vregs(total)

    def scale_task(r):
        scale = jnp.broadcast_to(1.0 / jnp.sum(pace.after(rowsum[r]), axis=-1, keepdims=True), (16, 128))
        stat_ref[0, r:r + 16, :] = rowmax[r]
        stat_ref[1, r:r + 16, :] = scale
        if r + 16 == bm:
            fence(s_ref, scale)
            fence(stat_ref, scale)
        return _vregs(scale)

    span = kw // len(p_refs)

    def prob_tasks(n):
        def task(r, c):
            rows = []
            for a in range(PARTS):
                rr = slice(a * bq + r, a * bq + r + 16)
                m, scale = pace.after(stat_ref[0, rr, :]), stat_ref[1, rr, :]
                cols = [b * kw + n * span + c for b in range(PARTS)]
                rows.append(jnp.concatenate([jnp.exp2(s_ref[rr, col:col + 128] - m) * scale for col in cols], axis=1))
            zs = _operands(jnp.concatenate(rows, axis=0), "a")
            for j, z in enumerate(zs):
                p_refs[n][j, c // 128, r:r + 16, :] = z.astype(BF16)
            if r + 16 == bq and c + 128 == span:
                fence(p_refs[n], zs[-1][0:8])
            return [z[0:8] for z in zs[6::7]]
        return [(functools.partial(task, r, c), 80) for r in range(0, bq, 16) for c in range(0, span, 128)]

    maxes = [(functools.partial(max_task, r), 3) for r in range(0, bm, 16)]
    stats = maxes[:2]
    for n, r in enumerate(range(0, bm, 16)):
        stats += [(functools.partial(sum_task, r), 70)] + maxes[n + 2:n + 3]
    stats += [(functools.partial(scale_task, r), 4) for r in range(0, bm, 16)]
    probs = prob_tasks(0)
    pace.spread(stats + gates[:1] + convs[-late:] + probs, (3 * nl + nl // 2 - 1) * (bm // 16), lag=10, parts=4)
    fence(hg_ref, project(pace, xn_ref, W_G, hg_ref, range(nl), untied=1))
    assert len(pace.tasks) >= 1 + late + len(probs)
    project(pace, xn_ref, W_Q, hq_ref, range(nl))
    fence(hq_ref, pace.recent[-1])
    project(pace, xn_ref, W_U, hu_ref, range(nl))
    fence(hu_ref, pace.recent[-1])
    assert len(pace.tasks) <= len(probs)
    fence(uc_ref, pace.recent[-1])
    project(pace, uc_ref, W_CONV, yc_ref, range(nl // 2))

    share = Tp // (nq - 1)
    assert share * (nq - 1) == Tp and share % 16 == 0 and 2 * bm <= share * (nq - 3)
    batch = jnp.where(i == 0, step // nq, jnp.minimum(step // nq + 1, B - 1))
    norms = norm_tasks(batch * Tp + jnp.maximum(i - 1, 0) * share, share, pace.after)
    later = (block_tasks(block_row(jnp.minimum(step + 2, B * nq - 1)), None) + norms[8:]
             + _merge(gates[1:], query_tasks()) + shift_tasks())
    cut = int(0.22 * len(later))
    for n, p_ref in enumerate(p_refs):
        if n == 0:
            pace.spread(_merge(prob_tasks(1), later[:cut] + norms[:8]), PRODUCTS * (bq // 16), lag=36, back=3, parts=7)
        else:
            pace.spread(later[cut:], PRODUCTS * (bq // 16), lag=20, back=2, parts=4)
        for j in [a * 7 + b for a in (6, 0, 3, 4, 2, 1, 5) for b in (4, 6, 5, 3, 2, 1, 0)]:
            t = pace.seen(_dot(pace.tie(_get(p_ref, (j,), bq)), _rows(_tile(kv_ref, (j,), n * span, span))))
            t = t if n == 0 else acc_ref[j] + t
            acc_ref[j] = t
        fence(acc_ref, t)

    def out_task(r):
        o = _assemble(lambda j: acc_ref[j, r:r + 16, :], ((0, 3, 4, 6, 2, 1, 5),) * LEVELS)
        out = []
        for a in range(PARTS):
            y = o[16 * a:16 * a + 16]
            _put(ob_ref, (), a * bq + r, y)
            out += _vregs(y[8:16])
        if r + 16 == bq:
            fence(ob_ref, y)
        return out
    pace.spread([(functools.partial(out_task, r), 1) for r in range(0, bq, 16)], (nl - nl // 2) * (bm // 16), lag=14, parts=8)
    fence(yc_ref, project(pace, uc_ref, W_CONV, yc_ref, range(nl // 2, nl)))
    pace.spread(u_tasks(pace.after), (nl - 1) * (bm // 16), lag=3, parts=4)
    for c in range(nl):
        lanes = slice(c * 128, (c + 1) * 128)
        lhs = _get(ob_ref, (), bm)
        ya = _dot(pace.tie(lhs) if c else _rows(lhs), _rows(_tile(w_ref, (W_ATT, c), 0, D)))
        for r in range(0, bm, 16):
            x = x_ref[rows16(block_row(step) + r), lanes].astype(F32)
            o_ref[r:r + 16, lanes] = (x + (yc_ref[r:r + 16, lanes] + ya[r:r + 16])).astype(o_ref.dtype)
    assert pace.idle()


@jax.jit
def pallas_standalone__conformer_family_branchformer__speech_kernel(
    x: jax.Array,
    w_q: jax.Array,
    w_k: jax.Array,
    w_v: jax.Array,
    w_ao: jax.Array,
    w_up: jax.Array,
    dw: jax.Array,
    w_dn: jax.Array,
    w_merge: jax.Array,
):
    B, T, D = x.shape
    weights = (w_q, w_k, w_v, w_ao, w_up, dw, w_dn, w_merge)
    assert all(a.dtype == BF16 for a in (x, *weights)) and D == 128 * PARTS and dw.shape[0] < 2 * HALO
    bm, bq = BLOCK, BLOCK // PARTS
    Tp = pl.cdiv(T, 256 * PARTS) * 256 * PARTS
    nq = pl.cdiv(T, bm)
    return pl.pallas_call(
        _kernel,
        grid=(B * nq,),
        in_specs=[pl.BlockSpec(memory_space=pl.ANY)] * (1 + len(weights)),
        out_specs=pl.BlockSpec((None, bm, D), lambda s: (s // nq, s % nq, 0)),
        out_shape=jax.ShapeDtypeStruct(x.shape, x.dtype),
        scratch_shapes=[pltpu.VMEM((B * Tp, D), BF16)] + [pltpu.VMEM((D, D), BF16)] * 7 + [
            pltpu.VMEM(dw.shape, BF16),
            pltpu.VMEM(w_merge.shape, BF16),
            pltpu.SemaphoreType.DMA((len(weights) + 3 * PARTS + B - 1,)),
            pltpu.VMEM((5, D // 128, D, 128), BF16),
            pltpu.VMEM((2 * HALO, D), F32),
            pltpu.VMEM((PRODUCTS, Tp // PARTS, 128), BF16),
            pltpu.VMEM((D // 128, bm + 16, 128), BF16),
            pltpu.VMEM((PRODUCTS, bq, 128), BF16),
            pltpu.VMEM((bm, D), F32),
            pltpu.VMEM((D // 128, bm + 16, 128), BF16),
            pltpu.VMEM((D // 128, bm + 2 * HALO, 128), F32),
            pltpu.VMEM((D // 128, bm + 8, 128), F32),
            pltpu.VMEM((bm + 8, Tp), F32),
            pltpu.VMEM((2, bm + 8, 128), F32),
            pltpu.VMEM((bm + 8, D), F32),
            pltpu.VMEM((bm + 8, D), F32),
            pltpu.VMEM((bm + 8, D), F32),
            pltpu.VMEM((bm + 8, D), F32),
            pltpu.VMEM((PRODUCTS + 1, bq, 128), F32),
            pltpu.VMEM((D // 128, bm + 16, 128), BF16),
            pltpu.VMEM((B * Tp, D), F32),
        ] + [pltpu.VMEM((PRODUCTS + 1, Tp // PARTS // 256, bq, 128), BF16)] * 2,
        compiler_params=pltpu.CompilerParams(dimension_semantics=("arbitrary",), vmem_limit_bytes=110 * 2**20),
    )(x, *weights)
```

```python
import functools
import math

import jax
import jax.numpy as jnp
from jax import lax
from jax.experimental import pallas as pl
from jax.experimental.pallas import tpu as pltpu

F32, BF16, U32 = jnp.float32, jnp.bfloat16, jnp.uint32
EPS = 1e-5
LOG2E = 1.4426950408889634
HALO = 16
LEVELS = 2
PARTS = 2 ** LEVELS
PRODUCTS = 7 ** LEVELS
BLOCK = 448
W_Q, W_U, W_G, W_ATT, W_CONV = range(5)


def _layernorm(x):
    c = x - jnp.mean(x, axis=-1, keepdims=True)
    return c * lax.rsqrt(jnp.mean(c * c, axis=-1, keepdims=True) + EPS)


def _gelu(x):
    c0 = math.sqrt(2.0 / math.pi)
    inner = x * (c0 + (c0 * 0.044715) * (x * x))
    half = 0.5 * x
    return half + half * jnp.tanh(inner)


def _dot(a, b):
    return jnp.dot(a, b, preferred_element_type=F32)


def _dot_nt(a, b):
    return lax.dot_general(a, b, (((1,), (1,)), ((), ())), preferred_element_type=F32)


def _words(x):
    return pltpu.bitcast(x, U32)


def _rows(words):
    return pltpu.bitcast(words, BF16)


def _put(ref, idx, r, x):
    for c in range(x.shape[1] // 128):
        ref[(*idx, c, slice(r, r + x.shape[0]))] = x[:, c * 128:(c + 1) * 128].astype(BF16)


def _tile(ref, idx, r, n):
    return ref.bitcast(U32)[(*idx, slice(r // 2, (r + n) // 2))]


def _get(ref, idx, n):
    return jnp.concatenate([_tile(ref, (*idx, c), 0, n) for c in range(ref.shape[-3])], axis=1)


def _vregs(x):
    return [x[r:r + 8, c:c + 128] for r in range(0, x.shape[0], 8) for c in range(0, x.shape[1], 128)]


def _operands(x, kind, level=LEVELS):
    if level == 0:
        return [x]
    r, c = x.shape[0] // 2, x.shape[1] // 2
    x11, x12, x21, x22 = x[:r, :c], x[:r, c:], x[r:, :c], x[r:, c:]
    if kind == "a":
        sums = [x11 + x22, x21 + x22, x11, x22, x11 + x12, x21 - x11, x12 - x22]
    elif kind == "b":
        sums = [x11 + x22, x11, x12 - x22, x21 - x11, x22, x11 + x12, x21 + x22]
    else:
        sums = [x11 + x22, x11, x21 - x22, x12 - x11, x22, x11 + x21, x12 + x22]
    return [z for s in sums for z in _operands(s, kind, level - 1)]


def _a_as_b(j, level=LEVELS):
    if level == 0:
        return 0
    n = 7 ** (level - 1)
    return (0, 6, 1, 4, 5, 3, 2)[j // n] * n + _a_as_b(j % n, level - 1)


_TERMS = (((0, 1), (3, 1), (4, -1), (6, 1)), ((2, 1), (4, 1)), ((1, 1), (3, 1)), ((0, 1), (1, -1), (2, 1), (5, 1)))


def _assemble(product, orders, transposed=False, base=0):
    if not orders:
        return product(base)
    n = 7 ** (len(orders) - 1)
    quads = [None] * 4
    for j in orders[0]:
        m = _assemble(product, orders[1:], transposed, base + j * n)
        for k, terms in enumerate(_TERMS):
            for i, sign in terms:
                if i == j and quads[k] is None:
                    quads[k] = (m, sign)
                elif i == j:
                    t, tsign = quads[k]
                    quads[k] = (t + m, sign) if sign == tsign else (t - m, 1) if tsign > 0 else (m - t, 1)
    assert all(sign > 0 for _, sign in quads)
    c11, c12, c21, c22 = [t for t, _ in quads]
    if transposed:
        c12, c21 = c21, c12
    return jnp.concatenate([jnp.concatenate([c11, c12], axis=1), jnp.concatenate([c21, c22], axis=1)], axis=0)


class _Pacer:
    def __init__(self, zero):
        self.keep = lax.broadcasted_iota(jnp.int32, (8, 128), 0) >= zero
        self.tasks, self.due, self.recent = [], [], []
        self.rate = self.credit = self.slot = self.back = 0

    def idle(self):
        return not self.tasks and not self.due

    def spread(self, tasks, slots, lag=0, back=0, parts=1):
        assert self.idle()
        self.tasks = list(tasks)
        self.rate = sum(c for _, c in tasks) / (slots - lag)
        self.credit = tasks[0][1]
        self.slot, self.end, self.lag, self.back, self.parts = 0, slots - 1, lag, back, parts

    def seen(self, y):
        self.recent.append(y[0:8, 0:128])
        return y

    def after(self, x):
        token = pltpu.bitcast(self.recent[max(0, len(self.recent) - 1 - self.back)], x.dtype)
        return jnp.concatenate([jnp.concatenate(
            [jnp.where(self.keep, x[r:r + 8, c:c + 128], token) for c in range(0, x.shape[1], 128)], axis=1)
            for r in range(0, x.shape[0], 8)], axis=0)

    @staticmethod
    def _any(xs):
        chains = [functools.reduce(lambda a, b: a | b, xs[n::2]) for n in range(min(2, len(xs)))]
        return functools.reduce(lambda a, b: a | b, chains)

    def tie(self, lhs):
        rows = []
        for r in range(0, lhs.shape[0], 8):
            while self.tasks and self.credit >= self.tasks[0][1] * (1 - 1e-6):
                fn, cost = self.tasks.pop(0)
                self.credit -= cost
                out = [pltpu.bitcast(v, U32) for v in fn()]
                n = min(len(out), self.parts)
                for m in range(n):
                    when = min(self.end, self.slot + self.lag + m * cost / self.rate / n)
                    self.due.append((when, self._any(out[m * len(out) // n:(m + 1) * len(out) // n])))
                self.due.sort(key=lambda d: d[0])
            token = None
            while self.due and self.due[0][0] <= self.slot:
                t = self.due.pop(0)[1]
                token = t if token is None else token | t
            self.slot += 1
            self.credit += self.rate
            t = lhs[r:r + 8]
            if token is not None:
                t0 = jnp.where(self.keep, t[:, 0:128], token)
                t = t0 if t.shape[1] == 128 else jnp.concatenate([t0, t[:, 128:]], axis=1)
            rows.append(t)
        return _rows(jnp.concatenate(rows, axis=0))


def _merge(xs, ys):
    keyed = [((n + 0.5) / len(xs), 0, n) for n in range(len(xs))] + [((n + 0.5) / len(ys), 1, n) for n in range(len(ys))]
    return [(xs, ys)[w][n] for _, w, n in sorted(keyed)]


def _run(tasks):
    for fn, _ in tasks:
        fn()


def _kernel(x_hbm, wq_hbm, wk_hbm, wv_hbm, wao_hbm, wup_hbm, dw_hbm, wdn_hbm, wm_hbm, o_ref,
            x_ref, wq_ref, wk_ref, wv_ref, wao_ref, wu_ref, wg_ref, wdn_ref, dw_ref, wm_ref, sems,
            w_ref, taps_ref, kv_ref, xn_ref, q_ref, u_ref, uc_ref, g_ref, gn_ref, s_ref,
            stat_ref, yc_ref, hg_ref, hq_ref, hu_ref, acc_ref, ob_ref, ln_ref, *p_refs):
    step = pl.program_id(0)
    B, T, D = x_hbm.shape
    K = dw_ref.shape[0]
    Tp = s_ref.shape[1]
    bm, bq = BLOCK, BLOCK // PARTS
    kw = Tp // PARTS
    nq = pl.cdiv(T, bm)
    nl = D // 128
    pad = K // 2
    i = step % nq
    zero = pl.multiple_of(jnp.minimum(step, 0) * 16, 16)

    def block_row(n):
        return (n // nq) * Tp + (n % nq) * bm

    def rows16(r):
        return pl.ds(r if isinstance(r, int) else pl.multiple_of(r, 16), 16)

    def fence(ref, val):
        val = pltpu.bitcast(val[-8:, -128:], ref.dtype)
        rows = val.shape[0]
        ref[tuple(n - 1 for n in ref.shape[:-2]) + (pl.ds(zero + ref.shape[-2] - rows, rows), pl.ds(0, 128))] = val

    def x_rows(r, gate):
        return _rows(gate(_words(x_ref[rows16(r), :]))).astype(F32)


    def block_tasks(r0, normalise):
        def task(r):
            y = _layernorm(x_rows(r0 + r, normalise)) if normalise else ln_ref[rows16(r0 + r), :]
            _put(xn_ref, (), r, y)
            if r + 16 == bm:
                fence(xn_ref, y)
            return _vregs(y[0:8])
        return [(functools.partial(task, r), 40 if normalise else 4) for r in range(0, bm, 16)]

    def norm_tasks(r0, n, gate):
        def task(r):
            y = _layernorm(x_rows(r0 + r, gate))
            ln_ref[rows16(r0 + r), :] = y
            return _vregs(y)
        return [(functools.partial(task, r), 50) for r in range(0, n, 16)]

    def gate_tasks(gate):
        def task(r):
            g = _layernorm(_gelu(gate(hg_ref[r:r + 16, :])))
            for c in range(nl):
                gn_ref[c, r:r + 16, :] = g[:, c * 128:(c + 1) * 128]
                if r < HALO:
                    g_ref[c, HALO + bm + r:HALO + bm + r + 16, :] = g[:, c * 128:(c + 1) * 128]
            if r + 16 == bm:
                fence(gn_ref, g)
            return _vregs(g)
        return [(functools.partial(task, r), 50) for r in range(0, bm, 16)]

    def shift_tasks():
        def move(src, r, dst, n):
            out = []
            for c in range(nl):
                y = src[c, r:r + n, :]
                g_ref[c, dst:dst + n, :] = y
                out += _vregs(y)
            return out
        return ([(functools.partial(move, g_ref, bm, 0, HALO), 8)]
                + [(functools.partial(move, gn_ref, r, HALO + r, 32), 16) for r in range(0, bm, 32)])

    def u_tasks(gate):
        def task(r):
            y = _gelu(gate(hu_ref[r:r + 16, :]))
            u_ref[r:r + 16, :] = y
            return _vregs(y)
        return [(functools.partial(task, r), 24) for r in range(0, bm, 16)]

    def query_tasks():
        def task(r):
            x = jnp.concatenate([hq_ref[a * bq + r:a * bq + r + 16, :] for a in range(PARTS)], axis=0)
            zs = _operands(x, "bt")
            for j, z in enumerate(zs):
                q_ref[j, r:r + 16, :] = z.astype(BF16)
            return [z[0:8] for z in zs[::2]]
        return [(functools.partial(task, r), 40) for r in range(0, bq, 16)]

    def key_tasks(base, r0, n, normalise):
        def task(r):
            rows = [base + a * kw + r0 + r for a in range(PARTS)]
            if normalise:
                xs = [_layernorm(x_rows(row, normalise)) for row in rows]
                for row, y in zip(rows, xs):
                    ln_ref[rows16(row), :] = y
            else:
                xs = [ln_ref[rows16(row), :] for row in rows]
            zs = _operands(jnp.concatenate(xs, axis=0), "b")
            for j, z in enumerate(zs):
                kv_ref[j, rows16(r0 + r), :] = z.astype(BF16)
            return [v for z in zs[::2] for v in _vregs(z)]
        return [(functools.partial(task, r), 160) for r in range(0, n, 16)]

    def project(pacer, src, w, dst, cols, untied=0):
        for n, c in enumerate(cols):
            lhs = _rows(_get(src, (), bm)) if n < untied else pacer.tie(_get(src, (), bm))
            y = pacer.seen(_dot(lhs, _rows(_tile(w_ref, (w, c), 0, D))))
            dst[0:bm, c * 128:(c + 1) * 128] = y
        return y

    copies = []

    def fetch(src, dst):
        copies.append(pltpu.make_async_copy(src, dst, sems.at[len(copies)]))
        return copies[-1]

    def fetch_x(b, r0, r1):
        return fetch(x_hbm.at[b, pl.ds(r0, r1 - r0)], x_ref.at[pl.ds(b * Tp + r0, r1 - r0)])

    def start(group):
        for c in group:
            c.start()

    def wait(group):
        for c in group:
            c.wait()

    cuts = (384, 832)

    def fetch_keys(r0, r1):
        return [fetch_x(0, a * kw + r0, min(T, a * kw + r1)) for a in range(1, PARTS)]

    group = [
        [fetch_x(0, 0, bm)],
        [fetch(wup_hbm.at[:, pl.ds(D, D)], wg_ref)],
        [fetch(wup_hbm.at[:, pl.ds(0, D)], wu_ref)],
        [fetch(wq_hbm, wq_ref), fetch(wk_hbm, wk_ref)] + fetch_keys(0, cuts[0]),
        [fetch(wv_hbm, wv_ref), fetch(wao_hbm, wao_ref), fetch_x(0, bm, kw)] + fetch_keys(*cuts),
        [fetch(wdn_hbm, wdn_ref), fetch(wm_hbm, wm_ref), fetch(dw_hbm, dw_ref)],
        fetch_keys(cuts[1], kw),
    ]
    assert cuts[0] <= bm and 2 * bm <= kw
    batches = [fetch_x(b, 0, T) for b in range(1, B)]

    @pl.when(step == 0)
    def _():
        start(group[0] + group[1])
        for b in range(B):
            x_ref[b * Tp + T:(b + 1) * Tp, :] = jnp.zeros((Tp - T, D), x_ref.dtype)
        for c in range(nl):
            g_ref[c, bm:bm + HALO, :] = jnp.zeros((HALO, 128), F32)
        wait(group[0])
        start(group[2] + group[3])
        early = _Pacer(zero)

        def weights(lhs, rhs_ref, r0):
            cols = [_dot(early.tie(lhs), rhs_ref[r0:r0 + D, c:c + 128]) for c in range(0, D, 128)]
            return jnp.concatenate([early.seen(y) for y in cols], axis=1)

        _run(block_tasks(0, lambda w: w))
        wait(group[1])
        start(group[4])
        _put(w_ref, (W_G,), 0, wg_ref[...])
        fence(hg_ref, project(early, xn_ref, W_G, hg_ref, range(nl)))
        wait(group[2])
        _put(w_ref, (W_U,), 0, wu_ref[...])
        early.spread(gate_tasks(early.after), nl * (bm // 16), lag=14, parts=2)
        fence(hu_ref, project(early, xn_ref, W_U, hu_ref, range(nl)))
        wait(group[3])
        start(group[5])
        early.spread(u_tasks(early.after) + shift_tasks() + key_tasks(0, 0, cuts[0], early.after),
                     D // 16 + nl * (bm // 16), lag=8, parts=12)
        qk = _dot_nt(early.tie(_words(wq_ref[...])), wk_ref[...])
        _put(w_ref, (W_Q,), 0, qk * (LOG2E * float(D) ** -0.5))
        fence(hq_ref, project(early, xn_ref, W_Q, hq_ref, range(nl)))
        wait(group[4])
        start(group[6])
        early.spread(query_tasks() + block_tasks(bm, early.after) + key_tasks(0, cuts[0], cuts[1] - cuts[0], early.after),
                     3 * nl * (D // 16), lag=8, parts=12)
        vo = weights(_words(wv_ref[...]), wao_ref, 0)
        wait(group[5])
        taps_ref[0:K, :] = dw_ref[...].astype(F32)
        _put(w_ref, (W_CONV,), 0, weights(_words(wdn_ref[...]), wm_ref, D))
        _put(w_ref, (W_ATT,), 0, weights(_words(vo.astype(BF16)), wm_ref, 0))
        assert early.idle()
        wait(group[6])
        start(batches)

        @pl.loop(cuts[1] // 64, kw // 64)
        def _(j):
            _run(key_tasks(0, j * 64, 64, lambda w: w))

    for n, copy in enumerate(batches):
        pl.when(step == n * nq + 1)(copy.wait)

    @pl.when(jnp.logical_and(i == 0, step > 0))
    def _():
        @pl.loop(0, kw // 16)
        def _(j):
            _run(key_tasks(block_row(step), j * 16, 16, None))

    pace = _Pacer(zero)
    gates = gate_tasks(pace.after)

    def conv_task(c, r):
        lanes = slice(c * 128, (c + 1) * 128)
        acc, partial = None, []
        for shift in range(8):
            if shift:
                partial.append(acc[0:8])
            taps = [k for k in range(K) if (HALO - pad + k) % 8 == shift]
            lo = HALO - pad + taps[0] + r
            window = g_ref[c, lo:lo + 16 + 8 * (len(taps) - 1), :]
            for n, k in enumerate(taps):
                t = window[8 * n:8 * n + 16] * taps_ref[k:k + 1, lanes]
                acc = t if acc is None else acc + t
        y = u_ref[r:r + 16, lanes] * acc
        uc_ref[c, r:r + 16, :] = y.astype(BF16)
        return partial + [y[0:8]]
    convs = [(functools.partial(conv_task, c, r), 48) for r in range(0, bm, 16) for c in range(nl)]
    late = nl * pl.cdiv(pad, 16)
    pace.spread(convs[:-late], PRODUCTS * (kw // 128) * (bq // 16), parts=8)

    peak = None
    for c0 in range(0, kw, 128):
        def product(j):
            return pace.seen(_dot_nt(pace.tie(_tile(q_ref, (j,), 0, bq)), _rows(_tile(kv_ref, (_a_as_b(j),), c0, 128))))
        s = _assemble(product, ((1, 3, 2, 4, 0, 5, 6), (2, 5, 4, 1, 0, 3, 6)), transposed=True)
        tiles = []
        for a in range(PARTS):
            t = s[:, a * 128:(a + 1) * 128]
            col0 = a * kw + c0
            if col0 + 128 > T:
                t = jnp.where(col0 + lax.broadcasted_iota(jnp.int32, t.shape, 1) < T, t, -jnp.inf)
            s_ref[0:bm, col0:col0 + 128] = t
            tiles.append(t)
        for n in range(0, PARTS, 2):
            t = jnp.maximum(tiles[n], tiles[n + 1])
            peak = t if peak is None else jnp.maximum(peak, t)
    fence(s_ref, tiles[-1])
    stat_ref[0, 0:bm, :] = peak
    fence(stat_ref, peak)

    rowmax, rowsum = {}, {}

    def max_task(r):
        rowmax[r] = jnp.broadcast_to(jnp.max(stat_ref[0, r:r + 16, :], axis=-1, keepdims=True), (16, 128))
        return _vregs(rowmax[r])

    def sum_task(r):
        total = None
        for c in range(0, Tp, 128):
            e = jnp.exp2(s_ref[r:r + 16, c:c + 128] - rowmax[r])
            total = e if total is None else total + e
        rowsum[r] = total
        return _vregs(total)

    def scale_task(r):
        scale = jnp.broadcast_to(1.0 / jnp.sum(pace.after(rowsum[r]), axis=-1, keepdims=True), (16, 128))
        stat_ref[0, r:r + 16, :] = rowmax[r]
        stat_ref[1, r:r + 16, :] = scale
        if r + 16 == bm:
            fence(s_ref, scale)
            fence(stat_ref, scale)
        return _vregs(scale)

    span = kw // len(p_refs)

    def prob_tasks(n):
        def task(r, c):
            rows = []
            for a in range(PARTS):
                rr = slice(a * bq + r, a * bq + r + 16)
                m, scale = pace.after(stat_ref[0, rr, :]), stat_ref[1, rr, :]
                cols = [b * kw + n * span + c for b in range(PARTS)]
                rows.append(jnp.concatenate([jnp.exp2(s_ref[rr, col:col + 128] - m) * scale for col in cols], axis=1))
            zs = _operands(jnp.concatenate(rows, axis=0), "a")
            for j, z in enumerate(zs):
                p_refs[n][j, c // 128, r:r + 16, :] = z.astype(BF16)
            if r + 16 == bq and c + 128 == span:
                fence(p_refs[n], zs[-1][0:8])
            return [z[0:8] for z in zs[6::7]]
        return [(functools.partial(task, r, c), 80) for r in range(0, bq, 16) for c in range(0, span, 128)]

    maxes = [(functools.partial(max_task, r), 3) for r in range(0, bm, 16)]
    stats = maxes[:2]
    for n, r in enumerate(range(0, bm, 16)):
        stats += [(functools.partial(sum_task, r), 70)] + maxes[n + 2:n + 3]
    stats += [(functools.partial(scale_task, r), 4) for r in range(0, bm, 16)]
    probs = prob_tasks(0)
    pace.spread(stats + gates[:1] + convs[-late:] + probs, (3 * nl + nl // 2 - 1) * (bm // 16), lag=10, parts=4)
    fence(hg_ref, project(pace, xn_ref, W_G, hg_ref, range(nl), untied=1))
    assert len(pace.tasks) >= 1 + late + len(probs)
    project(pace, xn_ref, W_Q, hq_ref, range(nl))
    fence(hq_ref, pace.recent[-1])
    project(pace, xn_ref, W_U, hu_ref, range(nl))
    fence(hu_ref, pace.recent[-1])
    assert len(pace.tasks) <= len(probs)
    fence(uc_ref, pace.recent[-1])
    project(pace, uc_ref, W_CONV, yc_ref, range(nl // 2))

    share = Tp // (nq - 1)
    assert share * (nq - 1) == Tp and share % 16 == 0 and 2 * bm <= share * (nq - 3)
    batch = jnp.where(i == 0, step // nq, jnp.minimum(step // nq + 1, B - 1))
    norms = norm_tasks(batch * Tp + jnp.maximum(i - 1, 0) * share, share, pace.after)
    later = (block_tasks(block_row(jnp.minimum(step + 2, B * nq - 1)), None) + norms[8:]
             + _merge(gates[1:], query_tasks()) + shift_tasks())
    cut = int(0.22 * len(later))
    for n, p_ref in enumerate(p_refs):
        if n == 0:
            pace.spread(_merge(prob_tasks(1), later[:cut] + norms[:8]), PRODUCTS * (bq // 16), lag=36, back=3, parts=7)
        else:
            pace.spread(later[cut:], PRODUCTS * (bq // 16), lag=20, back=2, parts=4)
        for j in [a * 7 + b for a in (6, 0, 3, 4, 2, 1, 5) for b in (4, 6, 5, 3, 2, 1, 0)]:
            t = pace.seen(_dot(pace.tie(_get(p_ref, (j,), bq)), _rows(_tile(kv_ref, (j,), n * span, span))))
            t = t if n == 0 else acc_ref[j] + t
            acc_ref[j] = t
        fence(acc_ref, t)

    def out_task(r):
        o = _assemble(lambda j: acc_ref[j, r:r + 16, :], ((0, 3, 4, 6, 2, 1, 5),) * LEVELS)
        out = []
        for a in range(PARTS):
            y = o[16 * a:16 * a + 16]
            _put(ob_ref, (), a * bq + r, y)
            out += _vregs(y[8:16])
        if r + 16 == bq:
            fence(ob_ref, y)
        return out
    pace.spread([(functools.partial(out_task, r), 1) for r in range(0, bq, 16)], (nl - nl // 2) * (bm // 16), lag=14, parts=8)
    fence(yc_ref, project(pace, uc_ref, W_CONV, yc_ref, range(nl // 2, nl)))
    pace.spread(u_tasks(pace.after), (nl - 1) * (bm // 16), lag=3, parts=4)
    for c in range(nl):
        lanes = slice(c * 128, (c + 1) * 128)
        lhs = _get(ob_ref, (), bm)
        ya = _dot(pace.tie(lhs) if c else _rows(lhs), _rows(_tile(w_ref, (W_ATT, c), 0, D)))
        for r in range(0, bm, 16):
            x = x_ref[rows16(block_row(step) + r), lanes].astype(F32)
            o_ref[r:r + 16, lanes] = (x + (yc_ref[r:r + 16, lanes] + ya[r:r + 16])).astype(o_ref.dtype)
    assert pace.idle()


@jax.jit
def pallas_standalone__conformer_family_branchformer__speech_kernel(
    x: jax.Array,
    w_q: jax.Array,
    w_k: jax.Array,
    w_v: jax.Array,
    w_ao: jax.Array,
    w_up: jax.Array,
    dw: jax.Array,
    w_dn: jax.Array,
    w_merge: jax.Array,
):
    B, T, D = x.shape
    weights = (w_q, w_k, w_v, w_ao, w_up, dw, w_dn, w_merge)
    assert all(a.dtype == BF16 for a in (x, *weights)) and D == 128 * PARTS and dw.shape[0] < 2 * HALO
    bm, bq = BLOCK, BLOCK // PARTS
    Tp = pl.cdiv(T, 256 * PARTS) * 256 * PARTS
    nq = pl.cdiv(T, bm)
    assert T + HALO <= nq * bm <= Tp
    return pl.pallas_call(
        _kernel,
        grid=(B * nq,),
        in_specs=[pl.BlockSpec(memory_space=pl.ANY)] * (1 + len(weights)),
        out_specs=pl.BlockSpec((None, bm, D), lambda s: (s // nq, s % nq, 0)),
        out_shape=jax.ShapeDtypeStruct(x.shape, x.dtype),
        scratch_shapes=[pltpu.VMEM((B * Tp, D), BF16)] + [pltpu.VMEM((D, D), BF16)] * 7 + [
            pltpu.VMEM(dw.shape, BF16),
            pltpu.VMEM(w_merge.shape, BF16),
            pltpu.SemaphoreType.DMA((len(weights) + 3 * PARTS + B - 1,)),
            pltpu.VMEM((5, D // 128, D, 128), BF16),
            pltpu.VMEM((2 * HALO, D), F32),
            pltpu.VMEM((PRODUCTS, Tp // PARTS, 128), BF16),
            pltpu.VMEM((D // 128, bm + 16, 128), BF16),
            pltpu.VMEM((PRODUCTS, bq, 128), BF16),
            pltpu.VMEM((bm, D), F32),
            pltpu.VMEM((D // 128, bm + 16, 128), BF16),
            pltpu.VMEM((D // 128, bm + 2 * HALO, 128), F32),
            pltpu.VMEM((D // 128, bm + 8, 128), F32),
            pltpu.VMEM((bm + 8, Tp), F32),
            pltpu.VMEM((2, bm + 8, 128), F32),
            pltpu.VMEM((bm + 8, D), F32),
            pltpu.VMEM((bm + 8, D), F32),
            pltpu.VMEM((bm + 8, D), F32),
            pltpu.VMEM((bm + 8, D), F32),
            pltpu.VMEM((PRODUCTS + 1, bq, 128), F32),
            pltpu.VMEM((D // 128, bm + 16, 128), BF16),
            pltpu.VMEM((B * Tp, D), F32),
        ] + [pltpu.VMEM((PRODUCTS + 1, Tp // PARTS // 256, bq, 128), BF16)] * 2,
        compiler_params=pltpu.CompilerParams(dimension_semantics=("arbitrary",), vmem_limit_bytes=110 * 2**20),
    )(x, *weights)
```
